```python
import jax
import jax.numpy as jnp

def _softmax(x, axis=-1):
    return jax.nn.softmax(x, axis=axis)

def _gelu(x):
    return jax.nn.gelu(x, approximate=True)

def _silu(x):
    return jax.nn.silu(x)

def _sigmoid(x):
    return jax.nn.sigmoid(x)

def _layernorm(x, axis=-1, eps=1e-05):
    m = jnp.mean(x, axis=axis, keepdims=True)
    v = jnp.var(x, axis=axis, keepdims=True)
    return (x - m) / jnp.sqrt(v + eps)

def _scatter_add(tgt, idx, src, axis=0):
    return tgt.at[idx].add(src)

def _segment_sum(src, seg, n):
    return jax.ops.segment_sum(src, seg, n)

class _Rng:

    def __init__(self, key):
        self._k = key

    def _next(self):
        self._k, sub = jax.random.split(self._k)
        return sub

    def normal(self, shape):
        return jax.random.normal(self._next(), shape, dtype=jnp.bfloat16)

    def randint(self, lo, hi, shape):
        return jax.random.randint(self._next(), shape, lo, hi, dtype=jnp.int32)

    def uniform(self, shape, lo=0.0, hi=1.0):
        return jax.random.uniform(self._next(), shape, jnp.bfloat16, lo, hi)

    def permutation(self, n):
        return jax.random.permutation(self._next(), n)
kernel_name = 'concat_heads__memory_aug_recurrent_mem_tr__ssm_conv_h3__prompt'

def setup_inputs():
    _rng = _Rng(jax.random.key(int.from_bytes(__import__("os").urandom(4), "little")))
    _w = lambda a: (lambda t: t.astype(jnp.bfloat16) if jnp.issubdtype(t.dtype, jnp.floating) else t)(jnp.asarray(a))

    def _A_setup():
        B, S, Dm = (1, 2048, 1024)
        H, Dh = (32, 128)
        M, seg = (8, 32)
        seg = min(seg, S)
        S = S // seg * seg
        return {'x': _w((lambda *s: _rng.normal(s) * 0.05)(B, S, Dm)), 'mem0': _w((lambda *s: _rng.normal(s) * 0.05)(B, M, Dm)), 'Wq': _w((lambda *s: _rng.normal(s) * 0.05)(Dm, H, Dh) * Dm ** (-0.5)), 'Wk': _w((lambda *s: _rng.normal(s) * 0.05)(Dm, H, Dh) * Dm ** (-0.5)), 'Wv': _w((lambda *s: _rng.normal(s) * 0.05)(Dm, H, Dh) * Dm ** (-0.5)), 'Wo': _w((lambda *s: _rng.normal(s) * 0.05)(H, Dh, Dm) * (H * Dh) ** (-0.5)), 'seg_len': seg}
    _A_in = _A_setup()

    def _B_setup():
        B, S, D = (1, 2048, 1024)
        ks = 4
        return {'q': _w((lambda *s: _rng.normal(s) * 0.05)(B, S, D)), 'k': _w((lambda *s: _rng.normal(s) * 0.05)(B, S, D)), 'v': _w((lambda *s: _rng.normal(s) * 0.05)(B, S, D)), 'shift_k': _w((lambda *s: _rng.normal(s) * 0.05)(D, ks) * 0.5), 'ssm_k': _w((lambda *s: _rng.normal(s) * 0.05)(D, S) * (1.0 / S ** 0.5)), 'ssm_D': _w((lambda *s: _rng.normal(s) * 0.05)(D))}
    _B_in = _B_setup()
    return {'A_x': _A_in['x'], 'A_mem0': _A_in['mem0'], 'A_Wq': _A_in['Wq'], 'A_Wk': _A_in['Wk'], 'A_Wv': _A_in['Wv'], 'A_Wo': _A_in['Wo'], 'A_seg_len': _A_in['seg_len'], 'B_q': _B_in['q'], 'B_k': _B_in['k'], 'B_v': _B_in['v'], 'B_shift_k': _B_in['shift_k'], 'B_ssm_k': _B_in['ssm_k'], 'B_ssm_D': _B_in['ssm_D']}

def reference(A_x, A_mem0, A_Wq, A_Wk, A_Wv, A_Wo, A_seg_len, B_q, B_k, B_v, B_shift_k, B_ssm_k, B_ssm_D):

    def _A_ref(x, mem0, Wq, Wk, Wv, Wo, seg_len):
        B, S, Dm = x.shape
        H, Dh = (Wq.shape[1], Wq.shape[2])
        M = mem0.shape[1]
        scale = Dh ** (-0.5)
        n_seg = S // seg_len
        L = M + seg_len
        idx = jnp.arange(L)
        mask = (idx[:, None] < M) | (idx[:, None] >= idx[None, :])
        mem = mem0
        outs = []
        for s in range(n_seg):
            xs = x[:, s * seg_len:(s + 1) * seg_len, :].copy()
            h = jnp.concatenate([mem, xs], axis=1)
            q = jnp.einsum('btd,dhe->bhte', h, Wq)
            k = jnp.einsum('btd,dhe->bhte', h, Wk)
            v = jnp.einsum('btd,dhe->bhte', h, Wv)
            scores = jnp.einsum('bhqe,bhke->bhqk', q, k) * scale
            scores = jnp.where(mask[None, None], scores, -1000000000.0)
            p = _softmax(scores, axis=-1)
            o = jnp.einsum('bhqk,bhke->bhqe', p, v)
            o = jnp.einsum('bhte,hed->btd', o, Wo)
            mem = o[:, :M, :].copy()
            outs.append(o[:, M:, :])
        return jnp.concatenate(outs, axis=1)

    def _B_ref(q, k, v, shift_k, ssm_k, ssm_D):
        B, S, D = q.shape
        ks = shift_k.shape[-1]
        k_pad = jnp.pad(k, ((0, 0), (ks - 1, 0), (0, 0)))
        k_shift = jnp.zeros_like(k)
        for t in range(ks):
            k_shift = k_shift + k_pad[:, t:t + S, :] * shift_k[:, ks - 1 - t][None, None, :]
        kv = k_shift * v
        L = 2 * S
        kv_pad = jnp.pad(kv, ((0, 0), (0, S), (0, 0)))
        kf_pad = jnp.pad(ssm_k, ((0, 0), (0, S)))
        kv_f = (lambda x, axes=(-2, -1): jnp.fft.rfft2(x.astype(jnp.float32), axes=axes))(kv_pad[:, None, :, :], axes=(1, 2))
        kf_f = (lambda x, axes=(-2, -1): jnp.fft.rfft2(x.astype(jnp.float32), axes=axes))(kf_pad[:, None, :], axes=(1, 2))
        kf_f = (lambda x, *d: x.transpose(*d))(kf_f, 1, 2, 0)
        y_f = kv_f * kf_f[None, :, :, :]
        y = (lambda x, s, axes=(-2, -1): jnp.fft.irfft2(x, s=s, axes=axes).astype(jnp.bfloat16))(y_f, (1, L), axes=(1, 2))[:, 0, :S, :]
        y = y + kv * ssm_D[None, None, :]
        return q * y
    a = _A_ref(A_x, A_mem0, A_Wq, A_Wk, A_Wv, A_Wo, A_seg_len)
    b = _B_ref(B_q, B_k, B_v, B_shift_k, B_ssm_k, B_ssm_D)
    return jnp.concatenate([a, b], axis=-1)
```

```python
import jax
import jax.numpy as jnp
import numpy as np
import ml_dtypes
from jax import lax
from jax.experimental import pallas as pl
from jax.experimental.pallas import tpu as pltpu

S, D, H, E, M, SEG = 2048, 1024, 32, 128, 8, 32
NSEG = S // SEG
FILL = 24
PRO = S - FILL * (NSEG - 1)
RING = 672
ROFF = 64
WS = 516
C = 128
NC = S // C
NT = D // 128
SKEW = tuple(int(c) for c in '2,3,4,5'.split(','))
BMODE = 'spread'
bf16, f32, u32 = jnp.bfloat16, jnp.float32, jnp.uint32


def head_of_slot(j):
    return (j // 16) * 16 + 2 * (j % 8) + ((j // 8) % 2)


def dft_consts():
    k = np.arange(C)[:, None].astype(np.float64)
    t = np.arange(C)[None, :].astype(np.float64)
    th = np.pi * (2 * k + 1) * t / (2 * C)
    F = np.concatenate([np.cos(th), -np.sin(th)], 0)
    G = np.concatenate([np.cos(th).T, -np.sin(th).T], 1) / C
    return F.astype(ml_dtypes.bfloat16), G.astype(ml_dtypes.bfloat16)


def kernel(x_hbm, mem0_hbm, wq_hbm, wk_hbm, wv_hbm, wo_hbm, k_hbm, v_hbm, q_hbm, h_hbm, sk_v, d_v, F_v, G_v,
           out_hbm,
           x_v, mem_v, wqkv, wo, wstage, wostage, ring, obuf_x, obuf, lo_scr, cur, sems, osem,
           kbuf, vbuf, hbuf, qbuf, bobuf, kf, kvbuf, xs, as_, ybuf, yprev, tapbuf, bsem):
    LO = 0xFFFF
    HI = np.uint32(0xFFFF0000)

    sgn = (1 - 2 * (lax.broadcasted_iota(jnp.int32, (8, 128), 0) % 2)).astype(f32)

    def in_dmas(t):
        sl = t % 2
        c0 = pl.multiple_of(t * 128, 128)
        return [pltpu.make_async_copy(k_hbm.at[:, pl.ds(c0, 128)], kbuf.at[sl], bsem.at[0, sl]),
                pltpu.make_async_copy(v_hbm.at[:, pl.ds(c0, 128)], vbuf.at[sl], bsem.at[1, sl]),
                pltpu.make_async_copy(h_hbm.at[pl.ds(c0, 128), :], hbuf.at[sl], bsem.at[2, sl])]

    def q_dma(t):
        sl = t % 2
        return pltpu.make_async_copy(q_hbm.at[:, pl.ds(pl.multiple_of(t * 128, 128), 128)], qbuf.at[sl], bsem.at[3, sl])

    def o_dma(t):
        sl = t % 2
        return pltpu.make_async_copy(bobuf.at[sl], out_hbm.at[:, pl.ds(pl.multiple_of(D + t * 128, 128), 128)], bsem.at[4, sl])

    def sp_k(sl, p):
        r0 = pl.multiple_of(p * 256, 256)
        kf[pl.ds(r0 + 8, 256), :] = kbuf[sl, pl.ds(r0, 256), :].astype(f32)

    def sp_x(t, sl, p, jj):
        w = [jnp.broadcast_to(tapbuf[t, j:j + 1, :], (8, 128)) for j in range(4)]
        r0 = pl.multiple_of(p * 256, 256)
        kvs = []
        for u in range(8):
            rows = []
            for hf in range(2):
                r = r0 + jj * 128 + u * 16 + hf * 8
                acc = kf[pl.ds(r + 5, 8), :] * w[3]
                acc = acc + kf[pl.ds(r + 6, 8), :] * w[2]
                acc = acc + kf[pl.ds(r + 7, 8), :] * w[1]
                acc = acc + kf[pl.ds(r + 8, 8), :] * w[0]
                rows.append(acc)
            ks = jnp.concatenate(rows, axis=0)
            vv = vbuf[sl, pl.ds(pl.multiple_of(r0 + jj * 128 + u * 16, 16), 16), :].astype(f32)
            kvs.append((ks * vv).astype(bf16))
        kv = jnp.concatenate(kvs, axis=0)
        kvbuf[sl, pl.ds(pl.multiple_of(r0 + jj * 128, 128), 128), :] = kv
        xs[sl, 2 * p + jj] = jnp.dot(F_v[...], kv, preferred_element_type=f32)

    def sp_a(sl, p, jj):
        j = 2 * p + jj
        hh = hbuf[sl, :, pl.ds(pl.multiple_of(j * 128, 128), 128)]
        as_[sl, j] = lax.dot_general(F_v[...], hh, (((1,), (1,)), ((), ())), preferred_element_type=f32)

    def cv(sl, p, b):
        i0 = 2 * p
        first = p == 0
        re = pl.ds(b * 8, 8)
        im = pl.ds(128 + b * 8, 8)
        y0r = y0i = y1r = y1i = None
        xr_prev = xs[sl, i0 + 1, re, :]
        xi_prev = xs[sl, i0 + 1, im, :]
        for l in range(NC):
            ar = as_[sl, l, re, :]
            ai = as_[sl, l, im, :]
            j = jnp.where(i0 - l >= 0, i0 - l, NC)
            xr = xs[sl, j, re, :]
            xim = xs[sl, j, im, :]
            p0r = ar * xr - ai * xim
            p0i = ar * xim + ai * xr
            p1r = ar * xr_prev - ai * xi_prev
            p1i = ar * xi_prev + ai * xr_prev
            if l == 0:
                y0r, y0i, y1r, y1i = p0r, p0i, p1r, p1i
            else:
                y0r, y0i, y1r, y1i = y0r + p0r, y0i + p0i, y1r + p1r, y1i + p1i
            xr_prev, xi_prev = xr, xim
        pr = jnp.where(first, 0.0, yprev[re, :])
        pi = jnp.where(first, 0.0, yprev[im, :])
        ybuf[0, re, :] = y0r - sgn * pi
        ybuf[0, im, :] = y0i + sgn * pr
        ybuf[1, re, :] = y1r - sgn * y0i
        ybuf[1, im, :] = y1i + sgn * y0r
        yprev[re, :] = y1r
        yprev[im, :] = y1i

    def inv(t, sl, p, jj):
        dv = jnp.broadcast_to(tapbuf[t, 4:5, :], (128, 128))
        y = jnp.dot(G_v[...], ybuf[jj].astype(bf16), preferred_element_type=f32)
        r = pl.multiple_of((2 * p + jj) * 128, 128)
        kv = kvbuf[sl, pl.ds(r, 128), :].astype(f32)
        qq = qbuf[sl, pl.ds(r, 128), :].astype(f32)
        bobuf[sl, pl.ds(r, 128), :] = (qq * (y + kv * dv)).astype(bf16)

    def wdma(c, slot, src):
        return pltpu.make_async_copy(src.at[:, pl.ds((c % 2) * 16, 16), :], wstage.at[slot], sems.at[slot])

    def start_w(c, slot):
        for m, src in enumerate((wq_hbm, wk_hbm, wv_hbm)):
            @pl.when(c // 2 == m)
            def _():
                wdma(c, slot, src).start()

    x0 = pltpu.make_async_copy(x_hbm.at[pl.ds(0, PRO)], x_v.at[pl.ds(0, PRO)], sems.at[2])
    x1 = pltpu.make_async_copy(x_hbm.at[pl.ds(PRO, S - PRO)], x_v.at[pl.ds(PRO, S - PRO)], sems.at[3])
    m0 = pltpu.make_async_copy(mem0_hbm, mem_v, sems.at[4])
    wod = pltpu.make_async_copy(wo_hbm, wostage, sems.at[5])
    for c in in_dmas(0):
        c.start()
    x0.start()
    start_w(0, 0)
    start_w(1, 1)
    for c in in_dmas(1):
        c.start()
    q_dma(0).start()

    kf[0:8, :] = jnp.zeros((8, 128), f32)
    for sl in range(2):
        xs[sl, NC] = jnp.zeros((256, 128), f32)
    yprev[...] = jnp.zeros((256, 128), f32)
    dd = d_v[...].astype(f32)
    sk = sk_v[...].astype(f32)
    for t in range(NT):
        tapbuf[t, 0:4, :] = sk[:, t * 128:(t + 1) * 128]
        tapbuf[t, 4:5, :] = dd[t:t + 1, :]
    obuf_x[pl.ds(0, FILL), :] = jnp.zeros((FILL, H * E), bf16)
    for c in in_dmas(0):
        c.wait()

    def sp0(p, _):
        sp_k(0, p)
        for jj in range(2):
            sp_x(0, 0, p, jj)
            sp_a(0, p, jj)
        return 0
    lax.fori_loop(0, 8, sp0, 0)

    def chunk_body(c, _):
        slot = c % 2
        wdma(c, slot, wq_hbm).wait()
        base = (c // 2) * 32 * WS + (c % 2) * 16 * WS

        def rl(i, _):
            for j in range(8):
                d = i * 16 + 2 * j
                a = pltpu.bitcast(wstage[slot, d], u32)
                b = pltpu.bitcast(wstage[slot, d + 1], u32)
                ev = (a & LO) | (b << 16)
                od = (a >> 16) | (b & HI)
                r = base + i * 8 + j
                wqkv[pl.ds(r, 8, stride=WS), :] = ev
                wqkv[pl.ds(r + 8 * WS, 8, stride=WS), :] = od
            return 0
        lax.fori_loop(0, D // 16, rl, 0)

        @pl.when(c + 2 < 6)
        def _():
            start_w(c + 2, slot)

        @pl.when(c == 0)
        def _():
            x0.wait()
            x1.start()
            m0.start()
            wod.start()

        def pro(jj, _):
            for i in range(4):
                sl = (c // 2) * 32 + (c % 2) * 16 + jj * 4 + i
                w = pltpu.bitcast(wqkv[pl.ds(sl * WS, 512), :], bf16)
                y = jnp.dot(x_v[pl.ds(0, PRO), :], w, preferred_element_type=f32)
                ring[sl, pl.ds(ROFF, PRO), :] = y.astype(bf16)
            return 0
        lax.fori_loop(0, 4, pro, 0)
        return 0
    lax.fori_loop(0, 6, chunk_body, 0)

    x1.wait()
    m0.wait()
    wod.wait()

    def wo_rl(i, _):
        for t in range(8):
            wo[t, pl.ds(i * 64, 64), :] = pltpu.bitcast(wostage[pl.ds(i * 128, 128), t * 128:(t + 1) * 128], u32)
        return 0
    lax.fori_loop(0, 32, wo_rl, 0)

    def fill_cur(s):
        rpos = pl.multiple_of((SEG * s + ROFF) % RING, 32)
        for sl in range(96):
            cur[sl] = pltpu.bitcast(ring[sl, pl.ds(rpos, SEG), :], u32)
    fill_cur(0)

    scale = E ** -0.5
    ri = lax.broadcasted_iota(jnp.int32, (SEG + M, SEG + M), 0)
    ci = lax.broadcasted_iota(jnp.int32, (SEG + M, SEG + M), 1)
    mask = (ri >= SEG) | (ci >= SEG) | (ci <= ri)

    def step(s, mem):
        bt = s // 8
        p = s % 8

        @pl.when(p == 0)
        def _():
            @pl.when(bt + 1 < NT)
            def _():
                for c in in_dmas(bt + 1):
                    c.wait()
                q_dma(bt + 1).start()

            @pl.when(bt + 2 < NT)
            def _():
                for c in in_dmas(bt + 2):
                    c.start()
            q_dma(bt).wait()

            @pl.when(bt >= 2)
            def _():
                o_dma(bt - 2).wait()

        bsl = bt % 2
        nt = jnp.minimum(bt + 1, NT - 1)
        nsl = (bt + 1) % 2
        btasks = {}
        if BMODE == 'spread':
            btasks[0] = [lambda: sp_k(nsl, p)]
            btasks[1] = [lambda: sp_x(nt, nsl, p, 0)]
            btasks[3] = [lambda: sp_a(nsl, p, 0)]
            btasks[5] = [lambda: sp_x(nt, nsl, p, 1)]
            btasks[7] = [lambda: sp_a(nsl, p, 1)]
            for b in range(16):
                btasks.setdefault(2 * b, []).append(lambda b=b: cv(bsl, p, b))
            btasks[34] = [lambda: inv(bt, bsl, p, 0)]
            btasks[36] = [lambda: inv(bt, bsl, p, 1)]

        xrow = pl.multiple_of(jnp.minimum(PRO + FILL * s, S - FILL), 8)
        xin = x_v[pl.ds(xrow, FILL), :]
        lhs = jnp.concatenate([mem.astype(bf16), xin], axis=0)
        wpos = pl.multiple_of((xrow + ROFF) % RING, 8)
        prow = pl.multiple_of(jnp.maximum(FILL * (s - 1), 0), 8)
        lo_scr[M:, :] = obuf_x[pl.ds(prow, FILL), :]
        parts, S_, P_, O_ = {}, {}, {}, {}

        def st_qkv(j):
            ps = []
            for m in range(3):
                sl = m * 32 + j
                w = pltpu.bitcast(wqkv[pl.ds(sl * WS, 512), :], bf16)
                y = jnp.dot(lhs, w, preferred_element_type=f32)
                ring[sl, pl.ds(wpos, FILL), :] = y[M:].astype(bf16)
                ps.append(y[:M].astype(bf16))
            parts[j] = ps

        def st_qk(j):
            q, k = [jnp.concatenate([pltpu.bitcast(cur[m * 32 + j], bf16), parts[j][m]], axis=0) for m in range(2)]
            S_[j] = lax.dot_general(q, k, (((1,), (1,)), ((), ())), preferred_element_type=f32)

        def st_sm(j):
            sc = jnp.where(mask, S_.pop(j) * scale, -1e9)
            e = jnp.exp(sc - jnp.max(sc, axis=-1, keepdims=True))
            P_[j] = (e / jnp.sum(e, axis=-1, keepdims=True)).astype(bf16)

        def st_pv(j):
            v = jnp.concatenate([pltpu.bitcast(cur[64 + j], bf16), parts[j][2]], axis=0)
            O_[j] = jnp.dot(P_.pop(j), v, preferred_element_type=f32)

        def st_ost(j):
            o = O_.pop(j)
            obuf_x[pl.ds(pl.multiple_of(SEG * s, 32), SEG), j * E:(j + 1) * E] = o[:SEG].astype(bf16)
            lo_scr[0:M, j * E:(j + 1) * E] = o[SEG:].astype(bf16)

        accs = {}

        def st_o(t, j0, j1):
            acc = accs.get(t)
            for j in range(j0, j1):
                hh = head_of_slot(j)
                w = pltpu.bitcast(wo[t, pl.ds(hh * 64, 64), :], bf16)
                y = jnp.dot(lo_scr[:, j * E:(j + 1) * E], w, preferred_element_type=f32)
                acc = y if acc is None else acc + y
            accs[t] = acc

        A, B_, C_, D_ = SKEW
        for t in range(H + D_ + 1):
            if t < H:
                st_qkv(t)
            elif t - H < 8:
                st_o(t - H, 0, 16)
            for f in btasks.get(t, []):
                f()
            if 0 <= t - A < H: st_qk(t - A)
            if 0 <= t - B_ < H: st_sm(t - B_)
            if 0 <= t - C_ < H: st_pv(t - C_)
            if 0 <= t - D_ < H: st_ost(t - D_)
        for t in range(D_ + 1, 8):
            st_o(t, 0, 16)
        fill_cur(jnp.minimum(s + 1, NSEG - 1))
        for t in range(8):
            st_o(t, 16, 32)
        y = jnp.concatenate([accs[t] for t in range(8)], axis=1)
        obuf[pl.ds(prow, FILL), :] = y[M:].astype(bf16)

        @pl.when(s > 0)
        def _():
            pltpu.make_async_copy(obuf.at[pl.ds(prow, FILL)], out_hbm.at[pl.ds(prow, FILL), pl.ds(0, D)], osem.at[0]).start()

        @pl.when(p == 7)
        def _():
            o_dma(bt).start()
        return y[:M]
    lax.fori_loop(0, NSEG, step, mem_v[...].astype(f32))

    r0 = FILL * (NSEG - 1)

    def epi(t, _):
        acc = None
        for j in range(H):
            hh = head_of_slot(j)
            w = pltpu.bitcast(wo[t, pl.ds(hh * 64, 64), :], bf16)
            y = jnp.dot(obuf_x[pl.ds(r0, PRO), j * E:(j + 1) * E], w, preferred_element_type=f32)
            acc = y if acc is None else acc + y
        obuf[pl.ds(r0, PRO), pl.ds(pl.multiple_of(t * 128, 128), 128)] = acc.astype(bf16)
        return 0
    lax.fori_loop(0, 8, epi, 0)
    ec = pltpu.make_async_copy(obuf.at[pl.ds(r0, PRO)], out_hbm.at[pl.ds(r0, PRO), pl.ds(0, D)], osem.at[1])
    ec.start()

    def owait(s, _):
        orow = pl.multiple_of(FILL * s, 8)
        pltpu.make_async_copy(obuf.at[pl.ds(orow, FILL)], out_hbm.at[pl.ds(orow, FILL), pl.ds(0, D)], osem.at[0]).wait()
        return 0
    lax.fori_loop(0, NSEG - 1, owait, 0)
    o_dma(NT - 2).wait()
    o_dma(NT - 1).wait()
    ec.wait()


@jax.jit
def run(A_x, A_mem0, A_Wq, A_Wk, A_Wv, A_Wo, B_q, B_k, B_v, B_shift_k, B_ssm_k, B_ssm_D):
    F, G = dft_consts()
    anyspec = pl.BlockSpec(memory_space=pl.ANY)
    vm = pl.BlockSpec(memory_space=pltpu.VMEM)
    out = pl.pallas_call(
        kernel,
        out_shape=jax.ShapeDtypeStruct((S, 2 * D), bf16),
        in_specs=[anyspec] * 10 + [vm] * 4, out_specs=anyspec,
        scratch_shapes=[
            pltpu.VMEM((S, D), bf16),
            pltpu.VMEM((M, D), bf16),
            pltpu.VMEM((96 * WS, E), u32),
            pltpu.VMEM((8, 2048, 128), u32),
            pltpu.VMEM((2, D, 16, E), bf16),
            pltpu.VMEM((H * E, D), bf16),
            pltpu.VMEM((96, RING, E), bf16),
            pltpu.VMEM((S, H * E), bf16),
            pltpu.VMEM((S, D), bf16),
            pltpu.VMEM((32, H * E), bf16),
            pltpu.VMEM((96, SEG // 2, E), u32),
            pltpu.SemaphoreType.DMA((6,)),
            pltpu.SemaphoreType.DMA((2,)),
            pltpu.VMEM((2, S, 128), bf16), pltpu.VMEM((2, S, 128), bf16), pltpu.VMEM((2, 128, S), bf16),
            pltpu.VMEM((2, S, 128), bf16), pltpu.VMEM((2, S, 128), bf16),
            pltpu.VMEM((S + 8, 128), f32), pltpu.VMEM((2, S, 128), bf16),
            pltpu.VMEM((2, NC + 1, 256, 128), f32), pltpu.VMEM((2, NC, 256, 128), f32),
            pltpu.VMEM((2, 256, 128), f32), pltpu.VMEM((256, 128), f32), pltpu.VMEM((NT, 8, 128), f32),
            pltpu.SemaphoreType.DMA((5, 2)),
        ],
        compiler_params=pltpu.CompilerParams(vmem_limit_bytes=120 * 1024 * 1024),
        name="fused",
    )(A_x.reshape(S, D), A_mem0.reshape(M, D), A_Wq, A_Wk, A_Wv, A_Wo.reshape(H * E, D),
      B_k.reshape(S, D), B_v.reshape(S, D), B_q.reshape(S, D), B_ssm_k, B_shift_k.T, B_ssm_D.reshape(8, 128), F, G)
    return out.reshape(1, S, 2 * D)


def pallas_concat_heads__memory_aug_recurrent_mem_tr__ssm_conv_h3__prompt_kernel(
    A_x, A_mem0, A_Wq, A_Wk, A_Wv, A_Wo, A_seg_len,
    B_q, B_k, B_v, B_shift_k, B_ssm_k, B_ssm_D,
):
    assert A_seg_len == SEG
    return run(A_x, A_mem0, A_Wq, A_Wk, A_Wv, A_Wo, B_q, B_k, B_v, B_shift_k, B_ssm_k, B_ssm_D)
```

```python
import jax
import jax.numpy as jnp
import numpy as np
import ml_dtypes
from jax import lax
from jax.experimental import pallas as pl
from jax.experimental.pallas import tpu as pltpu

S, D, H, E, M, SEG = 2048, 1024, 32, 128, 8, 32
NSEG = S // SEG
FILL = 24
PRO = S - FILL * (NSEG - 1)
RING = 672
ROFF = 64
WS = 516
C = 128
NC = S // C
NT = D // 128
SKEW = tuple(int(c) for c in '1,1,3,4'.split(','))
OCFG = [((0,14),[24,25,26,27,28,29,30,31]),((14,28),[32,32,33,33,34,34,35,35]),((28,32),[37]*8)]
FC = int('-1')
BLK = 2
import contextlib
SCOPES = '0' == '1'
scope = jax.named_scope if SCOPES else (lambda n: contextlib.nullcontext())
bf16, f32, u32 = jnp.bfloat16, jnp.float32, jnp.uint32


def head_of_slot(j):
    return (j // 16) * 16 + 2 * (j % 8) + ((j // 8) % 2)


def dft_consts():
    k = np.arange(C)[:, None].astype(np.float64)
    t = np.arange(C)[None, :].astype(np.float64)
    th = np.pi * (2 * k + 1) * t / (2 * C)
    F = np.concatenate([np.cos(th), -np.sin(th)], 0)
    G = np.concatenate([np.cos(th).T, -np.sin(th).T], 1) / C
    return F.astype(ml_dtypes.bfloat16), G.astype(ml_dtypes.bfloat16)


def kernel(x_hbm, mem0_hbm, wq_hbm, wk_hbm, wv_hbm, wo_hbm, k_hbm, v_hbm, q_hbm, h_hbm, sk_v, d_v, F_v, G_v,
           out_hbm,
           x_v, xp, mem_v, wqkv, wo, wstage, wostage, ring, obuf_x, obuf, lo_scr, cur, sems, osem,
           kbuf, vbuf, hbuf, qbuf, bobuf, kf, kvbuf, xs, as_, ybuf, tapbuf, bsem):
    LO = 0xFFFF
    HI = np.uint32(0xFFFF0000)
    sgn = (1 - 2 * (lax.broadcasted_iota(jnp.int32, (8, 128), 0) % 2)).astype(f32)

    def in_dmas(t):
        sl = t % 2
        c0 = pl.multiple_of(t * 128, 128)
        return [pltpu.make_async_copy(k_hbm.at[:, pl.ds(c0, 128)], kbuf.at[sl], bsem.at[0, sl]),
                pltpu.make_async_copy(v_hbm.at[:, pl.ds(c0, 128)], vbuf.at[sl], bsem.at[1, sl]),
                pltpu.make_async_copy(h_hbm.at[pl.ds(c0, 128), :], hbuf.at[sl], bsem.at[2, sl]),
                pltpu.make_async_copy(q_hbm.at[:, pl.ds(c0, 128)], qbuf.at[sl], bsem.at[3, sl])]

    def o_dma(t):
        sl = t % 2
        return pltpu.make_async_copy(bobuf.at[sl], out_hbm.at[:, pl.ds(pl.multiple_of(D + t * 128, 128), 128)], bsem.at[4, sl])

    def wdma(c, slot, src):
        return pltpu.make_async_copy(src.at[:, pl.ds((c % 2) * 16, 16), :], wstage.at[slot], sems.at[slot])

    def start_w(c, slot):
        for m, src in enumerate((wq_hbm, wk_hbm, wv_hbm)):
            @pl.when(c // 2 == m)
            def _():
                wdma(c, slot, src).start()

    def a_dma(c):
        rows = pl.ds(pl.multiple_of(c * 8 * FILL, 8), 8 * FILL)
        return pltpu.make_async_copy(obuf.at[rows], out_hbm.at[rows, pl.ds(0, D)], osem.at[0])

    x0 = pltpu.make_async_copy(x_hbm.at[pl.ds(0, PRO)], x_v.at[pl.ds(0, PRO)], sems.at[2])
    x1 = pltpu.make_async_copy(x_hbm.at[pl.ds(PRO, S - PRO)], x_v.at[pl.ds(PRO, S - PRO)], sems.at[3])
    m0 = pltpu.make_async_copy(mem0_hbm, mem_v, sems.at[4])
    wod = pltpu.make_async_copy(wo_hbm, wostage, sems.at[5])
    x0.start()
    start_w(0, 0)
    for c in in_dmas(0):
        c.start()
    start_w(1, 1)

    kf[0:8, :] = jnp.zeros((8, 128), f32)
    dd = d_v[...].astype(f32)
    sk = sk_v[...].astype(f32)
    for t in range(NT):
        tapbuf[t, 0:4, :] = sk[:, t * 128:(t + 1) * 128]
        tapbuf[t, 4:5, :] = dd[t:t + 1, :]
    obuf_x[pl.ds(0, FILL), :] = jnp.zeros((FILL, H * E), bf16)
    x0.wait()
    for kk in range(8):
        xp[kk, 0:PRO // 2, :] = pltpu.bitcast(x_v[0:PRO, kk * 128:(kk + 1) * 128], u32)

    def rl_rows(slot, base, i):
        for j in range(8):
            d = i * 16 + 2 * j
            a = pltpu.bitcast(wstage[slot, d], u32)
            b = pltpu.bitcast(wstage[slot, d + 1], u32)
            ev = (a & LO) | (b << 16)
            od = (a >> 16) | (b & HI)
            r = base + i * 8 + j
            wqkv[pl.ds(r, 8, stride=WS), :] = ev
            wqkv[pl.ds(r + 8 * WS, 8, stride=WS), :] = od

    def tile(t, _):
        sl = t % 2
        c = t - (t >= 4).astype(jnp.int32)
        with scope('binwait'):
            for cp in in_dmas(t):
                cp.wait()

        @pl.when(t + 1 < NT)
        def _():
            for cp in in_dmas(t + 1):
                cp.start()

        @pl.when(t >= 2)
        def _():
            o_dma(t - 2).wait()


        @pl.when((t != 3) & (t != 7))
        def _():
            slot = c % 2
            with scope('wwait'):
                wdma(c, slot, wq_hbm).wait()
            base = c * 16 * WS

            def rl(i, _):
                rl_rows(slot, base, i)
                return 0
            with scope('rl'):
                lax.fori_loop(0, D // 16, rl, 0)

            @pl.when(c + 2 < 6)
            def _():
                start_w(c + 2, slot)


        @pl.when(t == 3)
        def _():
            wod.start()

        @pl.when(t == 5)
        def _():
            x1.start()
            m0.start()

        @pl.when(t == 7)
        def _():
            wod.wait()

            def wo_rl(i, _):
                for n in range(8):
                    wo[n, pl.ds(i * 64, 64), :] = pltpu.bitcast(wostage[pl.ds(i * 128, 128), n * 128:(n + 1) * 128], u32)
                return 0
            lax.fori_loop(0, 32, wo_rl, 0)

        sc_ = scope('main'); sc_.__enter__()

        def adot(i):
            sl_ = t * 12 + i
            wv = pltpu.bitcast(wqkv[pl.ds(sl_ * WS, 512), :], bf16)
            for (m0, m1) in [(0, 536)]:
                xx = jnp.concatenate([pltpu.bitcast(xp[kk, m0 // 2:m1 // 2, :], bf16) for kk in range(8)], axis=1)
                y = jnp.dot(xx, wv, preferred_element_type=f32)
                ring[sl_, pl.ds(ROFF + m0, m1 - m0), :] = y.astype(bf16)

        w = [jnp.broadcast_to(tapbuf[t, j:j + 1, :], (8, 128)) for j in range(4)]
        kf[8:, :] = kbuf[sl].astype(f32)

        def spec(j):
            for u in range(8):
                rows = []
                for hf in range(2):
                    r = j * 128 + u * 16 + hf * 8
                    acc = kf[pl.ds(r + 5, 8), :] * w[3]
                    acc = acc + kf[pl.ds(r + 6, 8), :] * w[2]
                    acc = acc + kf[pl.ds(r + 7, 8), :] * w[1]
                    acc = acc + kf[pl.ds(r + 8, 8), :] * w[0]
                    rows.append(acc)
                ks = jnp.concatenate(rows, axis=0)
                rr = pl.ds(pl.multiple_of(j * 128 + u * 16, 16), 16)
                kvbuf[rr, :] = (ks * vbuf[sl, rr, :].astype(f32)).astype(bf16)
            rj = pl.ds(pl.multiple_of(j * 128, 128), 128)
            xx = jnp.dot(F_v[...], kvbuf[rj, :], preferred_element_type=f32)
            xs[j, 0:256, :] = xx
            xs[j, 256:384, :] = xx[:128] + xx[128:]
            a = lax.dot_general(F_v[...], hbuf[sl, :, rj], (((1,), (1,)), ((), ())), preferred_element_type=f32)
            as_[j, 0:256, :] = a
            as_[j, 256:384, :] = a[:128] + a[128:]

        def conv_gen(b):
            re = pl.ds(pl.multiple_of(b * 8, 8), 8)
            im = pl.ds(pl.multiple_of(128 + b * 8, 8), 8)
            sm = pl.ds(pl.multiple_of(256 + b * 8, 8), 8)
            prev = None
            for i0 in range(0, NC, BLK):
                acc = {}
                for j in range(0, i0 + BLK):
                    xr = xs[j, re, :]
                    xi = xs[j, im, :]
                    xsum = xs[j, sm, :]
                    for i in range(max(i0, j), i0 + BLK):
                        t_ = (as_[i - j, re, :] * xr, as_[i - j, im, :] * xi, as_[i - j, sm, :] * xsum)
                        acc[i] = t_ if i not in acc else tuple(u_ + v_ for u_, v_ in zip(acc[i], t_))
                    yield
                for i in range(i0, i0 + BLK):
                    p1, p2, p3 = acc[i]
                    yr, yi = p1 - p2, (p3 - p1) - p2
                    if prev is None:
                        ybuf[i, re, :] = yr
                        ybuf[i, im, :] = yi
                    else:
                        ybuf[i, re, :] = yr - sgn * prev[1]
                        ybuf[i, im, :] = yi + sgn * prev[0]
                    prev = (yr, yi)

        def conv(b):
            for _ in conv_gen(b):
                pass

        dv = jnp.broadcast_to(tapbuf[t, 4:5, :], (128, 128))

        def inv(i):
            y = jnp.dot(G_v[...], ybuf[i].astype(bf16), preferred_element_type=f32)
            rr = pl.ds(pl.multiple_of(i * 128, 128), 128)
            kv = kvbuf[rr, :].astype(f32)
            qq = qbuf[sl, rr, :].astype(f32)
            bobuf[sl, rr, :] = (qq * (y + kv * dv)).astype(bf16)

        for i in range(3):
            adot(i)
        for z in range(NC):
            spec(z)
        for z in range(16):
            if z % 2 == 0:
                adot(3 + z // 2)
            conv(z)
        for z in range(NC):
            inv(z)
        adot(11)
        sc_.__exit__(None, None, None)
        o_dma(t).start()
        return 0
    if '0' != '1':
        with scope('phase1'):
            lax.fori_loop(0, NT, tile, 0)
    else:
        x1.start(); m0.start()

    x1.wait()
    m0.wait()

    def fill_cur(s):
        rpos = pl.multiple_of((SEG * s + ROFF) % RING, 32)
        for sl in range(96):
            cur[sl] = pltpu.bitcast(ring[sl, pl.ds(rpos, SEG), :], u32)
    fill_cur(0)

    scale = E ** -0.5
    ri = lax.broadcasted_iota(jnp.int32, (SEG + M, SEG + M), 0)
    ci = lax.broadcasted_iota(jnp.int32, (SEG + M, SEG + M), 1)
    mask = (ri >= SEG) | (ci >= SEG) | (ci <= ri)

    def step(s, mem):
        xrow = pl.multiple_of(jnp.minimum(PRO + FILL * s, S - FILL), 8)
        xin = x_v[pl.ds(xrow, FILL), :]
        lhs = jnp.concatenate([mem.astype(bf16), xin], axis=0)
        wpos = pl.multiple_of((xrow + ROFF) % RING, 8)
        prow = pl.multiple_of(jnp.maximum(FILL * (s - 1), 0), 8)
        lo_scr[M:, :] = obuf_x[pl.ds(prow, FILL), :]
        parts, S_, P_, O_ = {}, {}, {}, {}

        def st_qkv(j):
            ps = []
            for m in range(3):
                sl = m * 32 + j
                w = pltpu.bitcast(wqkv[pl.ds(sl * WS, 512), :], bf16)
                y = jnp.dot(lhs, w, preferred_element_type=f32)
                ring[sl, pl.ds(wpos, FILL), :] = y[M:].astype(bf16)
                ps.append(y[:M].astype(bf16))
            parts[j] = ps

        npos = pl.multiple_of((SEG * jnp.minimum(s + 1, NSEG - 1) + ROFF) % RING, 32)

        def refill(sl):
            cur[sl] = pltpu.bitcast(ring[sl, pl.ds(npos, SEG), :], u32)

        def st_qk(j):
            q, k = [jnp.concatenate([pltpu.bitcast(cur[m * 32 + j], bf16), parts[j][m]], axis=0) for m in range(2)]
            S_[j] = lax.dot_general(q, k, (((1,), (1,)), ((), ())), preferred_element_type=f32)
            if FC < 0:
                refill(j)
                refill(32 + j)

        def st_sm(j):
            sc = jnp.where(mask, S_.pop(j) * scale, -1e9)
            e = jnp.exp(sc - jnp.max(sc, axis=-1, keepdims=True))
            P_[j] = (e / jnp.sum(e, axis=-1, keepdims=True)).astype(bf16)

        def st_pv(j):
            v = jnp.concatenate([pltpu.bitcast(cur[64 + j], bf16), parts[j][2]], axis=0)
            O_[j] = jnp.dot(P_.pop(j), v, preferred_element_type=f32)
            if FC < 0:
                refill(64 + j)

        def st_ost(j):
            o = O_.pop(j)
            obuf_x[pl.ds(pl.multiple_of(SEG * s, 32), SEG), j * E:(j + 1) * E] = o[:SEG].astype(bf16)
            lo_scr[0:M, j * E:(j + 1) * E] = o[SEG:].astype(bf16)

        accs = {}

        def st_o(t, j0, j1):
            acc = accs.get(t)
            for j in range(j0, j1):
                hh = head_of_slot(j)
                w = pltpu.bitcast(wo[t, pl.ds(hh * 64, 64), :], bf16)
                y = jnp.dot(lo_scr[:, j * E:(j + 1) * E], w, preferred_element_type=f32)
                acc = y if acc is None else acc + y
            accs[t] = acc

        A, B_, C_, D_ = SKEW
        assert FC < 0 or FC >= H + C_
        ou = {}
        for (j0, j1), slots in OCFG:
            for t_, sl_ in enumerate(slots):
                ou.setdefault(sl_, []).append((t_, j0, j1))
        last = max(max(ou), H - 1 + D_, FC)
        for t in range(last + 1):
            if t < H:
                st_qkv(t)
            if t == FC:
                fill_cur(jnp.minimum(s + 1, NSEG - 1))
            for u in ou.get(t, []):
                st_o(*u)
            if 0 <= t - A < H: st_qk(t - A)
            if 0 <= t - B_ < H: st_sm(t - B_)
            if 0 <= t - C_ < H: st_pv(t - C_)
            if 0 <= t - D_ < H: st_ost(t - D_)
        y = jnp.concatenate([accs[t] for t in range(8)], axis=1)
        obuf[pl.ds(prow, FILL), :] = y[M:].astype(bf16)
        return y[:M]

    def block(bt, mem):
        mem = lax.fori_loop(0, 8, lambda p, m: step(bt * 8 + p, m), mem)

        @pl.when(bt >= 1)
        def _():
            a_dma(bt - 1).start()
        return mem

    with scope('steps'):
        lax.fori_loop(0, NT, block, mem_v[...].astype(f32))

    r0 = FILL * (NSEG - 1)

    def epi(t, _):
        acc = None
        for j in range(H):
            hh = head_of_slot(j)
            w = pltpu.bitcast(wo[t, pl.ds(hh * 64, 64), :], bf16)
            y = jnp.dot(obuf_x[pl.ds(r0, PRO), j * E:(j + 1) * E], w, preferred_element_type=f32)
            acc = y if acc is None else acc + y
        obuf[pl.ds(r0, PRO), pl.ds(pl.multiple_of(t * 128, 128), 128)] = acc.astype(bf16)
        return 0
    with scope('epi'):
        lax.fori_loop(0, 8, epi, 0)
    e0 = (NT - 1) * 8 * FILL
    ec = pltpu.make_async_copy(obuf.at[pl.ds(e0, S - e0)], out_hbm.at[pl.ds(e0, S - e0), pl.ds(0, D)], osem.at[1])
    ec.start()
    for c in range(NT - 1):
        a_dma(c).wait()
    o_dma(NT - 2).wait()
    o_dma(NT - 1).wait()
    ec.wait()


@jax.jit
def run(A_x, A_mem0, A_Wq, A_Wk, A_Wv, A_Wo, B_q, B_k, B_v, B_shift_k, B_ssm_k, B_ssm_D):
    F, G = dft_consts()
    anyspec = pl.BlockSpec(memory_space=pl.ANY)
    vm = pl.BlockSpec(memory_space=pltpu.VMEM)
    out = pl.pallas_call(
        kernel,
        out_shape=jax.ShapeDtypeStruct((S, 2 * D), bf16),
        in_specs=[anyspec] * 10 + [vm] * 4, out_specs=anyspec,
        scratch_shapes=[
            pltpu.VMEM((S, D), bf16),
            pltpu.VMEM((8, 272, 128), u32),
            pltpu.VMEM((M, D), bf16),
            pltpu.VMEM((96 * WS, E), u32),
            pltpu.VMEM((8, 2048, 128), u32),
            pltpu.VMEM((2, D, 16, E), bf16),
            pltpu.VMEM((H * E, D), bf16),
            pltpu.VMEM((96, RING, E), bf16),
            pltpu.VMEM((S, H * E), bf16),
            pltpu.VMEM((S, D), bf16),
            pltpu.VMEM((32, H * E), bf16),
            pltpu.VMEM((96, SEG // 2, E), u32),
            pltpu.SemaphoreType.DMA((6,)),
            pltpu.SemaphoreType.DMA((2,)),
            pltpu.VMEM((2, S, 128), bf16), pltpu.VMEM((2, S, 128), bf16), pltpu.VMEM((2, 128, S), bf16),
            pltpu.VMEM((2, S, 128), bf16), pltpu.VMEM((2, S, 128), bf16),
            pltpu.VMEM((S + 8, 128), f32), pltpu.VMEM((S, 128), bf16),
            pltpu.VMEM((NC, 384, 128), f32), pltpu.VMEM((NC, 384, 128), f32),
            pltpu.VMEM((NC, 256, 128), f32), pltpu.VMEM((NT, 8, 128), f32),
            pltpu.SemaphoreType.DMA((5, 2)),
        ],
        compiler_params=pltpu.CompilerParams(vmem_limit_bytes=120 * 1024 * 1024),
        name="fused",
    )(A_x.reshape(S, D), A_mem0.reshape(M, D), A_Wq, A_Wk, A_Wv, A_Wo.reshape(H * E, D),
      B_k.reshape(S, D), B_v.reshape(S, D), B_q.reshape(S, D), B_ssm_k, B_shift_k.T, B_ssm_D.reshape(8, 128), F, G)
    return out.reshape(1, S, 2 * D)


def pallas_concat_heads__memory_aug_recurrent_mem_tr__ssm_conv_h3__prompt_kernel(
    A_x, A_mem0, A_Wq, A_Wk, A_Wv, A_Wo, A_seg_len,
    B_q, B_k, B_v, B_shift_k, B_ssm_k, B_ssm_D,
):
    assert A_seg_len == SEG
    return run(A_x, A_mem0, A_Wq, A_Wk, A_Wv, A_Wo, B_q, B_k, B_v, B_shift_k, B_ssm_k, B_ssm_D)
```

```python
import jax
import jax.numpy as jnp
import numpy as np
import ml_dtypes
from jax import lax
from jax.experimental import pallas as pl
from jax.experimental.pallas import tpu as pltpu

S, D, H, E, M, SEG = 2048, 1024, 32, 128, 8, 32
NSEG = S // SEG
FILL = 24
PRO = S - FILL * (NSEG - 1)
RING = 672
ROFF = 64
WS = 516
C = 128
NC = S // C
NT = D // 128
SKEW = tuple(int(c) for c in '1,1,3,4'.split(','))
OCFG = [((0,14),[24,25,26,27,28,29,30,31]),((14,28),[32,32,33,33,34,34,35,35]),((28,32),[37]*8)]
FC = int('-1')
BLK = int('4')
RLU = int('4')
import contextlib
SCOPES = '0' == '1'
scope = jax.named_scope if SCOPES else (lambda n: contextlib.nullcontext())
bf16, f32, u32 = jnp.bfloat16, jnp.float32, jnp.uint32


def head_of_slot(j):
    return (j // 16) * 16 + 2 * (j % 8) + ((j // 8) % 2)


def dft_consts():
    k = np.arange(C)[:, None].astype(np.float64)
    t = np.arange(C)[None, :].astype(np.float64)
    th = np.pi * (2 * k + 1) * t / (2 * C)
    F = np.concatenate([np.cos(th), -np.sin(th)], 0)
    G = np.concatenate([np.cos(th).T, -np.sin(th).T], 1) / C
    return F.astype(ml_dtypes.bfloat16), G.astype(ml_dtypes.bfloat16)


def kernel(x_hbm, mem0_hbm, wq_hbm, wk_hbm, wv_hbm, wo_hbm, k_hbm, v_hbm, q_hbm, h_hbm, sk_v, d_v, F_v, G_v,
           out_hbm,
           x_v, xp, mem_v, wqkv, wo, wstage, wostage, ring, obuf_x, obuf, lo_scr, cur, sems, osem,
           kbuf, vbuf, hbuf, qbuf, bobuf, kf, kvbuf, xs, as_, ybuf, tapbuf, bsem):
    LO = 0xFFFF
    HI = np.uint32(0xFFFF0000)
    sgn = (1 - 2 * (lax.broadcasted_iota(jnp.int32, (8, 128), 0) % 2)).astype(f32)

    def in_dmas(t):
        sl = t % 2
        c0 = pl.multiple_of(t * 128, 128)
        return [pltpu.make_async_copy(k_hbm.at[:, pl.ds(c0, 128)], kbuf.at[sl], bsem.at[0, sl]),
                pltpu.make_async_copy(v_hbm.at[:, pl.ds(c0, 128)], vbuf.at[sl], bsem.at[1, sl]),
                pltpu.make_async_copy(h_hbm.at[pl.ds(c0, 128), :], hbuf.at[sl], bsem.at[2, sl]),
                pltpu.make_async_copy(q_hbm.at[:, pl.ds(c0, 128)], qbuf.at[sl], bsem.at[3, sl])]

    def o_dma(t):
        sl = t % 2
        return pltpu.make_async_copy(bobuf.at[sl], out_hbm.at[:, pl.ds(pl.multiple_of(D + t * 128, 128), 128)], bsem.at[4, sl])

    def wdma(c, slot, src):
        return pltpu.make_async_copy(src.at[:, pl.ds((c % 2) * 16, 16), :], wstage.at[slot], sems.at[slot])

    def start_w(c, slot):
        for m, src in enumerate((wq_hbm, wk_hbm, wv_hbm)):
            @pl.when(c // 2 == m)
            def _():
                wdma(c, slot, src).start()

    def a_dma(c):
        rows = pl.ds(pl.multiple_of(c * 8 * FILL, 8), 8 * FILL)
        return pltpu.make_async_copy(obuf.at[rows], out_hbm.at[rows, pl.ds(0, D)], osem.at[0])

    x0 = pltpu.make_async_copy(x_hbm.at[pl.ds(0, PRO)], x_v.at[pl.ds(0, PRO)], sems.at[2])
    x1 = pltpu.make_async_copy(x_hbm.at[pl.ds(PRO, S - PRO)], x_v.at[pl.ds(PRO, S - PRO)], sems.at[3])
    m0 = pltpu.make_async_copy(mem0_hbm, mem_v, sems.at[4])
    wod = pltpu.make_async_copy(wo_hbm, wostage, sems.at[5])
    pre_ = scope('pre'); pre_.__enter__()
    x0.start()
    start_w(0, 0)
    for c in in_dmas(0):
        c.start()

    kf[0:8, :] = jnp.zeros((8, 128), f32)
    dd = d_v[...].astype(f32)
    sk = sk_v[...].astype(f32)
    for t in range(NT):
        tapbuf[t, 0:4, :] = sk[:, t * 128:(t + 1) * 128]
        tapbuf[t, 4:5, :] = dd[t:t + 1, :]
    obuf_x[pl.ds(0, FILL), :] = jnp.zeros((FILL, H * E), bf16)
    x0.wait()
    for kk in range(8):
        xp[kk, 0:PRO // 2, :] = pltpu.bitcast(x_v[0:PRO, kk * 128:(kk + 1) * 128], u32)

    def rl_rows(slot, base, i):
        for j in range(8):
            d = i * 16 + 2 * j
            a = pltpu.bitcast(wstage[slot, d], u32)
            b = pltpu.bitcast(wstage[slot, d + 1], u32)
            ev = (a & LO) | (b << 16)
            od = (a >> 16) | (b & HI)
            r = base + i * 8 + j
            wqkv[pl.ds(r, 8, stride=WS), :] = ev
            wqkv[pl.ds(r + 8 * WS, 8, stride=WS), :] = od

    pre_.__exit__(None, None, None)
    def tile(t, _):
        sl = t % 2
        c = t - (t >= 4).astype(jnp.int32)
        with scope('binwait'):
            for cp in in_dmas(t):
                cp.wait()

        @pl.when(t + 1 < NT)
        def _():
            for cp in in_dmas(t + 1):
                cp.start()

        @pl.when(t == 0)
        def _():
            wdma(1, 1, wq_hbm).start()

        @pl.when(t >= 2)
        def _():
            o_dma(t - 2).wait()


        @pl.when((t != 3) & (t != 7))
        def _():
            slot = c % 2
            with scope('wwait'):
                wdma(c, slot, wq_hbm).wait()
            base = c * 16 * WS

            def rl(i, _):
                for r_ in range(RLU):
                    rl_rows(slot, base, i * RLU + r_)
                return 0
            with scope('rl'):
                lax.fori_loop(0, D // 16 // RLU, rl, 0)

            @pl.when(c + 2 < 6)
            def _():
                start_w(c + 2, slot)


        @pl.when(t == 3)
        def _():
            wod.start()

        @pl.when(t == 5)
        def _():
            x1.start()
            m0.start()

        @pl.when(t == 7)
        def _():
            wod.wait()

            def wo_rl(i, _):
                for n in range(8):
                    wo[n, pl.ds(i * 64, 64), :] = pltpu.bitcast(wostage[pl.ds(i * 128, 128), n * 128:(n + 1) * 128], u32)
                return 0
            lax.fori_loop(0, 32, wo_rl, 0)

        sc_ = scope('main'); sc_.__enter__()

        def adot(i):
            sl_ = t * 12 + i
            wv = pltpu.bitcast(wqkv[pl.ds(sl_ * WS, 512), :], bf16)
            for (m0, m1) in [(0, 536)]:
                xx = jnp.concatenate([pltpu.bitcast(xp[kk, m0 // 2:m1 // 2, :], bf16) for kk in range(8)], axis=1)
                y = jnp.dot(xx, wv, preferred_element_type=f32)
                ring[sl_, pl.ds(ROFF + m0, m1 - m0), :] = y.astype(bf16)

        w = [jnp.broadcast_to(tapbuf[t, j:j + 1, :], (8, 128)) for j in range(4)]
        kf[8:, :] = kbuf[sl].astype(f32)

        def spec(j):
            for u in range(8):
                rows = []
                for hf in range(2):
                    r = j * 128 + u * 16 + hf * 8
                    acc = kf[pl.ds(r + 5, 8), :] * w[3]
                    acc = acc + kf[pl.ds(r + 6, 8), :] * w[2]
                    acc = acc + kf[pl.ds(r + 7, 8), :] * w[1]
                    acc = acc + kf[pl.ds(r + 8, 8), :] * w[0]
                    rows.append(acc)
                ks = jnp.concatenate(rows, axis=0)
                rr = pl.ds(pl.multiple_of(j * 128 + u * 16, 16), 16)
                kvbuf[rr, :] = (ks * vbuf[sl, rr, :].astype(f32)).astype(bf16)
            rj = pl.ds(pl.multiple_of(j * 128, 128), 128)
            xs[j] = jnp.dot(F_v[...], kvbuf[rj, :], preferred_element_type=f32)
            as_[j] = lax.dot_general(F_v[...], hbuf[sl, :, rj], (((1,), (1,)), ((), ())), preferred_element_type=f32)

        zz = jnp.minimum(t, 0)

        def conv_gen(b):
            re = pl.ds(pl.multiple_of(b * 8, 8), 8)
            im = pl.ds(pl.multiple_of(128 + b * 8, 8), 8)
            prev = None
            for i0 in range(0, NC, BLK):
                acc = {}
                for j in range(0, i0 + BLK):
                    xr = xs[zz + j, re, :]
                    xi = xs[zz + j, im, :]
                    xsum = xr + xi
                    for i in range(max(i0, j), i0 + BLK):
                        ar = as_[zz + (i - j), re, :]
                        ai = as_[zz + (i - j), im, :]
                        t_ = (ar * xr, ai * xi, (ar + ai) * xsum)
                        acc[i] = t_ if i not in acc else tuple(u_ + v_ for u_, v_ in zip(acc[i], t_))
                    yield
                for i in range(i0, i0 + BLK):
                    p1, p2, p3 = acc[i]
                    yr, yi = p1 - p2, (p3 - p1) - p2
                    if prev is None:
                        ybuf[i, re, :] = yr
                        ybuf[i, im, :] = yi
                    else:
                        ybuf[i, re, :] = yr - sgn * prev[1]
                        ybuf[i, im, :] = yi + sgn * prev[0]
                    prev = (yr, yi)

        def conv(b):
            for _ in conv_gen(b):
                pass

        dv = jnp.broadcast_to(tapbuf[t, 4:5, :], (128, 128))

        def inv(i):
            y = jnp.dot(G_v[...], ybuf[zz + i].astype(bf16), preferred_element_type=f32)
            rr = pl.ds(pl.multiple_of(i * 128, 128), 128)
            kv = kvbuf[pl.ds(pl.multiple_of(zz * 16 + i * 128, 16), 128), :].astype(f32)
            qq = qbuf[sl, rr, :].astype(f32)
            bobuf[sl, rr, :] = (qq * (y + kv * dv)).astype(bf16)

        for i in range(3):
            adot(i)
        for z in range(NC):
            spec(z)
        for z in range(16):
            if z % 2 == 0:
                adot(3 + z // 2)
            conv(z)
        for z in range(NC):
            inv(z)
        adot(11)
        sc_.__exit__(None, None, None)
        o_dma(t).start()
        return 0
    if '0' != '1':
        with scope('phase1'):
            lax.fori_loop(0, NT, tile, 0)
    else:
        x1.start(); m0.start()

    mid_ = scope('mid'); mid_.__enter__()
    x1.wait()
    m0.wait()

    def fill_cur(s):
        rpos = pl.multiple_of((SEG * s + ROFF) % RING, 32)
        for sl in range(96):
            cur[sl] = pltpu.bitcast(ring[sl, pl.ds(rpos, SEG), :], u32)
    fill_cur(0)

    mid_.__exit__(None, None, None)
    scale = E ** -0.5
    ri = lax.broadcasted_iota(jnp.int32, (SEG + M, SEG + M), 0)
    ci = lax.broadcasted_iota(jnp.int32, (SEG + M, SEG + M), 1)
    mask = (ri >= SEG) | (ci >= SEG) | (ci <= ri)

    def step(s, mem):
        xrow = pl.multiple_of(jnp.minimum(PRO + FILL * s, S - FILL), 8)
        xin = x_v[pl.ds(xrow, FILL), :]
        lhs = jnp.concatenate([mem.astype(bf16), xin], axis=0)
        wpos = pl.multiple_of((xrow + ROFF) % RING, 8)
        prow = pl.multiple_of(jnp.maximum(FILL * (s - 1), 0), 8)
        lo_scr[M:, :] = obuf_x[pl.ds(prow, FILL), :]
        parts, S_, P_, O_ = {}, {}, {}, {}

        def st_qkv(j):
            ps = []
            for m in range(3):
                sl = m * 32 + j
                w = pltpu.bitcast(wqkv[pl.ds(sl * WS, 512), :], bf16)
                y = jnp.dot(lhs, w, preferred_element_type=f32)
                ring[sl, pl.ds(wpos, FILL), :] = y[M:].astype(bf16)
                ps.append(y[:M].astype(bf16))
            parts[j] = ps

        npos = pl.multiple_of((SEG * jnp.minimum(s + 1, NSEG - 1) + ROFF) % RING, 32)

        def refill(sl):
            cur[sl] = pltpu.bitcast(ring[sl, pl.ds(npos, SEG), :], u32)

        def st_qk(j):
            q, k = [jnp.concatenate([pltpu.bitcast(cur[m * 32 + j], bf16), parts[j][m]], axis=0) for m in range(2)]
            S_[j] = lax.dot_general(q, k, (((1,), (1,)), ((), ())), preferred_element_type=f32)
            if FC < 0:
                refill(j)
                refill(32 + j)

        def st_sm(j):
            sc = jnp.where(mask, S_.pop(j) * scale, -1e9)
            e = jnp.exp(sc - jnp.max(sc, axis=-1, keepdims=True))
            P_[j] = (e / jnp.sum(e, axis=-1, keepdims=True)).astype(bf16)

        def st_pv(j):
            v = jnp.concatenate([pltpu.bitcast(cur[64 + j], bf16), parts[j][2]], axis=0)
            O_[j] = jnp.dot(P_.pop(j), v, preferred_element_type=f32)
            if FC < 0:
                refill(64 + j)

        def st_ost(j):
            o = O_.pop(j)
            obuf_x[pl.ds(pl.multiple_of(SEG * s, 32), SEG), j * E:(j + 1) * E] = o[:SEG].astype(bf16)
            lo_scr[0:M, j * E:(j + 1) * E] = o[SEG:].astype(bf16)

        accs = {}

        def st_o(t, j0, j1):
            acc = accs.get(t)
            for j in range(j0, j1):
                hh = head_of_slot(j)
                w = pltpu.bitcast(wo[t, pl.ds(hh * 64, 64), :], bf16)
                y = jnp.dot(lo_scr[:, j * E:(j + 1) * E], w, preferred_element_type=f32)
                acc = y if acc is None else acc + y
            accs[t] = acc

        A, B_, C_, D_ = SKEW
        assert FC < 0 or FC >= H + C_
        ou = {}
        for (j0, j1), slots in OCFG:
            for t_, sl_ in enumerate(slots):
                ou.setdefault(sl_, []).append((t_, j0, j1))
        last = max(max(ou), H - 1 + D_, FC)
        for t in range(last + 1):
            if t < H:
                st_qkv(t)
            if t == FC:
                fill_cur(jnp.minimum(s + 1, NSEG - 1))
            for u in ou.get(t, []):
                st_o(*u)
            if 0 <= t - A < H: st_qk(t - A)
            if 0 <= t - B_ < H: st_sm(t - B_)
            if 0 <= t - C_ < H: st_pv(t - C_)
            if 0 <= t - D_ < H: st_ost(t - D_)
        y = jnp.concatenate([accs[t] for t in range(8)], axis=1)
        obuf[pl.ds(prow, FILL), :] = y[M:].astype(bf16)
        return y[:M]

    def block(bt, mem):
        UN = int('2')

        def steps_(p, m):
            for u in range(UN):
                m = step(bt * 8 + p * UN + u, m)
            return m
        mem = lax.fori_loop(0, 8 // UN, steps_, mem)

        @pl.when(bt >= 1)
        def _():
            a_dma(bt - 1).start()
        return mem

    with scope('steps'):
        lax.fori_loop(0, NT, block, mem_v[...].astype(f32))

    r0 = FILL * (NSEG - 1)
    e0 = (NT - 1) * 8 * FILL
    tail = pltpu.make_async_copy(obuf.at[pl.ds(e0, r0 - e0)], out_hbm.at[pl.ds(e0, r0 - e0), pl.ds(0, D)], osem.at[1])
    tail.start()

    def e_dma(t):
        cols = pl.ds(pl.multiple_of(t * 128, 128), 128)
        return pltpu.make_async_copy(obuf.at[pl.ds(r0, PRO), cols], out_hbm.at[pl.ds(r0, PRO), cols], osem.at[2])

    def epi(t, _):
        acc = None
        for j in range(H):
            hh = head_of_slot(j)
            w = pltpu.bitcast(wo[t, pl.ds(hh * 64, 64), :], bf16)
            y = jnp.dot(obuf_x[pl.ds(r0, PRO), j * E:(j + 1) * E], w, preferred_element_type=f32)
            acc = y if acc is None else acc + y
        obuf[pl.ds(r0, PRO), pl.ds(pl.multiple_of(t * 128, 128), 128)] = acc.astype(bf16)
        e_dma(t).start()
        return 0
    with scope('epi'):
        lax.fori_loop(0, 8, epi, 0)
    post_ = scope('post'); post_.__enter__()
    for c in range(NT - 1):
        a_dma(c).wait()
    o_dma(NT - 2).wait()
    o_dma(NT - 1).wait()
    tail.wait()
    for t in range(8):
        e_dma(t).wait()
    post_.__exit__(None, None, None)


@jax.jit
def run(A_x, A_mem0, A_Wq, A_Wk, A_Wv, A_Wo, B_q, B_k, B_v, B_shift_k, B_ssm_k, B_ssm_D):
    F, G = dft_consts()
    anyspec = pl.BlockSpec(memory_space=pl.ANY)
    vm = pl.BlockSpec(memory_space=pltpu.VMEM)
    out = pl.pallas_call(
        kernel,
        out_shape=jax.ShapeDtypeStruct((S, 2 * D), bf16),
        in_specs=[anyspec] * 10 + [vm] * 4, out_specs=anyspec,
        scratch_shapes=[
            pltpu.VMEM((S, D), bf16),
            pltpu.VMEM((8, 272, 128), u32),
            pltpu.VMEM((M, D), bf16),
            pltpu.VMEM((96 * WS, E), u32),
            pltpu.VMEM((8, 2048, 128), u32),
            pltpu.VMEM((2, D, 16, E), bf16),
            pltpu.VMEM((H * E, D), bf16),
            pltpu.VMEM((96, RING, E), bf16),
            pltpu.VMEM((S, H * E), bf16),
            pltpu.VMEM((S, D), bf16),
            pltpu.VMEM((32, H * E), bf16),
            pltpu.VMEM((96, SEG // 2, E), u32),
            pltpu.SemaphoreType.DMA((6,)),
            pltpu.SemaphoreType.DMA((3,)),
            pltpu.VMEM((2, S, 128), bf16), pltpu.VMEM((2, S, 128), bf16), pltpu.VMEM((2, 128, S), bf16),
            pltpu.VMEM((2, S, 128), bf16), pltpu.VMEM((2, S, 128), bf16),
            pltpu.VMEM((S + 8, 128), f32), pltpu.VMEM((S, 128), bf16),
            pltpu.VMEM((NC, 256, 128), f32), pltpu.VMEM((NC, 256, 128), f32),
            pltpu.VMEM((NC, 256, 128), f32), pltpu.VMEM((NT, 8, 128), f32),
            pltpu.SemaphoreType.DMA((5, 2)),
        ],
        compiler_params=pltpu.CompilerParams(vmem_limit_bytes=120 * 1024 * 1024),
        name="fused",
    )(A_x.reshape(S, D), A_mem0.reshape(M, D), A_Wq, A_Wk, A_Wv, A_Wo.reshape(H * E, D),
      B_k.reshape(S, D), B_v.reshape(S, D), B_q.reshape(S, D), B_ssm_k, B_shift_k.T, B_ssm_D.reshape(8, 128), F, G)
    return out.reshape(1, S, 2 * D)


def pallas_concat_heads__memory_aug_recurrent_mem_tr__ssm_conv_h3__prompt_kernel(
    A_x, A_mem0, A_Wq, A_Wk, A_Wv, A_Wo, A_seg_len,
    B_q, B_k, B_v, B_shift_k, B_ssm_k, B_ssm_D,
):
    assert A_seg_len == SEG
    return run(A_x, A_mem0, A_Wq, A_Wk, A_Wv, A_Wo, B_q, B_k, B_v, B_shift_k, B_ssm_k, B_ssm_D)
```

```python
import jax
import jax.numpy as jnp
import numpy as np
import ml_dtypes
from jax import lax
from jax.experimental import pallas as pl
from jax.experimental.pallas import tpu as pltpu

S, D, H, E, M, SEG = 2048, 1024, 32, 128, 8, 32
NSEG = S // SEG
FILL = 24
PRO = S - FILL * (NSEG - 1)
RING = 672
ROFF = 64
WS = 516
C = 128
NC = S // C
NT = D // 128
SKEW = tuple(int(c) for c in '1,1,4,4'.split(','))
OCFG = [((0, 4), [11, 12, 13, 14, 15, 16, 17, 18]), ((4, 26), [32, 33, 34, 35, 36, 37, 38, 39]), ((26, 32), [40] * 8)]
BLK = int('4')
RLU = int('8')
import contextlib
SCOPES = '0' == '1'
scope = jax.named_scope if SCOPES else (lambda n: contextlib.nullcontext())
bf16, f32, u32 = jnp.bfloat16, jnp.float32, jnp.uint32


def head_of_slot(j):
    return (j // 16) * 16 + 2 * (j % 8) + ((j // 8) % 2)


def dft_consts():
    k = np.arange(C)[:, None].astype(np.float64)
    t = np.arange(C)[None, :].astype(np.float64)
    th = np.pi * (2 * k + 1) * t / (2 * C)
    F = np.concatenate([np.cos(th), -np.sin(th)], 0)
    G = np.concatenate([np.cos(th).T, -np.sin(th).T], 1) / C
    return F.astype(ml_dtypes.bfloat16), G.astype(ml_dtypes.bfloat16)


def kernel(x_hbm, mem0_hbm, wq_hbm, wk_hbm, wv_hbm, wo_hbm, k_hbm, v_hbm, q_hbm, h_hbm, sk_v, d_v, F_v, G_v,
           out_hbm,
           x_v, xp, mem_v, wqkv, wo, wstage, wostage, ring, obuf_x, obuf, lo_scr, cur, sems, osem,
           kbuf, vbuf, hbuf, qbuf, bobuf, kf, kvbuf, xs, as_, ybuf, tapbuf, bsem):
    LO = 0xFFFF
    HI = np.uint32(0xFFFF0000)
    sgn = (1 - 2 * (lax.broadcasted_iota(jnp.int32, (8, 128), 0) % 2)).astype(f32)

    def in_dmas(t):
        sl = t % 2
        c0 = pl.multiple_of(t * 128, 128)
        return [pltpu.make_async_copy(k_hbm.at[:, pl.ds(c0, 128)], kbuf.at[sl], bsem.at[0, sl]),
                pltpu.make_async_copy(v_hbm.at[:, pl.ds(c0, 128)], vbuf.at[sl], bsem.at[1, sl]),
                pltpu.make_async_copy(h_hbm.at[pl.ds(c0, 128), :], hbuf.at[sl], bsem.at[2, sl]),
                pltpu.make_async_copy(q_hbm.at[:, pl.ds(c0, 128)], qbuf.at[sl], bsem.at[3, sl])]

    def o_dma(t):
        sl = t % 2
        return pltpu.make_async_copy(bobuf.at[sl], out_hbm.at[:, pl.ds(pl.multiple_of(D + t * 128, 128), 128)], bsem.at[4, sl])

    def wdma(c, slot, src):
        return pltpu.make_async_copy(src.at[:, pl.ds((c % 2) * 16, 16), :], wstage.at[slot], sems.at[slot])

    def start_w(c, slot):
        for m, src in enumerate((wq_hbm, wk_hbm, wv_hbm)):
            @pl.when(c // 2 == m)
            def _():
                wdma(c, slot, src).start()

    def a_dma(c):
        rows = pl.ds(pl.multiple_of(c * 8 * FILL, 8), 8 * FILL)
        return pltpu.make_async_copy(obuf.at[rows], out_hbm.at[rows, pl.ds(0, D)], osem.at[0])

    x0 = pltpu.make_async_copy(x_hbm.at[pl.ds(0, PRO)], x_v.at[pl.ds(0, PRO)], sems.at[2])
    x1 = pltpu.make_async_copy(x_hbm.at[pl.ds(PRO, S - PRO)], x_v.at[pl.ds(PRO, S - PRO)], sems.at[3])
    m0 = pltpu.make_async_copy(mem0_hbm, mem_v, sems.at[4])
    wod = pltpu.make_async_copy(wo_hbm, wostage, sems.at[5])
    pre_ = scope('pre'); pre_.__enter__()
    x0.start()
    start_w(0, 0)
    for c in in_dmas(0):
        c.start()

    kf[0:8, :] = jnp.zeros((8, 128), f32)
    dd = d_v[...].astype(f32)
    sk = sk_v[...].astype(f32)
    for t in range(NT):
        tapbuf[t, 0:4, :] = sk[:, t * 128:(t + 1) * 128]
        tapbuf[t, 4:5, :] = dd[t:t + 1, :]
    obuf_x[pl.ds(0, FILL), :] = jnp.zeros((FILL, H * E), bf16)
    x0.wait()
    for kk in range(8):
        xp[kk, 0:PRO // 2, :] = pltpu.bitcast(x_v[0:PRO, kk * 128:(kk + 1) * 128], u32)

    def rl_rows(slot, base, i):
        for j in range(8):
            d = i * 16 + 2 * j
            a = pltpu.bitcast(wstage[slot, d], u32)
            b = pltpu.bitcast(wstage[slot, d + 1], u32)
            ev = (a & LO) | (b << 16)
            od = (a >> 16) | (b & HI)
            r = base + i * 8 + j
            wqkv[pl.ds(r, 8, stride=WS), :] = ev
            wqkv[pl.ds(r + 8 * WS, 8, stride=WS), :] = od

    pre_.__exit__(None, None, None)
    def tile(t, _):
        sl = t % 2
        c = t - (t >= 4).astype(jnp.int32)
        with scope('binwait'):
            for cp in in_dmas(t):
                cp.wait()

        @pl.when(t + 1 < NT)
        def _():
            for cp in in_dmas(t + 1):
                cp.start()

        @pl.when(t == 0)
        def _():
            wdma(1, 1, wq_hbm).start()

        @pl.when(t >= 2)
        def _():
            o_dma(t - 2).wait()


        @pl.when((t != 3) & (t != 7))
        def _():
            slot = c % 2
            with scope('wwait'):
                wdma(c, slot, wq_hbm).wait()
            base = c * 16 * WS

            def rl(i, _):
                for r_ in range(RLU):
                    rl_rows(slot, base, i * RLU + r_)
                return 0
            with scope('rl'):
                lax.fori_loop(0, D // 16 // RLU, rl, 0)

            @pl.when(c + 2 < 6)
            def _():
                start_w(c + 2, slot)


        @pl.when(t == 3)
        def _():
            wod.start()

        @pl.when(t == 5)
        def _():
            x1.start()
            m0.start()

        @pl.when(t == 7)
        def _():
            wod.wait()

            def wo_rl(i, _):
                for n in range(8):
                    wo[n, pl.ds(i * 64, 64), :] = pltpu.bitcast(wostage[pl.ds(i * 128, 128), n * 128:(n + 1) * 128], u32)
                return 0
            lax.fori_loop(0, 32, wo_rl, 0)

        sc_ = scope('main'); sc_.__enter__()

        def adot(i):
            sl_ = t * 12 + i
            wv = pltpu.bitcast(wqkv[pl.ds(sl_ * WS, 512), :], bf16)
            for (m0, m1) in [(0, 536)]:
                xx = jnp.concatenate([pltpu.bitcast(xp[kk, m0 // 2:m1 // 2, :], bf16) for kk in range(8)], axis=1)
                y = jnp.dot(xx, wv, preferred_element_type=f32)
                ring[sl_, pl.ds(ROFF + m0, m1 - m0), :] = y.astype(bf16)

        w = [jnp.broadcast_to(tapbuf[t, j:j + 1, :], (8, 128)) for j in range(4)]
        kf[8:, :] = kbuf[sl].astype(f32)

        zz = jnp.minimum(t, 0)

        def spec(j):
            for u in range(8):
                rows = []
                for hf in range(2):
                    r = j * 128 + u * 16 + hf * 8
                    acc = kf[pl.ds(r + 5, 8), :] * w[3]
                    acc = acc + kf[pl.ds(r + 6, 8), :] * w[2]
                    acc = acc + kf[pl.ds(r + 7, 8), :] * w[1]
                    acc = acc + kf[pl.ds(r + 8, 8), :] * w[0]
                    rows.append(acc)
                ks = jnp.concatenate(rows, axis=0)
                rr = pl.ds(pl.multiple_of(j * 128 + u * 16, 16), 16)
                kvbuf[pl.ds(pl.multiple_of(zz * 16 + j * 128 + u * 16, 16), 16), :] = (ks * vbuf[sl, rr, :].astype(f32)).astype(bf16)
            rj = pl.ds(pl.multiple_of(j * 128, 128), 128)
            xs[j] = jnp.dot(F_v[...], kvbuf[rj, :], preferred_element_type=f32)
            as_[j] = lax.dot_general(F_v[...], hbuf[sl, :, rj], (((1,), (1,)), ((), ())), preferred_element_type=f32)

        def conv_gen(b):
            re = pl.ds(pl.multiple_of(b * 8, 8), 8)
            im = pl.ds(pl.multiple_of(128 + b * 8, 8), 8)
            prev = None
            for i0 in range(0, NC, BLK):
                acc = {}
                acache = {}
                for j in range(0, i0 + BLK):
                    xr = xs[zz + j, re, :]
                    xi = xs[zz + j, im, :]
                    xsum = xr + xi
                    for i in range(max(i0, j), i0 + BLK):
                        if i - j not in acache:
                            ar = as_[zz + (i - j), re, :]
                            ai = as_[zz + (i - j), im, :]
                            acache[i - j] = (ar, ai, ar + ai)
                        ar, ai, asum = acache[i - j]
                        t_ = (ar * xr, ai * xi, asum * xsum)
                        acc[i] = t_ if i not in acc else tuple(u_ + v_ for u_, v_ in zip(acc[i], t_))
                    yield
                for i in range(i0, i0 + BLK):
                    p1, p2, p3 = acc[i]
                    yr, yi = p1 - p2, (p3 - p1) - p2
                    if prev is None:
                        ybuf[zz + i, re, :] = yr
                        ybuf[zz + i, im, :] = yi
                    else:
                        ybuf[zz + i, re, :] = yr - sgn * prev[1]
                        ybuf[zz + i, im, :] = yi + sgn * prev[0]
                    prev = (yr, yi)

        def conv(b):
            for _ in conv_gen(b):
                pass

        dv = jnp.broadcast_to(tapbuf[t, 4:5, :], (128, 128))

        def inv(i):
            y = jnp.dot(G_v[...], ybuf[i].astype(bf16), preferred_element_type=f32)
            rr = pl.ds(pl.multiple_of(i * 128, 128), 128)
            kv = kvbuf[rr, :].astype(f32)
            qq = qbuf[sl, rr, :].astype(f32)
            bobuf[sl, rr, :] = (qq * (y + kv * dv)).astype(bf16)

        for i in range(3):
            adot(i)
        for z in range(NC):
            spec(z)
        for z in range(16):
            if z % 2 == 0:
                adot(3 + z // 2)
            conv(z)
        for z in range(NC):
            inv(z)
        adot(11)
        sc_.__exit__(None, None, None)
        o_dma(t).start()
        return 0
    if '0' != '1':
        with scope('phase1'):
            lax.fori_loop(0, NT, tile, 0)
    else:
        x1.start(); m0.start()

    mid_ = scope('mid'); mid_.__enter__()
    x1.wait()
    m0.wait()

    def fill_cur(s):
        rpos = pl.multiple_of((SEG * s + ROFF) % RING, 32)
        for sl in range(96):
            cur[sl] = pltpu.bitcast(ring[sl, pl.ds(rpos, SEG), :], u32)
    fill_cur(0)

    mid_.__exit__(None, None, None)
    scale = E ** -0.5
    L2 = 2 * (SEG + M)
    ri = lax.broadcasted_iota(jnp.int32, (L2, L2), 0)
    ci = lax.broadcasted_iota(jnp.int32, (L2, L2), 1)

    def head_and_pos(i):
        is_mem = i >= 2 * SEG
        hd = jnp.where(is_mem, (i - 2 * SEG) // M, i // SEG)
        return is_mem, hd, i % SEG
    r_mem, r_hd, r_pos = head_and_pos(ri)
    c_mem, c_hd, c_pos = head_and_pos(ci)
    same_head = r_hd == c_hd
    visible = r_mem | c_mem | (c_pos <= r_pos)
    keep = same_head & visible
    fill = jnp.where(same_head, -1e9, -jnp.inf).astype(f32)

    def step(s, mem):
        xrow = pl.multiple_of(jnp.minimum(PRO + FILL * s, S - FILL), 8)
        xin = x_v[pl.ds(xrow, FILL), :]
        lhs = jnp.concatenate([mem.astype(bf16), xin], axis=0)
        wpos = pl.multiple_of((xrow + ROFF) % RING, 8)
        prow = pl.multiple_of(jnp.maximum(FILL * (s - 1), 0), 8)
        lo_scr[M:, :] = obuf_x[pl.ds(prow, FILL), :]
        parts, S_, P_, O_ = {}, {}, {}, {}

        def st_qkv(j):
            ps = []
            for m in range(3):
                sl = m * 32 + j
                w = pltpu.bitcast(wqkv[pl.ds(sl * WS, 512), :], bf16)
                y = jnp.dot(lhs, w, preferred_element_type=f32)
                ring[sl, pl.ds(wpos, FILL), :] = y[M:].astype(bf16)
                ps.append(y[:M])
            parts[j] = ps

        npos = pl.multiple_of((SEG * jnp.minimum(s + 1, NSEG - 1) + ROFF) % RING, 32)

        def refill(sl):
            cur[sl] = pltpu.bitcast(ring[sl, pl.ds(npos, SEG), :], u32)

        def pair(m, p_):
            ja, jb = 2 * p_, 2 * p_ + 1
            mm = jnp.concatenate([parts[ja][m], parts[jb][m]], axis=0).astype(bf16)
            return jnp.concatenate([pltpu.bitcast(cur[m * 32 + ja], bf16), pltpu.bitcast(cur[m * 32 + jb], bf16), mm], axis=0)

        def st_qk(p_):
            q, k = pair(0, p_), pair(1, p_)
            S_[p_] = lax.dot_general(q, k, (((1,), (1,)), ((), ())), preferred_element_type=f32)
            for j in (2 * p_, 2 * p_ + 1):
                refill(j)
                refill(32 + j)

        def st_sm(p_):
            sc = jnp.where(keep, S_.pop(p_) * scale, fill)
            e = jnp.exp(sc - jnp.max(sc, axis=-1, keepdims=True))
            P_[p_] = (e / jnp.sum(e, axis=-1, keepdims=True)).astype(bf16)

        def st_pv(p_):
            O_[p_] = jnp.dot(P_.pop(p_), pair(2, p_), preferred_element_type=f32)
            for j in (2 * p_, 2 * p_ + 1):
                refill(64 + j)

        def st_ost(p_):
            o = O_.pop(p_)
            for z, j in enumerate((2 * p_, 2 * p_ + 1)):
                obuf_x[pl.ds(pl.multiple_of(SEG * s, 32), SEG), j * E:(j + 1) * E] = o[z * SEG:(z + 1) * SEG].astype(bf16)
                lo_scr[0:M, j * E:(j + 1) * E] = o[2 * SEG + z * M:2 * SEG + (z + 1) * M].astype(bf16)

        accs = {}

        def st_o(t, j0, j1):
            acc = accs.get(t)
            for j in range(j0, j1):
                hh = head_of_slot(j)
                w = pltpu.bitcast(wo[t, pl.ds(hh * 64, 64), :], bf16)
                y = jnp.dot(lo_scr[:, j * E:(j + 1) * E], w, preferred_element_type=f32)
                acc = y if acc is None else acc + y
            accs[t] = acc

        A, B_, C_, D_ = SKEW
        ou = {}
        for (j0, j1), slots in OCFG:
            for t_, sl_ in enumerate(slots):
                ou.setdefault(sl_, []).append((t_, j0, j1))
        last = max(max(ou), H - 1 + D_)

        def due(t, lag):
            u = t - lag - 1
            return u // 2 if (u >= 0 and u % 2 == 0 and u // 2 < H // 2) else None
        for t in range(last + 1):
            if t < H:
                st_qkv(t)
            for u in ou.get(t, []):
                st_o(*u)
            for lag, fn in ((A, st_qk), (B_, st_sm), (C_, st_pv), (D_, st_ost)):
                p_ = due(t, lag)
                if p_ is not None:
                    fn(p_)
        y = jnp.concatenate([accs[t] for t in range(8)], axis=1)
        obuf[pl.ds(prow, FILL), :] = y[M:].astype(bf16)
        return y[:M]

    def block(bt, mem):
        UN = int('2')

        def steps_(p, m):
            for u in range(UN):
                m = step(bt * 8 + p * UN + u, m)
            return m
        mem = lax.fori_loop(0, 8 // UN, steps_, mem)

        @pl.when(bt >= 1)
        def _():
            a_dma(bt - 1).start()
        return mem

    with scope('steps'):
        lax.fori_loop(0, NT, block, mem_v[...].astype(f32))

    r0 = FILL * (NSEG - 1)
    e0 = (NT - 1) * 8 * FILL
    tail = pltpu.make_async_copy(obuf.at[pl.ds(e0, r0 - e0)], out_hbm.at[pl.ds(e0, r0 - e0), pl.ds(0, D)], osem.at[1])
    tail.start()

    def e_dma(t):
        cols = pl.ds(pl.multiple_of(t * 128, 128), 128)
        return pltpu.make_async_copy(obuf.at[pl.ds(r0, PRO), cols], out_hbm.at[pl.ds(r0, PRO), cols], osem.at[2])

    def epi(t, _):
        acc = None
        for j in range(H):
            hh = head_of_slot(j)
            w = pltpu.bitcast(wo[t, pl.ds(hh * 64, 64), :], bf16)
            y = jnp.dot(obuf_x[pl.ds(r0, PRO), j * E:(j + 1) * E], w, preferred_element_type=f32)
            acc = y if acc is None else acc + y
        obuf[pl.ds(r0, PRO), pl.ds(pl.multiple_of(t * 128, 128), 128)] = acc.astype(bf16)
        e_dma(t).start()
        return 0
    with scope('epi'):
        lax.fori_loop(0, 8, epi, 0)
    post_ = scope('post'); post_.__enter__()
    for c in range(NT - 1):
        a_dma(c).wait()
    o_dma(NT - 2).wait()
    o_dma(NT - 1).wait()
    tail.wait()
    for t in range(8):
        e_dma(t).wait()
    post_.__exit__(None, None, None)


@jax.jit
def run(A_x, A_mem0, A_Wq, A_Wk, A_Wv, A_Wo, B_q, B_k, B_v, B_shift_k, B_ssm_k, B_ssm_D):
    F, G = dft_consts()
    anyspec = pl.BlockSpec(memory_space=pl.ANY)
    vm = pl.BlockSpec(memory_space=pltpu.VMEM)
    out = pl.pallas_call(
        kernel,
        out_shape=jax.ShapeDtypeStruct((S, 2 * D), bf16),
        in_specs=[anyspec] * 10 + [vm] * 4, out_specs=anyspec,
        scratch_shapes=[
            pltpu.VMEM((S, D), bf16),
            pltpu.VMEM((8, 272, 128), u32),
            pltpu.VMEM((M, D), bf16),
            pltpu.VMEM((96 * WS, E), u32),
            pltpu.VMEM((8, 2048, 128), u32),
            pltpu.VMEM((2, D, 16, E), bf16),
            pltpu.VMEM((H * E, D), bf16),
            pltpu.VMEM((96, RING, E), bf16),
            pltpu.VMEM((S, H * E), bf16),
            pltpu.VMEM((S, D), bf16),
            pltpu.VMEM((32, H * E), bf16),
            pltpu.VMEM((96, SEG // 2, E), u32),
            pltpu.SemaphoreType.DMA((6,)),
            pltpu.SemaphoreType.DMA((3,)),
            pltpu.VMEM((2, S, 128), bf16), pltpu.VMEM((2, S, 128), bf16), pltpu.VMEM((2, 128, S), bf16),
            pltpu.VMEM((2, S, 128), bf16), pltpu.VMEM((2, S, 128), bf16),
            pltpu.VMEM((S + 8, 128), f32), pltpu.VMEM((S, 128), bf16),
            pltpu.VMEM((NC, 256, 128), f32), pltpu.VMEM((NC, 256, 128), f32),
            pltpu.VMEM((NC, 256, 128), f32), pltpu.VMEM((NT, 8, 128), f32),
            pltpu.SemaphoreType.DMA((5, 2)),
        ],
        compiler_params=pltpu.CompilerParams(vmem_limit_bytes=120 * 1024 * 1024),
        name="fused",
    )(A_x.reshape(S, D), A_mem0.reshape(M, D), A_Wq, A_Wk, A_Wv, A_Wo.reshape(H * E, D),
      B_k.reshape(S, D), B_v.reshape(S, D), B_q.reshape(S, D), B_ssm_k, B_shift_k.T, B_ssm_D.reshape(8, 128), F, G)
    return out.reshape(1, S, 2 * D)


def pallas_concat_heads__memory_aug_recurrent_mem_tr__ssm_conv_h3__prompt_kernel(
    A_x, A_mem0, A_Wq, A_Wk, A_Wv, A_Wo, A_seg_len,
    B_q, B_k, B_v, B_shift_k, B_ssm_k, B_ssm_D,
):
    assert A_seg_len == SEG
    return run(A_x, A_mem0, A_Wq, A_Wk, A_Wv, A_Wo, B_q, B_k, B_v, B_shift_k, B_ssm_k, B_ssm_D)
```

```python
import jax
import jax.numpy as jnp
import numpy as np
import ml_dtypes
from jax import lax
from jax.experimental import pallas as pl
from jax.experimental.pallas import tpu as pltpu

S, D, H, E, M, SEG = 2048, 1024, 32, 128, 8, 32
NSEG = S // SEG
FILL = 24
PRO = S - FILL * NSEG
EPI = S - FILL * (NSEG - 1) - M
RING = 576
ROFF = 64
WS = 516
C = 128
NC = S // C
NT = D // 128
SKEW = tuple(int(c) for c in '1,1,4,4'.split(','))
OCFG = [((0, 4), [11, 12, 13, 14, 15, 16, 17, 18]), ((4, 26), [32, 33, 34, 35, 36, 37, 38, 39]), ((26, 32), [40] * 8)]
BLK = int('4')
RLU = int('8')
import contextlib
SCOPES = '0' == '1'
scope = jax.named_scope if SCOPES else (lambda n: contextlib.nullcontext())
bf16, f32, u32 = jnp.bfloat16, jnp.float32, jnp.uint32


def head_of_slot(j):
    return (j // 16) * 16 + 2 * (j % 8) + ((j // 8) % 2)


def dft_consts():
    k = np.arange(C)[:, None].astype(np.float64)
    t = np.arange(C)[None, :].astype(np.float64)
    th = np.pi * (2 * k + 1) * t / (2 * C)
    F = np.concatenate([np.cos(th), -np.sin(th)], 0)
    G = np.concatenate([np.cos(th).T, -np.sin(th).T], 1) / C
    return F.astype(ml_dtypes.bfloat16), G.astype(ml_dtypes.bfloat16)


def kernel(x_hbm, mem0_hbm, wq_hbm, wk_hbm, wv_hbm, wo_hbm, k_hbm, v_hbm, q_hbm, h_hbm, sk_v, d_v, F_v, G_v,
           out_hbm,
           x_v, xp, mem_v, wqkv, wo, wstage, wostage, ring, obuf_x, obuf, lo_scr, cur, sems, osem,
           kbuf, vbuf, hbuf, qbuf, bobuf, kf, kvbuf, xs, as_, ybuf, tapbuf, bsem):
    LO = 0xFFFF
    HI = np.uint32(0xFFFF0000)
    sgn = (1 - 2 * (lax.broadcasted_iota(jnp.int32, (8, 128), 0) % 2)).astype(f32)

    def in_dmas(t):
        sl = t % 2
        c0 = pl.multiple_of(t * 128, 128)
        return [pltpu.make_async_copy(k_hbm.at[:, pl.ds(c0, 128)], kbuf.at[sl], bsem.at[0, sl]),
                pltpu.make_async_copy(v_hbm.at[:, pl.ds(c0, 128)], vbuf.at[sl], bsem.at[1, sl]),
                pltpu.make_async_copy(h_hbm.at[pl.ds(c0, 128), :], hbuf.at[sl], bsem.at[2, sl]),
                pltpu.make_async_copy(q_hbm.at[:, pl.ds(c0, 128)], qbuf.at[sl], bsem.at[3, sl])]

    def o_dma(t):
        sl = t % 2
        return pltpu.make_async_copy(bobuf.at[sl], out_hbm.at[:, pl.ds(pl.multiple_of(D + t * 128, 128), 128)], bsem.at[4, sl])

    def wdma(c, slot, src):
        return pltpu.make_async_copy(src.at[:, pl.ds((c % 2) * 16, 16), :], wstage.at[slot], sems.at[slot])

    def start_w(c, slot):
        for m, src in enumerate((wq_hbm, wk_hbm, wv_hbm)):
            @pl.when(c // 2 == m)
            def _():
                wdma(c, slot, src).start()

    def a_dma(c):
        rows = pl.ds(pl.multiple_of(c * 8 * FILL, 8), 8 * FILL)
        return pltpu.make_async_copy(obuf.at[rows], out_hbm.at[rows, pl.ds(0, D)], osem.at[0])

    x0 = pltpu.make_async_copy(x_hbm.at[pl.ds(0, PRO)], x_v.at[pl.ds(0, PRO)], sems.at[2])
    x1 = pltpu.make_async_copy(x_hbm.at[pl.ds(PRO, S - PRO)], x_v.at[pl.ds(PRO, S - PRO)], sems.at[3])
    m0 = pltpu.make_async_copy(mem0_hbm, mem_v, sems.at[4])
    wod = pltpu.make_async_copy(wo_hbm, wostage, sems.at[5])
    pre_ = scope('pre'); pre_.__enter__()
    x0.start()
    start_w(0, 0)
    for c in in_dmas(0):
        c.start()

    kf[0:8, :] = jnp.zeros((8, 128), f32)
    dd = d_v[...].astype(f32)
    sk = sk_v[...].astype(f32)
    for t in range(NT):
        tapbuf[t, 0:4, :] = sk[:, t * 128:(t + 1) * 128]
        tapbuf[t, 4:5, :] = dd[t:t + 1, :]
    obuf_x[pl.ds(0, FILL), :] = jnp.zeros((FILL, H * E), bf16)
    x0.wait()
    for kk in range(8):
        xp[kk, 0:PRO // 2, :] = pltpu.bitcast(x_v[0:PRO, kk * 128:(kk + 1) * 128], u32)

    def rl_rows(slot, base, i):
        for j in range(8):
            d = i * 16 + 2 * j
            a = pltpu.bitcast(wstage[slot, d], u32)
            b = pltpu.bitcast(wstage[slot, d + 1], u32)
            ev = (a & LO) | (b << 16)
            od = (a >> 16) | (b & HI)
            r = base + i * 8 + j
            wqkv[pl.ds(r, 8, stride=WS), :] = ev
            wqkv[pl.ds(r + 8 * WS, 8, stride=WS), :] = od

    pre_.__exit__(None, None, None)
    def tile(t, _):
        sl = t % 2
        c = t - (t >= 4).astype(jnp.int32)
        with scope('binwait'):
            for cp in in_dmas(t):
                cp.wait()

        @pl.when(t + 1 < NT)
        def _():
            for cp in in_dmas(t + 1):
                cp.start()

        @pl.when(t == 0)
        def _():
            wdma(1, 1, wq_hbm).start()

        @pl.when(t >= 2)
        def _():
            o_dma(t - 2).wait()


        @pl.when((t != 3) & (t != 7))
        def _():
            slot = c % 2
            with scope('wwait'):
                wdma(c, slot, wq_hbm).wait()
            base = c * 16 * WS

            def rl(i, _):
                for r_ in range(RLU):
                    rl_rows(slot, base, i * RLU + r_)
                return 0
            with scope('rl'):
                lax.fori_loop(0, D // 16 // RLU, rl, 0)

            @pl.when(c + 2 < 6)
            def _():
                start_w(c + 2, slot)


        @pl.when(t == 3)
        def _():
            wod.start()

        @pl.when(t == 5)
        def _():
            x1.start()
            m0.start()

        @pl.when(t == 7)
        def _():
            wod.wait()

            def wo_rl(i, _):
                for n in range(8):
                    wo[n, pl.ds(i * 64, 64), :] = pltpu.bitcast(wostage[pl.ds(i * 128, 128), n * 128:(n + 1) * 128], u32)
                return 0
            lax.fori_loop(0, 32, wo_rl, 0)

        sc_ = scope('main'); sc_.__enter__()

        def adot(i):
            sl_ = t * 12 + i
            wv = pltpu.bitcast(wqkv[pl.ds(sl_ * WS, 512), :], bf16)
            for (m0, m1) in [(0, PRO)]:
                xx = jnp.concatenate([pltpu.bitcast(xp[kk, m0 // 2:m1 // 2, :], bf16) for kk in range(8)], axis=1)
                y = jnp.dot(xx, wv, preferred_element_type=f32)
                ring[sl_, pl.ds(ROFF + m0, m1 - m0), :] = y.astype(bf16)

        w = [jnp.broadcast_to(tapbuf[t, j:j + 1, :], (8, 128)) for j in range(4)]
        kf[8:, :] = kbuf[sl].astype(f32)

        zz = jnp.minimum(t, 0)

        def spec(j):
            for u in range(8):
                rows = []
                for hf in range(2):
                    r = j * 128 + u * 16 + hf * 8
                    acc = kf[pl.ds(r + 5, 8), :] * w[3]
                    acc = acc + kf[pl.ds(r + 6, 8), :] * w[2]
                    acc = acc + kf[pl.ds(r + 7, 8), :] * w[1]
                    acc = acc + kf[pl.ds(r + 8, 8), :] * w[0]
                    rows.append(acc)
                ks = jnp.concatenate(rows, axis=0)
                rr = pl.ds(pl.multiple_of(j * 128 + u * 16, 16), 16)
                kvbuf[pl.ds(pl.multiple_of(zz * 16 + j * 128 + u * 16, 16), 16), :] = (ks * vbuf[sl, rr, :].astype(f32)).astype(bf16)
            rj = pl.ds(pl.multiple_of(j * 128, 128), 128)
            xs[j] = jnp.dot(F_v[...], kvbuf[rj, :], preferred_element_type=f32)
            as_[j] = lax.dot_general(F_v[...], hbuf[sl, :, rj], (((1,), (1,)), ((), ())), preferred_element_type=f32)

        def conv_gen(b):
            re = pl.ds(pl.multiple_of(b * 8, 8), 8)
            im = pl.ds(pl.multiple_of(128 + b * 8, 8), 8)
            prev = None
            for i0 in range(0, NC, BLK):
                acc = {}
                acache = {}
                for j in range(0, i0 + BLK):
                    xr = xs[zz + j, re, :]
                    xi = xs[zz + j, im, :]
                    xsum = xr + xi
                    for i in range(max(i0, j), i0 + BLK):
                        if i - j not in acache:
                            ar = as_[zz + (i - j), re, :]
                            ai = as_[zz + (i - j), im, :]
                            acache[i - j] = (ar, ai, ar + ai)
                        ar, ai, asum = acache[i - j]
                        t_ = (ar * xr, ai * xi, asum * xsum)
                        acc[i] = t_ if i not in acc else tuple(u_ + v_ for u_, v_ in zip(acc[i], t_))
                    yield
                for i in range(i0, i0 + BLK):
                    p1, p2, p3 = acc[i]
                    yr, yi = p1 - p2, (p3 - p1) - p2
                    if prev is None:
                        ybuf[zz + i, re, :] = yr
                        ybuf[zz + i, im, :] = yi
                    else:
                        ybuf[zz + i, re, :] = yr - sgn * prev[1]
                        ybuf[zz + i, im, :] = yi + sgn * prev[0]
                    prev = (yr, yi)

        def conv(b):
            for _ in conv_gen(b):
                pass

        dv = jnp.broadcast_to(tapbuf[t, 4:5, :], (128, 128))

        def inv(i):
            y = jnp.dot(G_v[...], ybuf[i].astype(bf16), preferred_element_type=f32)
            rr = pl.ds(pl.multiple_of(i * 128, 128), 128)
            kv = kvbuf[rr, :].astype(f32)
            qq = qbuf[sl, rr, :].astype(f32)
            bobuf[sl, rr, :] = (qq * (y + kv * dv)).astype(bf16)

        for i in range(3):
            adot(i)
        for z in range(NC):
            spec(z)
        for z in range(16):
            if z % 2 == 0:
                adot(3 + z // 2)
            conv(z)
        for z in range(NC):
            inv(z)
        adot(11)
        sc_.__exit__(None, None, None)
        o_dma(t).start()
        return 0
    if '0' != '1':
        with scope('phase1'):
            lax.fori_loop(0, NT, tile, 0)
    else:
        x1.start(); m0.start()

    mid_ = scope('mid'); mid_.__enter__()
    x1.wait()
    m0.wait()

    def fill_cur(s):
        rpos = pl.multiple_of((SEG * s + ROFF) % RING, 32)
        for sl in range(96):
            cur[sl] = pltpu.bitcast(ring[sl, pl.ds(rpos, SEG), :], u32)
    fill_cur(0)

    mid_.__exit__(None, None, None)
    scale = E ** -0.5
    L2 = 2 * (SEG + M)
    ri = lax.broadcasted_iota(jnp.int32, (L2, L2), 0)
    ci = lax.broadcasted_iota(jnp.int32, (L2, L2), 1)

    def head_and_pos(i):
        is_mem = i >= 2 * SEG
        hd = jnp.where(is_mem, (i - 2 * SEG) // M, i // SEG)
        return is_mem, hd, i % SEG
    r_mem, r_hd, r_pos = head_and_pos(ri)
    c_mem, c_hd, c_pos = head_and_pos(ci)
    same_head = r_hd == c_hd
    visible = r_mem | c_mem | (c_pos <= r_pos)
    keep = same_head & visible
    fill = jnp.where(same_head, -1e9, -jnp.inf).astype(f32)

    def step(s, mem, tail=False):
        fresh = FILL - M * (NSEG - 1 - s)
        final = s == NSEG - 1
        xrow = pl.multiple_of(PRO + FILL * s, 8)
        xin = x_v[pl.ds(xrow, FILL), :]
        lhs = jnp.concatenate([mem.astype(bf16), xin], axis=0)
        wpos = pl.multiple_of((FILL * s) % RING, 8)
        prow = pl.multiple_of(jnp.maximum(FILL * (s - 1), 0), 8)
        lo_scr[M:, :] = obuf_x[pl.ds(prow, FILL), :]
        parts, S_, P_, O_ = {}, {}, {}, {}

        newx = {}

        def st_qkv(j):
            ps = []
            for m in range(3):
                sl = m * 32 + j
                w = pltpu.bitcast(wqkv[pl.ds(sl * WS, 512), :], bf16)
                y = jnp.dot(lhs, w, preferred_element_type=f32)
                ring[sl, pl.ds(wpos, FILL), :] = y[M:].astype(bf16)
                if tail:
                    newx[sl] = y[M:]
                ps.append(y[:M])
            parts[j] = ps

        npos = pl.multiple_of((SEG * (s + 1) + ROFF) % RING, 32)

        def refill(sl):
            cur[sl] = pltpu.bitcast(ring[sl, pl.ds(npos, SEG), :], u32)

        def tokens(sl):
            c_ = pltpu.bitcast(cur[sl], bf16)
            if tail:
                o_ = c_.astype(f32)
                n_ = newx.pop(sl)
                f0, f1, f2 = n_[0:8], n_[8:16], n_[16:24]
                c_ = jnp.concatenate([
                    o_[0:8],
                    jnp.where(fresh == 24, f0, o_[8:16]),
                    jnp.where(fresh == 24, f1, jnp.where(fresh == 16, f0, o_[16:24])),
                    jnp.where(fresh == 24, f2, jnp.where(fresh == 16, f1, f0)),
                ], axis=0).astype(bf16)
            return c_

        def pair(m, p_):
            ja, jb = 2 * p_, 2 * p_ + 1
            mm = jnp.concatenate([parts[ja][m], parts[jb][m]], axis=0).astype(bf16)
            return jnp.concatenate([tokens(m * 32 + ja), tokens(m * 32 + jb), mm], axis=0)

        def st_qk(p_):
            q, k = pair(0, p_), pair(1, p_)
            S_[p_] = lax.dot_general(q, k, (((1,), (1,)), ((), ())), preferred_element_type=f32)
            for j in (2 * p_, 2 * p_ + 1):
                refill(j)
                refill(32 + j)

        def st_sm(p_):
            sc = jnp.where(keep, S_.pop(p_) * scale, fill)
            e = jnp.exp(sc - jnp.max(sc, axis=-1, keepdims=True))
            P_[p_] = (e / jnp.sum(e, axis=-1, keepdims=True)).astype(bf16)

        def st_pv(p_):
            O_[p_] = jnp.dot(P_.pop(p_), pair(2, p_), preferred_element_type=f32)
            for j in (2 * p_, 2 * p_ + 1):
                refill(64 + j)

        def st_ost(p_):
            o = O_.pop(p_)
            for z, j in enumerate((2 * p_, 2 * p_ + 1)):
                obuf_x[pl.ds(pl.multiple_of(SEG * s, 32), SEG), j * E:(j + 1) * E] = o[z * SEG:(z + 1) * SEG].astype(bf16)
                om = o[2 * SEG + z * M:2 * SEG + (z + 1) * M].astype(bf16)
                if tail:
                    om = jnp.where(final, obuf_x[pl.ds(S - EPI - M, M), j * E:(j + 1) * E], om)
                lo_scr[0:M, j * E:(j + 1) * E] = om

        accs = {}

        def st_o(t, j0, j1):
            acc = accs.get(t)
            for j in range(j0, j1):
                hh = head_of_slot(j)
                w = pltpu.bitcast(wo[t, pl.ds(hh * 64, 64), :], bf16)
                y = jnp.dot(lo_scr[:, j * E:(j + 1) * E], w, preferred_element_type=f32)
                acc = y if acc is None else acc + y
            accs[t] = acc

        A, B_, C_, D_ = SKEW
        ou = {}
        for (j0, j1), slots in OCFG:
            for t_, sl_ in enumerate(slots):
                ou.setdefault(sl_, []).append((t_, j0, j1))
        last = max(max(ou), H - 1 + D_)

        def due(t, lag):
            u = t - lag - 1
            return u // 2 if (u >= 0 and u % 2 == 0 and u // 2 < H // 2) else None
        for t in range(last + 1):
            if t < H:
                st_qkv(t)
            for u in ou.get(t, []):
                st_o(*u)
            for lag, fn in ((A, st_qk), (B_, st_sm), (C_, st_pv), (D_, st_ost)):
                p_ = due(t, lag)
                if p_ is not None:
                    fn(p_)
        y = jnp.concatenate([accs[t] for t in range(8)], axis=1)
        obuf[pl.ds(prow, FILL), :] = y[M:].astype(bf16)
        if tail:
            obuf[pl.ds(S - EPI - M, M), :] = y[:M].astype(bf16)
        return y[:M]

    NLOOP = NSEG - 3

    def main_step(u, mem):
        mem = step(u, mem)

        @pl.when((u % 8 == 0) & (u >= 8))
        def _():
            a_dma(u // 8 - 1).start()
        return mem

    with scope('steps'):
        mem = lax.fori_loop(0, NLOOP, main_step, mem_v[...].astype(f32))
        lax.fori_loop(NLOOP, NSEG, lambda s_, m_: step(s_, m_, tail=True), mem)

    r0 = S - EPI
    e0 = (NT - 1) * 8 * FILL
    tail = pltpu.make_async_copy(obuf.at[pl.ds(e0, r0 - e0)], out_hbm.at[pl.ds(e0, r0 - e0), pl.ds(0, D)], osem.at[1])
    tail.start()

    def e_dma(t):
        cols = pl.ds(pl.multiple_of(t * 128, 128), 128)
        return pltpu.make_async_copy(obuf.at[pl.ds(r0, EPI), cols], out_hbm.at[pl.ds(r0, EPI), cols], osem.at[2])

    def epi(t, _):
        acc = None
        for j in range(H):
            hh = head_of_slot(j)
            w = pltpu.bitcast(wo[t, pl.ds(hh * 64, 64), :], bf16)
            y = jnp.dot(obuf_x[pl.ds(r0, EPI), j * E:(j + 1) * E], w, preferred_element_type=f32)
            acc = y if acc is None else acc + y
        obuf[pl.ds(r0, EPI), pl.ds(pl.multiple_of(t * 128, 128), 128)] = acc.astype(bf16)
        e_dma(t).start()
        return 0
    with scope('epi'):
        lax.fori_loop(0, 8, epi, 0)
    post_ = scope('post'); post_.__enter__()
    for c in range(NT - 1):
        a_dma(c).wait()
    o_dma(NT - 2).wait()
    o_dma(NT - 1).wait()
    tail.wait()
    for t in range(8):
        e_dma(t).wait()
    post_.__exit__(None, None, None)


@jax.jit
def run(A_x, A_mem0, A_Wq, A_Wk, A_Wv, A_Wo, B_q, B_k, B_v, B_shift_k, B_ssm_k, B_ssm_D):
    F, G = dft_consts()
    anyspec = pl.BlockSpec(memory_space=pl.ANY)
    vm = pl.BlockSpec(memory_space=pltpu.VMEM)
    out = pl.pallas_call(
        kernel,
        out_shape=jax.ShapeDtypeStruct((S, 2 * D), bf16),
        in_specs=[anyspec] * 10 + [vm] * 4, out_specs=anyspec,
        scratch_shapes=[
            pltpu.VMEM((S, D), bf16),
            pltpu.VMEM((8, PRO // 2, 128), u32),
            pltpu.VMEM((M, D), bf16),
            pltpu.VMEM((96 * WS, E), u32),
            pltpu.VMEM((8, 2048, 128), u32),
            pltpu.VMEM((2, D, 16, E), bf16),
            pltpu.VMEM((H * E, D), bf16),
            pltpu.VMEM((96, RING, E), bf16),
            pltpu.VMEM((S, H * E), bf16),
            pltpu.VMEM((S, D), bf16),
            pltpu.VMEM((32, H * E), bf16),
            pltpu.VMEM((96, SEG // 2, E), u32),
            pltpu.SemaphoreType.DMA((6,)),
            pltpu.SemaphoreType.DMA((3,)),
            pltpu.VMEM((2, S, 128), bf16), pltpu.VMEM((2, S, 128), bf16), pltpu.VMEM((2, 128, S), bf16),
            pltpu.VMEM((2, S, 128), bf16), pltpu.VMEM((2, S, 128), bf16),
            pltpu.VMEM((S + 8, 128), f32), pltpu.VMEM((S, 128), bf16),
            pltpu.VMEM((NC, 256, 128), f32), pltpu.VMEM((NC, 256, 128), f32),
            pltpu.VMEM((NC, 256, 128), f32), pltpu.VMEM((NT, 8, 128), f32),
            pltpu.SemaphoreType.DMA((5, 2)),
        ],
        compiler_params=pltpu.CompilerParams(vmem_limit_bytes=120 * 1024 * 1024),
        name="fused",
    )(A_x.reshape(S, D), A_mem0.reshape(M, D), A_Wq, A_Wk, A_Wv, A_Wo.reshape(H * E, D),
      B_k.reshape(S, D), B_v.reshape(S, D), B_q.reshape(S, D), B_ssm_k, B_shift_k.T, B_ssm_D.reshape(8, 128), F, G)
    return out.reshape(1, S, 2 * D)


def pallas_concat_heads__memory_aug_recurrent_mem_tr__ssm_conv_h3__prompt_kernel(
    A_x, A_mem0, A_Wq, A_Wk, A_Wv, A_Wo, A_seg_len,
    B_q, B_k, B_v, B_shift_k, B_ssm_k, B_ssm_D,
):
    assert A_seg_len == SEG
    return run(A_x, A_mem0, A_Wq, A_Wk, A_Wv, A_Wo, B_q, B_k, B_v, B_shift_k, B_ssm_k, B_ssm_D)
```

```python
import jax
import jax.numpy as jnp
import numpy as np
import ml_dtypes
from jax import lax
from jax.experimental import pallas as pl
from jax.experimental.pallas import tpu as pltpu

S, D, H, E, M, SEG = 2048, 1024, 32, 128, 8, 32
NSEG = S // SEG
FILL = 24
PRO = S - FILL * NSEG
EPI = S - FILL * (NSEG - 1) - M
RING = 576
ROFF = 64
WS = 516
C = 128
NC = S // C
NT = D // 128
SKEW = tuple(int(c) for c in '1,1,4,4'.split(','))
OCFG = [((0, 4), [11, 12, 13, 14, 15, 16, 17, 18]), ((4, 26), [32, 33, 34, 35, 36, 37, 38, 39]), ((26, 32), [40] * 8)]
BLK = int('4')
RLU = int('8')
import contextlib
SCOPES = '0' == '1'
scope = jax.named_scope if SCOPES else (lambda n: contextlib.nullcontext())
bf16, f32, u32 = jnp.bfloat16, jnp.float32, jnp.uint32


def head_of_slot(j):
    return (j // 16) * 16 + 2 * (j % 8) + ((j // 8) % 2)


def dft_consts():
    k = np.arange(C)[:, None].astype(np.float64)
    t = np.arange(C)[None, :].astype(np.float64)
    th = np.pi * (2 * k + 1) * t / (2 * C)
    F = np.concatenate([np.cos(th), -np.sin(th)], 0)
    G = np.concatenate([np.cos(th).T, -np.sin(th).T], 1) / C
    return F.astype(ml_dtypes.bfloat16), G.astype(ml_dtypes.bfloat16)


def kernel(x_hbm, mem0_hbm, wq_hbm, wk_hbm, wv_hbm, wo_hbm, k_hbm, v_hbm, q_hbm, h_hbm, sk_v, d_v, F_v, G_v,
           out_hbm,
           x_v, xp, mem_v, wqkv, wo, wstage, wostage, ring, obuf_x, obuf, lo_scr, cur, sems, osem, qsem,
           kbuf, vbuf, hbuf, qbuf, bobuf, kf, kvbuf, xs, as_, ybuf, tapbuf, bsem):
    LO = 0xFFFF
    HI = np.uint32(0xFFFF0000)
    sgn = (1 - 2 * (lax.broadcasted_iota(jnp.int32, (8, 128), 0) % 2)).astype(f32)

    def in_dmas(t):
        sl = t % 2
        c0 = pl.multiple_of(t * 128, 128)
        return [pltpu.make_async_copy(k_hbm.at[:, pl.ds(c0, 128)], kbuf.at[sl], bsem.at[0, sl]),
                pltpu.make_async_copy(v_hbm.at[:, pl.ds(c0, 128)], vbuf.at[sl], bsem.at[1, sl]),
                pltpu.make_async_copy(h_hbm.at[pl.ds(c0, 128), :], hbuf.at[sl], bsem.at[2, sl]),
                pltpu.make_async_copy(q_hbm.at[:, pl.ds(c0, 128)], qbuf.at[sl], bsem.at[3, sl])]

    def o_dma(t):
        sl = t % 2
        return pltpu.make_async_copy(bobuf.at[sl], out_hbm.at[:, pl.ds(pl.multiple_of(D + t * 128, 128), 128)], bsem.at[4, sl])

    def wdma(c, slot, src):
        return pltpu.make_async_copy(src.at[:, pl.ds((c % 2) * 16, 16), :], wstage.at[slot], sems.at[slot])

    def start_w(c, slot):
        for m, src in enumerate((wq_hbm, wk_hbm, wv_hbm)):
            @pl.when(c // 2 == m)
            def _():
                wdma(c, slot, src).start()

    def a_dma(c):
        rows = pl.ds(pl.multiple_of(c * 8 * FILL, 8), 8 * FILL)
        return pltpu.make_async_copy(obuf.at[rows], out_hbm.at[rows, pl.ds(0, D)], osem.at[0])

    x0 = pltpu.make_async_copy(x_hbm.at[pl.ds(0, PRO)], x_v.at[pl.ds(0, PRO)], sems.at[2])
    x1 = pltpu.make_async_copy(x_hbm.at[pl.ds(PRO, S - PRO)], x_v.at[pl.ds(PRO, S - PRO)], sems.at[3])
    m0 = pltpu.make_async_copy(mem0_hbm, mem_v, sems.at[4])
    wod = pltpu.make_async_copy(wo_hbm, wostage, sems.at[5])
    pre_ = scope('pre'); pre_.__enter__()
    NQ = 4
    RQ = D // NQ

    def w0_dma(i):
        rows = pl.ds(i * RQ, RQ)
        return pltpu.make_async_copy(wq_hbm.at[rows, pl.ds(0, 16), :], wstage.at[0, rows], qsem.at[i])
    for i in range(NQ):
        w0_dma(i).start()
    x0.start()

    kf[0:8, :] = jnp.zeros((8, 128), f32)
    dd = d_v[...].astype(f32)
    sk = sk_v[...].astype(f32)
    for t in range(NT):
        tapbuf[t, 0:4, :] = sk[:, t * 128:(t + 1) * 128]
        tapbuf[t, 4:5, :] = dd[t:t + 1, :]
    obuf_x[pl.ds(0, FILL), :] = jnp.zeros((FILL, H * E), bf16)
    def rl_rows(slot, base, i):
        for j in range(8):
            d = i * 16 + 2 * j
            a = pltpu.bitcast(wstage[slot, d], u32)
            b = pltpu.bitcast(wstage[slot, d + 1], u32)
            ev = (a & LO) | (b << 16)
            od = (a >> 16) | (b & HI)
            r = base + i * 8 + j
            wqkv[pl.ds(r, 8, stride=WS), :] = ev
            wqkv[pl.ds(r + 8 * WS, 8, stride=WS), :] = od

    def adot(sl_):
        wv = pltpu.bitcast(wqkv[pl.ds(sl_ * WS, 512), :], bf16)
        xx = jnp.concatenate([pltpu.bitcast(xp[kk], bf16) for kk in range(8)], axis=1)
        y = jnp.dot(xx, wv, preferred_element_type=f32)
        ring[sl_, pl.ds(ROFF, PRO), :] = y.astype(bf16)

    def relayout(c, slot, after_wait=None):
        wdma(c, slot, wq_hbm).wait()
        if after_wait is not None:
            after_wait()
        base = c * 16 * WS

        def rl(i, _):
            for r_ in range(RLU):
                rl_rows(slot, base, i * RLU + r_)
            return 0
        lax.fori_loop(0, D // 16 // RLU, rl, 0)

    def more_dmas():
        for c in in_dmas(0):
            c.start()
        start_w(1, 1)
        for c in in_dmas(1):
            c.start()
    for i in range(NQ):
        w0_dma(i).wait()
        if i == NQ - 1:
            more_dmas()

        def rlq(u, _, i=i):
            for r_ in range(RLU):
                rl_rows(0, 0, i * (RQ // 16) + u * RLU + r_)
            return 0
        lax.fori_loop(0, RQ // 16 // RLU, rlq, 0)
    start_w(2, 0)
    x0.wait()
    for kk in range(8):
        xp[kk, 0:PRO // 2, :] = pltpu.bitcast(x_v[0:PRO, kk * 128:(kk + 1) * 128], u32)


    def first_slots(u, _):
        for i in range(4):
            adot(u * 4 + i)
        return 0
    lax.fori_loop(0, 4, first_slots, 0)
    pre_.__exit__(None, None, None)
    def tile(t, _):
        sl = t % 2
        c = t + 1 - (t >= 3).astype(jnp.int32) - (t >= 6).astype(jnp.int32)
        with scope('binwait'):
            for cp in in_dmas(t):
                cp.wait()


        @pl.when(t >= 2)
        def _():
            o_dma(t - 2).wait()


        @pl.when((t != 2) & (t != 5) & (t != 7))
        def _():
            with scope('rl'):
                relayout(c, c % 2)

            @pl.when(c + 2 < 6)
            def _():
                start_w(c + 2, c % 2)

        @pl.when(t == 2)
        def _():
            wod.start()

        @pl.when(t == 5)
        def _():
            x1.start()
            m0.start()

        @pl.when(t == 7)
        def _():
            wod.wait()

            def wo_rl(i, _):
                for n in range(8):
                    wo[n, pl.ds(i * 64, 64), :] = pltpu.bitcast(wostage[pl.ds(i * 128, 128), n * 128:(n + 1) * 128], u32)
                return 0
            lax.fori_loop(0, 32, wo_rl, 0)

        sc_ = scope('main'); sc_.__enter__()

        w = [jnp.broadcast_to(tapbuf[t, j:j + 1, :], (8, 128)) for j in range(4)]
        kf[8:, :] = kbuf[sl].astype(f32)

        zz = jnp.minimum(t, 0)

        def spec(j):
            for u in range(8):
                rows = []
                for hf in range(2):
                    r = j * 128 + u * 16 + hf * 8
                    acc = kf[pl.ds(r + 5, 8), :] * w[3]
                    acc = acc + kf[pl.ds(r + 6, 8), :] * w[2]
                    acc = acc + kf[pl.ds(r + 7, 8), :] * w[1]
                    acc = acc + kf[pl.ds(r + 8, 8), :] * w[0]
                    rows.append(acc)
                ks = jnp.concatenate(rows, axis=0)
                rr = pl.ds(pl.multiple_of(j * 128 + u * 16, 16), 16)
                kvbuf[pl.ds(pl.multiple_of(zz * 16 + j * 128 + u * 16, 16), 16), :] = (ks * vbuf[sl, rr, :].astype(f32)).astype(bf16)
            rj = pl.ds(pl.multiple_of(j * 128, 128), 128)
            xs[j] = jnp.dot(F_v[...], kvbuf[rj, :], preferred_element_type=f32)
            as_[j] = lax.dot_general(F_v[...], hbuf[sl, :, rj], (((1,), (1,)), ((), ())), preferred_element_type=f32)

        def conv_gen(b):
            re = pl.ds(pl.multiple_of(b * 8, 8), 8)
            im = pl.ds(pl.multiple_of(128 + b * 8, 8), 8)
            prev = None
            for i0 in range(0, NC, BLK):
                acc = {}
                acache = {}
                for j in range(0, i0 + BLK):
                    xr = xs[zz + j, re, :]
                    xi = xs[zz + j, im, :]
                    xsum = xr + xi
                    for i in range(max(i0, j), i0 + BLK):
                        if i - j not in acache:
                            ar = as_[zz + (i - j), re, :]
                            ai = as_[zz + (i - j), im, :]
                            acache[i - j] = (ar, ai, ar + ai)
                        ar, ai, asum = acache[i - j]
                        t_ = (ar * xr, ai * xi, asum * xsum)
                        acc[i] = t_ if i not in acc else tuple(u_ + v_ for u_, v_ in zip(acc[i], t_))
                    yield
                for i in range(i0, i0 + BLK):
                    p1, p2, p3 = acc[i]
                    yr, yi = p1 - p2, (p3 - p1) - p2
                    if prev is None:
                        ybuf[zz + i, re, :] = yr
                        ybuf[zz + i, im, :] = yi
                    else:
                        ybuf[zz + i, re, :] = yr - sgn * prev[1]
                        ybuf[zz + i, im, :] = yi + sgn * prev[0]
                    prev = (yr, yi)

        def conv(b):
            for _ in conv_gen(b):
                pass

        dv = jnp.broadcast_to(tapbuf[t, 4:5, :], (128, 128))

        def inv(i):
            y = jnp.dot(G_v[...], ybuf[i].astype(bf16), preferred_element_type=f32)
            rr = pl.ds(pl.multiple_of(i * 128, 128), 128)
            kv = kvbuf[rr, :].astype(f32)
            qq = qbuf[sl, rr, :].astype(f32)
            bobuf[sl, rr, :] = (qq * (y + kv * dv)).astype(bf16)

        P0, PZ, PE = (3, (0, 3, 6, 9, 12, 15), 1)
        assert P0 + len(PZ) + PE == 10
        nxt = iter(range(10))
        for _ in range(P0):
            adot(16 + 10 * t + next(nxt))
        for z in range(NC):
            spec(z)
        for z in range(16):
            if z in PZ:
                adot(16 + 10 * t + next(nxt))
            conv(z)
        for z in range(NC):
            inv(z)
        for _ in range(PE):
            adot(16 + 10 * t + next(nxt))
        sc_.__exit__(None, None, None)
        o_dma(t).start()

        @pl.when(t + 2 < NT)
        def _():
            for cp in in_dmas(t + 2):
                cp.start()
        return 0
    if '0' != '1':
        with scope('phase1'):
            lax.fori_loop(0, NT, tile, 0)
    else:
        x1.start(); m0.start()

    mid_ = scope('mid'); mid_.__enter__()
    x1.wait()
    m0.wait()

    def fill_cur(s):
        rpos = pl.multiple_of((SEG * s + ROFF) % RING, 32)
        for sl in range(96):
            cur[sl] = pltpu.bitcast(ring[sl, pl.ds(rpos, SEG), :], u32)
    fill_cur(0)

    mid_.__exit__(None, None, None)
    scale = E ** -0.5
    L2 = 2 * (SEG + M)
    ri = lax.broadcasted_iota(jnp.int32, (L2, L2), 0)
    ci = lax.broadcasted_iota(jnp.int32, (L2, L2), 1)

    def head_and_pos(i):
        is_mem = i >= 2 * SEG
        hd = jnp.where(is_mem, (i - 2 * SEG) // M, i // SEG)
        return is_mem, hd, i % SEG
    r_mem, r_hd, r_pos = head_and_pos(ri)
    c_mem, c_hd, c_pos = head_and_pos(ci)
    same_head = r_hd == c_hd
    visible = r_mem | c_mem | (c_pos <= r_pos)
    keep = same_head & visible
    fill = jnp.where(same_head, -1e9, -jnp.inf).astype(f32)

    def step(s, mem, tail=False):
        fresh = FILL - M * (NSEG - 1 - s)
        final = s == NSEG - 1
        xrow = pl.multiple_of(PRO + FILL * s, 8)
        xin = x_v[pl.ds(xrow, FILL), :]
        lhs = jnp.concatenate([mem.astype(bf16), xin], axis=0)
        wpos = pl.multiple_of((FILL * s) % RING, 8)
        prow = pl.multiple_of(jnp.maximum(FILL * (s - 1), 0), 8)
        lo_scr[M:, :] = obuf_x[pl.ds(prow, FILL), :]
        parts, S_, P_, O_ = {}, {}, {}, {}

        newx = {}

        def st_qkv(j):
            ps = []
            for m in range(3):
                sl = m * 32 + j
                w = pltpu.bitcast(wqkv[pl.ds(sl * WS, 512), :], bf16)
                y = jnp.dot(lhs, w, preferred_element_type=f32)
                ring[sl, pl.ds(wpos, FILL), :] = y[M:].astype(bf16)
                if tail:
                    newx[sl] = y[M:]
                ps.append(y[:M])
            parts[j] = ps

        npos = pl.multiple_of((SEG * (s + 1) + ROFF) % RING, 32)

        def refill(sl):
            cur[sl] = pltpu.bitcast(ring[sl, pl.ds(npos, SEG), :], u32)

        def tokens(sl):
            c_ = pltpu.bitcast(cur[sl], bf16)
            if tail:
                o_ = c_.astype(f32)
                n_ = newx.pop(sl)
                f0, f1, f2 = n_[0:8], n_[8:16], n_[16:24]
                c_ = jnp.concatenate([
                    o_[0:8],
                    jnp.where(fresh == 24, f0, o_[8:16]),
                    jnp.where(fresh == 24, f1, jnp.where(fresh == 16, f0, o_[16:24])),
                    jnp.where(fresh == 24, f2, jnp.where(fresh == 16, f1, f0)),
                ], axis=0).astype(bf16)
            return c_

        def pair(m, p_):
            ja, jb = 2 * p_, 2 * p_ + 1
            mm = jnp.concatenate([parts[ja][m], parts[jb][m]], axis=0).astype(bf16)
            return jnp.concatenate([tokens(m * 32 + ja), tokens(m * 32 + jb), mm], axis=0)

        def st_qk(p_):
            q, k = pair(0, p_), pair(1, p_)
            S_[p_] = lax.dot_general(q, k, (((1,), (1,)), ((), ())), preferred_element_type=f32)
            for j in (2 * p_, 2 * p_ + 1):
                refill(j)
                refill(32 + j)

        def st_sm(p_):
            sc = jnp.where(keep, S_.pop(p_) * scale, fill)
            e = jnp.exp(sc - jnp.max(sc, axis=-1, keepdims=True))
            P_[p_] = (e / jnp.sum(e, axis=-1, keepdims=True)).astype(bf16)

        def st_pv(p_):
            O_[p_] = jnp.dot(P_.pop(p_), pair(2, p_), preferred_element_type=f32)
            for j in (2 * p_, 2 * p_ + 1):
                refill(64 + j)

        def st_ost(p_):
            o = O_.pop(p_)
            for z, j in enumerate((2 * p_, 2 * p_ + 1)):
                obuf_x[pl.ds(pl.multiple_of(SEG * s, 32), SEG), j * E:(j + 1) * E] = o[z * SEG:(z + 1) * SEG].astype(bf16)
                om = o[2 * SEG + z * M:2 * SEG + (z + 1) * M].astype(bf16)
                if tail:
                    om = jnp.where(final, obuf_x[pl.ds(S - EPI - M, M), j * E:(j + 1) * E], om)
                lo_scr[0:M, j * E:(j + 1) * E] = om

        accs = {}

        def st_o(t, j0, j1):
            acc = accs.get(t)
            for j in range(j0, j1):
                hh = head_of_slot(j)
                w = pltpu.bitcast(wo[t, pl.ds(hh * 64, 64), :], bf16)
                y = jnp.dot(lo_scr[:, j * E:(j + 1) * E], w, preferred_element_type=f32)
                acc = y if acc is None else acc + y
            accs[t] = acc

        A, B_, C_, D_ = SKEW
        ou = {}
        for (j0, j1), slots in OCFG:
            for t_, sl_ in enumerate(slots):
                ou.setdefault(sl_, []).append((t_, j0, j1))
        last = max(max(ou), H - 1 + D_)

        def due(t, lag):
            u = t - lag - 1
            return u // 2 if (u >= 0 and u % 2 == 0 and u // 2 < H // 2) else None
        for t in range(last + 1):
            if t < H:
                st_qkv(t)
            for u in ou.get(t, []):
                st_o(*u)
            for lag, fn in ((A, st_qk), (B_, st_sm), (C_, st_pv), (D_, st_ost)):
                p_ = due(t, lag)
                if p_ is not None:
                    fn(p_)
        y = jnp.concatenate([accs[t] for t in range(8)], axis=1)
        obuf[pl.ds(prow, FILL), :] = y[M:].astype(bf16)
        if tail:
            obuf[pl.ds(S - EPI - M, M), :] = y[:M].astype(bf16)
        return y[:M]

    NLOOP = NSEG - 3

    def main_step(u, mem):
        mem = step(u, mem)

        @pl.when((u % 8 == 0) & (u >= 8))
        def _():
            a_dma(u // 8 - 1).start()
        return mem

    with scope('steps'):
        mem = lax.fori_loop(0, NLOOP, main_step, mem_v[...].astype(f32))
        lax.fori_loop(NLOOP, NSEG, lambda s_, m_: step(s_, m_, tail=True), mem)

    r0 = S - EPI
    e0 = (NT - 1) * 8 * FILL
    tail = pltpu.make_async_copy(obuf.at[pl.ds(e0, r0 - e0)], out_hbm.at[pl.ds(e0, r0 - e0), pl.ds(0, D)], osem.at[1])
    tail.start()

    def e_dma(t):
        cols = pl.ds(pl.multiple_of(t * 128, 128), 128)
        return pltpu.make_async_copy(obuf.at[pl.ds(r0, EPI), cols], out_hbm.at[pl.ds(r0, EPI), cols], osem.at[2])

    def epi(t, _):
        acc = None
        for j in range(H):
            hh = head_of_slot(j)
            w = pltpu.bitcast(wo[t, pl.ds(hh * 64, 64), :], bf16)
            y = jnp.dot(obuf_x[pl.ds(r0, EPI), j * E:(j + 1) * E], w, preferred_element_type=f32)
            acc = y if acc is None else acc + y
        obuf[pl.ds(r0, EPI), pl.ds(pl.multiple_of(t * 128, 128), 128)] = acc.astype(bf16)
        e_dma(t).start()
        return 0
    with scope('epi'):
        lax.fori_loop(0, 8, epi, 0)
    post_ = scope('post'); post_.__enter__()
    for c in range(NT - 1):
        a_dma(c).wait()
    o_dma(NT - 2).wait()
    o_dma(NT - 1).wait()
    tail.wait()
    for t in range(8):
        e_dma(t).wait()
    post_.__exit__(None, None, None)


@jax.jit
def run(A_x, A_mem0, A_Wq, A_Wk, A_Wv, A_Wo, B_q, B_k, B_v, B_shift_k, B_ssm_k, B_ssm_D):
    F, G = dft_consts()
    anyspec = pl.BlockSpec(memory_space=pl.ANY)
    vm = pl.BlockSpec(memory_space=pltpu.VMEM)
    out = pl.pallas_call(
        kernel,
        out_shape=jax.ShapeDtypeStruct((S, 2 * D), bf16),
        in_specs=[anyspec] * 10 + [vm] * 4, out_specs=anyspec,
        scratch_shapes=[
            pltpu.VMEM((S, D), bf16),
            pltpu.VMEM((8, PRO // 2, 128), u32),
            pltpu.VMEM((M, D), bf16),
            pltpu.VMEM((96 * WS, E), u32),
            pltpu.VMEM((8, 2048, 128), u32),
            pltpu.VMEM((2, D, 16, E), bf16),
            pltpu.VMEM((H * E, D), bf16),
            pltpu.VMEM((96, RING, E), bf16),
            pltpu.VMEM((S, H * E), bf16),
            pltpu.VMEM((S, D), bf16),
            pltpu.VMEM((32, H * E), bf16),
            pltpu.VMEM((96, SEG // 2, E), u32),
            pltpu.SemaphoreType.DMA((6,)),
            pltpu.SemaphoreType.DMA((3,)),
            pltpu.SemaphoreType.DMA((4,)),
            pltpu.VMEM((2, S, 128), bf16), pltpu.VMEM((2, S, 128), bf16), pltpu.VMEM((2, 128, S), bf16),
            pltpu.VMEM((2, S, 128), bf16), pltpu.VMEM((2, S, 128), bf16),
            pltpu.VMEM((S + 8, 128), f32), pltpu.VMEM((S, 128), bf16),
            pltpu.VMEM((NC, 256, 128), f32), pltpu.VMEM((NC, 256, 128), f32),
            pltpu.VMEM((NC, 256, 128), f32), pltpu.VMEM((NT, 8, 128), f32),
            pltpu.SemaphoreType.DMA((5, 2)),
        ],
        compiler_params=pltpu.CompilerParams(vmem_limit_bytes=120 * 1024 * 1024),
        name="fused",
    )(A_x.reshape(S, D), A_mem0.reshape(M, D), A_Wq, A_Wk, A_Wv, A_Wo.reshape(H * E, D),
      B_k.reshape(S, D), B_v.reshape(S, D), B_q.reshape(S, D), B_ssm_k, B_shift_k.T, B_ssm_D.reshape(8, 128), F, G)
    return out.reshape(1, S, 2 * D)


def pallas_concat_heads__memory_aug_recurrent_mem_tr__ssm_conv_h3__prompt_kernel(
    A_x, A_mem0, A_Wq, A_Wk, A_Wv, A_Wo, A_seg_len,
    B_q, B_k, B_v, B_shift_k, B_ssm_k, B_ssm_D,
):
    assert A_seg_len == SEG
    return run(A_x, A_mem0, A_Wq, A_Wk, A_Wv, A_Wo, B_q, B_k, B_v, B_shift_k, B_ssm_k, B_ssm_D)
```

```python
import jax
import jax.numpy as jnp
import numpy as np
import ml_dtypes
from jax import lax
from jax.experimental import pallas as pl
from jax.experimental.pallas import tpu as pltpu

S, D, H, E, M, SEG = 2048, 1024, 32, 128, 8, 32
NSEG = S // SEG
FILL = 24
PRO = S - FILL * NSEG
EPI = S - FILL * (NSEG - 1) - M
RING = 576
ROFF = 64
WS = 516
C = 128
NC = S // C
NT = D // 128
SKEW = tuple(int(c) for c in '1,1,4,4'.split(','))
OCFG = [((0, 4), [11, 12, 13, 14, 15, 16, 17, 18]), ((4, 26), [32, 33, 34, 35, 36, 37, 38, 39]), ((26, 32), [40] * 8)]
BLK = int('4')
RLU = int('8')
MD = int('1')
MB = int('3')
PIECES = (128, 128, 256, 512)
KUM = int('16')
POFF = tuple(sum(PIECES[:i]) for i in range(len(PIECES)))
import contextlib
SCOPES = '0' == '1'
scope = jax.named_scope if SCOPES else (lambda n: contextlib.nullcontext())
NQ = len(PIECES)
bf16, f32, u32 = jnp.bfloat16, jnp.float32, jnp.uint32


def head_of_slot(j):
    return (j // 16) * 16 + 2 * (j % 8) + ((j // 8) % 2)


def dft_consts():
    k = np.arange(C)[:, None].astype(np.float64)
    t = np.arange(C)[None, :].astype(np.float64)
    th = np.pi * (2 * k + 1) * t / (2 * C)
    F = np.concatenate([np.cos(th), -np.sin(th)], 0)
    G = np.concatenate([np.cos(th).T, -np.sin(th).T], 1) / C
    return F.astype(ml_dtypes.bfloat16), G.astype(ml_dtypes.bfloat16)


def kernel(x_hbm, mem0_hbm, wq_hbm, wk_hbm, wv_hbm, wo_hbm, k_hbm, v_hbm, q_hbm, h_hbm, sk_v, d_v, F_v, G_v,
           out_hbm,
           x_v, xp, mem_v, wqkv, wo, wstage, wostage, ring, obuf_x, obuf, lo_scr, cur, sems, osem, qsem, xsem, pacc,
           kbuf, vbuf, hbuf, qbuf, bobuf, kf, kvbuf, xs, as_, ybuf, tapbuf, bsem):
    LO = 0xFFFF
    HI = np.uint32(0xFFFF0000)
    sgn = (1 - 2 * (lax.broadcasted_iota(jnp.int32, (8, 128), 0) % 2)).astype(f32)

    def in_dmas(t):
        sl = t % 2
        c0 = pl.multiple_of(t * 128, 128)
        return [pltpu.make_async_copy(k_hbm.at[:, pl.ds(c0, 128)], kbuf.at[sl], bsem.at[0, sl]),
                pltpu.make_async_copy(v_hbm.at[:, pl.ds(c0, 128)], vbuf.at[sl], bsem.at[1, sl]),
                pltpu.make_async_copy(h_hbm.at[pl.ds(c0, 128), :], hbuf.at[sl], bsem.at[2, sl]),
                pltpu.make_async_copy(q_hbm.at[:, pl.ds(c0, 128)], qbuf.at[sl], bsem.at[3, sl])]

    def o_dma(t):
        sl = t % 2
        return pltpu.make_async_copy(bobuf.at[sl], out_hbm.at[:, pl.ds(pl.multiple_of(D + t * 128, 128), 128)], bsem.at[4, sl])

    def wdma(c, slot, src):
        return pltpu.make_async_copy(src.at[:, pl.ds((c % 2) * 16, 16), :], wstage.at[slot], sems.at[slot])

    def start_w(c, slot):
        for m, src in enumerate((wq_hbm, wk_hbm, wv_hbm)):
            @pl.when(c // 2 == m)
            def _():
                wdma(c, slot, src).start()

    def a_dma(c):
        rows = pl.ds(pl.multiple_of(c * 8 * FILL, 8), 8 * FILL)
        return pltpu.make_async_copy(obuf.at[rows], out_hbm.at[rows, pl.ds(0, D)], osem.at[0])

    x1 = pltpu.make_async_copy(x_hbm.at[pl.ds(PRO, S - PRO)], x_v.at[pl.ds(PRO, S - PRO)], sems.at[3])
    m0 = pltpu.make_async_copy(mem0_hbm, mem_v, sems.at[4])
    wod = pltpu.make_async_copy(wo_hbm, wostage, sems.at[5])
    pre_ = scope('pre'); pre_.__enter__()

    def w0_dma(i):
        rows = pl.ds(POFF[i], PIECES[i])
        return pltpu.make_async_copy(wq_hbm.at[rows, pl.ds(0, 16), :], wstage.at[0, rows], qsem.at[i])

    def xq_dma(i):
        cols = pl.ds(POFF[i], PIECES[i])
        return pltpu.make_async_copy(x_hbm.at[pl.ds(0, PRO), cols], x_v.at[pl.ds(0, PRO), cols], xsem.at[i])
    for i in range(NQ):
        xq_dma(i).start()
        w0_dma(i).start()

    kf[0:8, :] = jnp.zeros((8, 128), f32)
    dd = d_v[...].astype(f32)
    sk = sk_v[...].astype(f32)
    for t in range(NT):
        tapbuf[t, 0:4, :] = sk[:, t * 128:(t + 1) * 128]
        tapbuf[t, 4:5, :] = dd[t:t + 1, :]
    obuf_x[pl.ds(0, FILL), :] = jnp.zeros((FILL, H * E), bf16)
    def rl_rows(slot, base, i):
        for j in range(8):
            d = i * 16 + 2 * j
            a = pltpu.bitcast(wstage[slot, d], u32)
            b = pltpu.bitcast(wstage[slot, d + 1], u32)
            ev = (a & LO) | (b << 16)
            od = (a >> 16) | (b & HI)
            r = base + i * 8 + j
            wqkv[pl.ds(r, 8, stride=WS), :] = ev
            wqkv[pl.ds(r + 8 * WS, 8, stride=WS), :] = od

    def adot(sl_):
        wv = pltpu.bitcast(wqkv[pl.ds(sl_ * WS, 512), :], bf16)
        xx = jnp.concatenate([pltpu.bitcast(xp[kk], bf16) for kk in range(8)], axis=1)
        y = jnp.dot(xx, wv, preferred_element_type=f32)
        ring[sl_, pl.ds(ROFF, PRO), :] = y.astype(bf16)

    def relayout(c, slot, after_wait=None):
        with scope('wwait'):
            wdma(c, slot, wq_hbm).wait()
        if after_wait is not None:
            after_wait()
        base = c * 16 * WS

        def rl(i, _):
            for r_ in range(RLU):
                rl_rows(slot, base, i * RLU + r_)
            return 0
        lax.fori_loop(0, D // 16 // RLU, rl, 0)

    def more_dmas():
        start_w(1, 1)
    for i in range(NQ):
        with scope('qw%d' % i):
            xq_dma(i).wait()
            w0_dma(i).wait()
        if i == MD:
            more_dmas()
        if i == MB:
            for c in in_dmas(0):
                c.start()
        RQ = PIECES[i]
        KU = max(1, min(16, KUM * 128 // RQ))
        kks = range(POFF[i] // 128, (POFF[i] + RQ) // 128)
        for kk in kks:
            xp[kk, 0:PRO // 2, :] = pltpu.bitcast(x_v[0:PRO, kk * 128:(kk + 1) * 128], u32)

        RLQ = min(RLU, RQ // 16)

        def rlq(u, _, i=i, RLQ=RLQ):
            for r_ in range(RLQ):
                rl_rows(0, 0, POFF[i] // 16 + u * RLQ + r_)
            return 0
        if RQ // 16 // RLQ == 1:
            rlq(0, 0)
        else:
            lax.fori_loop(0, RQ // 16 // RLQ, rlq, 0)

        def part(u, _, i=i, kks=kks, KU=KU, RQ=RQ):
            for r_ in range(KU):
                sl_ = u * KU + r_
                wv = pltpu.bitcast(wqkv[pl.ds(sl_ * WS + POFF[i] // 2, RQ // 2), :], bf16)
                xx = jnp.concatenate([pltpu.bitcast(xp[kk], bf16) for kk in kks], axis=1)
                y = jnp.dot(xx, wv, preferred_element_type=f32)
                if i == 0:
                    pacc[sl_] = y
                elif i < NQ - 1:
                    pacc[sl_] = pacc[sl_] + y
                else:
                    ring[sl_, pl.ds(ROFF, PRO), :] = (pacc[sl_] + y).astype(bf16)
            return 0
        with scope('qp%d' % i):
            if KU == 16:
                part(0, 0)
            else:
                lax.fori_loop(0, 16 // KU, part, 0)
    pre_.__exit__(None, None, None)
    def tile(t, _):
        sl = t % 2
        c = t + 1 - (t >= 3).astype(jnp.int32) - (t >= 6).astype(jnp.int32)

        @pl.when(t >= 2)
        def _():
            o_dma(t - 2).wait()


        @pl.when((t != 2) & (t != 5) & (t != 7))
        def _():
            def early():
                @pl.when(t == 0)
                def _():
                    start_w(2, 0)
                    for cp in in_dmas(1):
                        cp.start()
            with scope('rl'):
                relayout(c, c % 2, early)

            @pl.when(c + 2 < 6)
            def _():
                start_w(c + 2, c % 2)

        @pl.when(t == 2)
        def _():
            wod.start(priority=1)

        @pl.when(t == 5)
        def _():
            x1.start()
            m0.start()

        @pl.when(t == 7)
        def _():
            wod.wait()

            def wo_rl(i, _):
                for n in range(8):
                    wo[n, pl.ds(i * 64, 64), :] = pltpu.bitcast(wostage[pl.ds(i * 128, 128), n * 128:(n + 1) * 128], u32)
                return 0
            lax.fori_loop(0, 32, wo_rl, 0)

        with scope('binwait'):
            for cp in in_dmas(t):
                cp.wait()

        sc_ = scope('main'); sc_.__enter__()

        w = [jnp.broadcast_to(tapbuf[t, j:j + 1, :], (8, 128)) for j in range(4)]
        kf[8:, :] = kbuf[sl].astype(f32)

        zz = jnp.minimum(t, 0)

        def spec(j):
            for u in range(8):
                rows = []
                for hf in range(2):
                    r = j * 128 + u * 16 + hf * 8
                    acc = kf[pl.ds(r + 5, 8), :] * w[3]
                    acc = acc + kf[pl.ds(r + 6, 8), :] * w[2]
                    acc = acc + kf[pl.ds(r + 7, 8), :] * w[1]
                    acc = acc + kf[pl.ds(r + 8, 8), :] * w[0]
                    rows.append(acc)
                ks = jnp.concatenate(rows, axis=0)
                rr = pl.ds(pl.multiple_of(j * 128 + u * 16, 16), 16)
                kvbuf[pl.ds(pl.multiple_of(zz * 16 + j * 128 + u * 16, 16), 16), :] = (ks * vbuf[sl, rr, :].astype(f32)).astype(bf16)
            rj = pl.ds(pl.multiple_of(j * 128, 128), 128)
            xs[j] = jnp.dot(F_v[...], kvbuf[rj, :], preferred_element_type=f32)
            as_[j] = lax.dot_general(F_v[...], hbuf[sl, :, rj], (((1,), (1,)), ((), ())), preferred_element_type=f32)

        def conv_gen(b):
            re = pl.ds(pl.multiple_of(b * 8, 8), 8)
            im = pl.ds(pl.multiple_of(128 + b * 8, 8), 8)
            prev = None
            for i0 in range(0, NC, BLK):
                acc = {}
                acache = {}
                for j in range(0, i0 + BLK):
                    xr = xs[zz + j, re, :]
                    xi = xs[zz + j, im, :]
                    xsum = xr + xi
                    for i in range(max(i0, j), i0 + BLK):
                        if i - j not in acache:
                            ar = as_[zz + (i - j), re, :]
                            ai = as_[zz + (i - j), im, :]
                            acache[i - j] = (ar, ai, ar + ai)
                        ar, ai, asum = acache[i - j]
                        t_ = (ar * xr, ai * xi, asum * xsum)
                        acc[i] = t_ if i not in acc else tuple(u_ + v_ for u_, v_ in zip(acc[i], t_))
                    yield
                for i in range(i0, i0 + BLK):
                    p1, p2, p3 = acc[i]
                    yr, yi = p1 - p2, (p3 - p1) - p2
                    if prev is None:
                        ybuf[zz + i, re, :] = yr
                        ybuf[zz + i, im, :] = yi
                    else:
                        ybuf[zz + i, re, :] = yr - sgn * prev[1]
                        ybuf[zz + i, im, :] = yi + sgn * prev[0]
                    prev = (yr, yi)

        def conv(b):
            for _ in conv_gen(b):
                pass

        dv = jnp.broadcast_to(tapbuf[t, 4:5, :], (128, 128))

        def inv(i):
            y = jnp.dot(G_v[...], ybuf[i].astype(bf16), preferred_element_type=f32)
            rr = pl.ds(pl.multiple_of(i * 128, 128), 128)
            kv = kvbuf[rr, :].astype(f32)
            qq = qbuf[sl, rr, :].astype(f32)
            bobuf[sl, rr, :] = (qq * (y + kv * dv)).astype(bf16)

        P0, PZ, PE = (3, (0, 3, 6, 9, 12, 15), 1)
        assert P0 + len(PZ) + PE == 10
        nxt = iter(range(10))
        for _ in range(P0):
            adot(16 + 10 * t + next(nxt))
        for z in range(NC):
            spec(z)
        for z in range(16):
            if z in PZ:
                adot(16 + 10 * t + next(nxt))
            conv(z)
        for z in range(NC):
            inv(z)
        for _ in range(PE):
            adot(16 + 10 * t + next(nxt))
        sc_.__exit__(None, None, None)
        o_dma(t).start()

        @pl.when(t + 2 < NT)
        def _():
            for cp in in_dmas(t + 2):
                cp.start()
        return 0
    if '0' != '1':
        with scope('phase1'):
            lax.fori_loop(0, NT, tile, 0)
    else:
        x1.start(); m0.start()

    mid_ = scope('mid'); mid_.__enter__()
    x1.wait()
    m0.wait()

    def fill_cur(s):
        rpos = pl.multiple_of((SEG * s + ROFF) % RING, 32)
        for sl in range(96):
            cur[sl] = pltpu.bitcast(ring[sl, pl.ds(rpos, SEG), :], u32)
    fill_cur(0)

    mid_.__exit__(None, None, None)
    scale = E ** -0.5
    L2 = 2 * (SEG + M)
    ri = lax.broadcasted_iota(jnp.int32, (L2, L2), 0)
    ci = lax.broadcasted_iota(jnp.int32, (L2, L2), 1)

    def head_and_pos(i):
        is_mem = i >= 2 * SEG
        hd = jnp.where(is_mem, (i - 2 * SEG) // M, i // SEG)
        return is_mem, hd, i % SEG
    r_mem, r_hd, r_pos = head_and_pos(ri)
    c_mem, c_hd, c_pos = head_and_pos(ci)
    same_head = r_hd == c_hd
    visible = r_mem | c_mem | (c_pos <= r_pos)
    keep = same_head & visible
    fill = jnp.where(same_head, -1e9, -jnp.inf).astype(f32)

    def step(s, mem, tail=False):
        fresh = FILL - M * (NSEG - 1 - s)
        final = s == NSEG - 1
        xrow = pl.multiple_of(PRO + FILL * s, 8)
        xin = x_v[pl.ds(xrow, FILL), :]
        lhs = jnp.concatenate([mem.astype(bf16), xin], axis=0)
        wpos = pl.multiple_of((FILL * s) % RING, 8)
        prow = pl.multiple_of(jnp.maximum(FILL * (s - 1), 0), 8)
        lo_scr[M:, :] = obuf_x[pl.ds(prow, FILL), :]
        parts, S_, P_, O_ = {}, {}, {}, {}

        newx = {}

        def st_qkv(j):
            ps = []
            for m in range(3):
                sl = m * 32 + j
                w = pltpu.bitcast(wqkv[pl.ds(sl * WS, 512), :], bf16)
                y = jnp.dot(lhs, w, preferred_element_type=f32)
                ring[sl, pl.ds(wpos, FILL), :] = y[M:].astype(bf16)
                if tail:
                    newx[sl] = y[M:]
                ps.append(y[:M])
            parts[j] = ps

        npos = pl.multiple_of((SEG * (s + 1) + ROFF) % RING, 32)

        def refill(sl):
            cur[sl] = pltpu.bitcast(ring[sl, pl.ds(npos, SEG), :], u32)

        def tokens(sl):
            c_ = pltpu.bitcast(cur[sl], bf16)
            if tail:
                o_ = c_.astype(f32)
                n_ = newx.pop(sl)
                f0, f1, f2 = n_[0:8], n_[8:16], n_[16:24]
                c_ = jnp.concatenate([
                    o_[0:8],
                    jnp.where(fresh == 24, f0, o_[8:16]),
                    jnp.where(fresh == 24, f1, jnp.where(fresh == 16, f0, o_[16:24])),
                    jnp.where(fresh == 24, f2, jnp.where(fresh == 16, f1, f0)),
                ], axis=0).astype(bf16)
            return c_

        def pair(m, p_):
            ja, jb = 2 * p_, 2 * p_ + 1
            mm = jnp.concatenate([parts[ja][m], parts[jb][m]], axis=0).astype(bf16)
            return jnp.concatenate([tokens(m * 32 + ja), tokens(m * 32 + jb), mm], axis=0)

        def st_qk(p_):
            q, k = pair(0, p_), pair(1, p_)
            S_[p_] = lax.dot_general(q, k, (((1,), (1,)), ((), ())), preferred_element_type=f32)
            for j in (2 * p_, 2 * p_ + 1):
                refill(j)
                refill(32 + j)

        def st_sm(p_):
            sc = jnp.where(keep, S_.pop(p_) * scale, fill)
            e = jnp.exp(sc - jnp.max(sc, axis=-1, keepdims=True))
            P_[p_] = (e / jnp.sum(e, axis=-1, keepdims=True)).astype(bf16)

        def st_pv(p_):
            O_[p_] = jnp.dot(P_.pop(p_), pair(2, p_), preferred_element_type=f32)
            for j in (2 * p_, 2 * p_ + 1):
                refill(64 + j)

        def st_ost(p_):
            o = O_.pop(p_)
            for z, j in enumerate((2 * p_, 2 * p_ + 1)):
                obuf_x[pl.ds(pl.multiple_of(SEG * s, 32), SEG), j * E:(j + 1) * E] = o[z * SEG:(z + 1) * SEG].astype(bf16)
                om = o[2 * SEG + z * M:2 * SEG + (z + 1) * M].astype(bf16)
                if tail:
                    om = jnp.where(final, obuf_x[pl.ds(S - EPI - M, M), j * E:(j + 1) * E], om)
                lo_scr[0:M, j * E:(j + 1) * E] = om

        accs = {}

        def st_o(t, j0, j1):
            acc = accs.get(t)
            for j in range(j0, j1):
                hh = head_of_slot(j)
                w = pltpu.bitcast(wo[t, pl.ds(hh * 64, 64), :], bf16)
                y = jnp.dot(lo_scr[:, j * E:(j + 1) * E], w, preferred_element_type=f32)
                acc = y if acc is None else acc + y
            accs[t] = acc

        A, B_, C_, D_ = SKEW
        ou = {}
        for (j0, j1), slots in OCFG:
            for t_, sl_ in enumerate(slots):
                ou.setdefault(sl_, []).append((t_, j0, j1))
        last = max(max(ou), H - 1 + D_)

        def due(t, lag):
            u = t - lag - 1
            return u // 2 if (u >= 0 and u % 2 == 0 and u // 2 < H // 2) else None
        for t in range(last + 1):
            if t < H:
                st_qkv(t)
            for u in ou.get(t, []):
                st_o(*u)
            for lag, fn in ((A, st_qk), (B_, st_sm), (C_, st_pv), (D_, st_ost)):
                p_ = due(t, lag)
                if p_ is not None:
                    fn(p_)
        y = jnp.concatenate([accs[t] for t in range(8)], axis=1)
        obuf[pl.ds(prow, FILL), :] = y[M:].astype(bf16)
        if tail:
            obuf[pl.ds(S - EPI - M, M), :] = y[:M].astype(bf16)
        return y[:M]

    NLOOP = NSEG - 3

    def main_step(u, mem):
        mem = step(u, mem)

        @pl.when((u % 8 == 0) & (u >= 8))
        def _():
            a_dma(u // 8 - 1).start()
        return mem

    with scope('steps'):
        mem = lax.fori_loop(0, NLOOP, main_step, mem_v[...].astype(f32))
        lax.fori_loop(NLOOP, NSEG, lambda s_, m_: step(s_, m_, tail=True), mem)

    r0 = S - EPI
    e0 = (NT - 1) * 8 * FILL
    tail = pltpu.make_async_copy(obuf.at[pl.ds(e0, r0 - e0)], out_hbm.at[pl.ds(e0, r0 - e0), pl.ds(0, D)], osem.at[1])
    tail.start()

    def e_dma(t):
        cols = pl.ds(pl.multiple_of(t * 128, 128), 128)
        return pltpu.make_async_copy(obuf.at[pl.ds(r0, EPI), cols], out_hbm.at[pl.ds(r0, EPI), cols], osem.at[2])

    def epi(t, _):
        acc = None
        for j in range(H):
            hh = head_of_slot(j)
            w = pltpu.bitcast(wo[t, pl.ds(hh * 64, 64), :], bf16)
            y = jnp.dot(obuf_x[pl.ds(r0, EPI), j * E:(j + 1) * E], w, preferred_element_type=f32)
            acc = y if acc is None else acc + y
        obuf[pl.ds(r0, EPI), pl.ds(pl.multiple_of(t * 128, 128), 128)] = acc.astype(bf16)
        e_dma(t).start()
        return 0
    with scope('epi'):
        lax.fori_loop(0, 8, epi, 0)
    post_ = scope('post'); post_.__enter__()
    for c in range(NT - 1):
        a_dma(c).wait()
    o_dma(NT - 2).wait()
    o_dma(NT - 1).wait()
    tail.wait()
    for t in range(8):
        e_dma(t).wait()
    post_.__exit__(None, None, None)


@jax.jit
def run(A_x, A_mem0, A_Wq, A_Wk, A_Wv, A_Wo, B_q, B_k, B_v, B_shift_k, B_ssm_k, B_ssm_D):
    F, G = dft_consts()
    anyspec = pl.BlockSpec(memory_space=pl.ANY)
    vm = pl.BlockSpec(memory_space=pltpu.VMEM)
    out = pl.pallas_call(
        kernel,
        out_shape=jax.ShapeDtypeStruct((S, 2 * D), bf16),
        in_specs=[anyspec] * 10 + [vm] * 4, out_specs=anyspec,
        scratch_shapes=[
            pltpu.VMEM((S, D), bf16),
            pltpu.VMEM((8, PRO // 2, 128), u32),
            pltpu.VMEM((M, D), bf16),
            pltpu.VMEM((96 * WS, E), u32),
            pltpu.VMEM((8, 2048, 128), u32),
            pltpu.VMEM((2, D, 16, E), bf16),
            pltpu.VMEM((H * E, D), bf16),
            pltpu.VMEM((96, RING, E), bf16),
            pltpu.VMEM((S, H * E), bf16),
            pltpu.VMEM((S, D), bf16),
            pltpu.VMEM((32, H * E), bf16),
            pltpu.VMEM((96, SEG // 2, E), u32),
            pltpu.SemaphoreType.DMA((6,)),
            pltpu.SemaphoreType.DMA((3,)),
            pltpu.SemaphoreType.DMA((NQ,)),
            pltpu.SemaphoreType.DMA((NQ,)),
            pltpu.VMEM((16, PRO, E), f32),
            pltpu.VMEM((2, S, 128), bf16), pltpu.VMEM((2, S, 128), bf16), pltpu.VMEM((2, 128, S), bf16),
            pltpu.VMEM((2, S, 128), bf16), pltpu.VMEM((2, S, 128), bf16),
            pltpu.VMEM((S + 8, 128), f32), pltpu.VMEM((S, 128), bf16),
            pltpu.VMEM((NC, 256, 128), f32), pltpu.VMEM((NC, 256, 128), f32),
            pltpu.VMEM((NC, 256, 128), f32), pltpu.VMEM((NT, 8, 128), f32),
            pltpu.SemaphoreType.DMA((5, 2)),
        ],
        compiler_params=pltpu.CompilerParams(vmem_limit_bytes=120 * 1024 * 1024),
        name="fused",
    )(A_x.reshape(S, D), A_mem0.reshape(M, D), A_Wq, A_Wk, A_Wv, A_Wo.reshape(H * E, D),
      B_k.reshape(S, D), B_v.reshape(S, D), B_q.reshape(S, D), B_ssm_k, B_shift_k.T, B_ssm_D.reshape(8, 128), F, G)
    return out.reshape(1, S, 2 * D)


def pallas_concat_heads__memory_aug_recurrent_mem_tr__ssm_conv_h3__prompt_kernel(
    A_x, A_mem0, A_Wq, A_Wk, A_Wv, A_Wo, A_seg_len,
    B_q, B_k, B_v, B_shift_k, B_ssm_k, B_ssm_D,
):
    assert A_seg_len == SEG
    return run(A_x, A_mem0, A_Wq, A_Wk, A_Wv, A_Wo, B_q, B_k, B_v, B_shift_k, B_ssm_k, B_ssm_D)
```

```python
import jax
import jax.numpy as jnp
import numpy as np
import ml_dtypes
from jax import lax
from jax.experimental import pallas as pl
from jax.experimental.pallas import tpu as pltpu

S, D, H, E, M, SEG = 2048, 1024, 32, 128, 8, 32
NSEG = S // SEG
FILL = 24
PRO = S - FILL * NSEG
EPI = S - FILL * (NSEG - 1) - M
RING = 576
ROFF = 64
WS = 516
C = 128
NC = S // C
NT = D // 128
SKEW = tuple(int(c) for c in '1,1,4,4'.split(','))
OCFG = [((0, 24), [29, 30, 31, 32, 33, 34, 35, 36]), ((24, 32), [40] * 8)]
BLK = int('4')
RLU = int('16')
MD = int('1')
MB = int('3')
PIECES = (128, 128, 256, 512)
KUM = int('16')
KM = int('6')
UN = int('3')
POFF = tuple(sum(PIECES[:i]) for i in range(len(PIECES)))
import contextlib
SCOPES = '0' == '1'
scope = jax.named_scope if SCOPES else (lambda n: contextlib.nullcontext())
NQ = len(PIECES)
bf16, f32, u32 = jnp.bfloat16, jnp.float32, jnp.uint32


def head_of_slot(j):
    return (j // 16) * 16 + 2 * (j % 8) + ((j // 8) % 2)


def dft_consts():
    k = np.arange(C)[:, None].astype(np.float64)
    t = np.arange(C)[None, :].astype(np.float64)
    th = np.pi * (2 * k + 1) * t / (2 * C)
    F = np.concatenate([np.cos(th), -np.sin(th)], 0)
    G = np.concatenate([np.cos(th).T, -np.sin(th).T], 1) / C
    return F.astype(ml_dtypes.bfloat16), G.astype(ml_dtypes.bfloat16)


def kernel(x_hbm, mem0_hbm, wq_hbm, wk_hbm, wv_hbm, wo_hbm, k_hbm, v_hbm, q_hbm, h_hbm, sk_v, d_v, F_v, G_v,
           out_hbm,
           x_v, xp, mem_v, wqkv, wo, wstage, wostage, ring, obuf_x, obuf, lo_scr, cur, sems, osem, qsem, xsem, pacc,
           kbuf, vbuf, hbuf, qbuf, bobuf, kf, kvbuf, xs, as_, ybuf, tapbuf, bsem):
    LO = 0xFFFF
    HI = np.uint32(0xFFFF0000)
    sgn = (1 - 2 * (lax.broadcasted_iota(jnp.int32, (8, 128), 0) % 2)).astype(f32)

    def in_dmas(t):
        sl = t % 2
        c0 = pl.multiple_of(t * 128, 128)
        return [pltpu.make_async_copy(k_hbm.at[:, pl.ds(c0, 128)], kbuf.at[sl], bsem.at[0, sl]),
                pltpu.make_async_copy(v_hbm.at[:, pl.ds(c0, 128)], vbuf.at[sl], bsem.at[1, sl]),
                pltpu.make_async_copy(h_hbm.at[pl.ds(c0, 128), :], hbuf.at[sl], bsem.at[2, sl]),
                pltpu.make_async_copy(q_hbm.at[:, pl.ds(c0, 128)], qbuf.at[sl], bsem.at[3, sl])]

    def o_dma(t):
        sl = t % 2
        return pltpu.make_async_copy(bobuf.at[sl], out_hbm.at[:, pl.ds(pl.multiple_of(D + t * 128, 128), 128)], bsem.at[4, sl])

    def wdma(c, slot, src):
        return pltpu.make_async_copy(src.at[:, pl.ds((c % 2) * 16, 16), :], wstage.at[slot], sems.at[slot])

    def start_w(c, slot):
        for m, src in enumerate((wq_hbm, wk_hbm, wv_hbm)):
            @pl.when(c // 2 == m)
            def _():
                wdma(c, slot, src).start()

    def a_dma(c):
        rows = pl.ds(pl.multiple_of(c * 8 * FILL, 8), 8 * FILL)
        return pltpu.make_async_copy(obuf.at[rows], out_hbm.at[rows, pl.ds(0, D)], osem.at[0])

    x1 = pltpu.make_async_copy(x_hbm.at[pl.ds(PRO, S - PRO)], x_v.at[pl.ds(PRO, S - PRO)], sems.at[3])
    m0 = pltpu.make_async_copy(mem0_hbm, mem_v, sems.at[4])
    wod = pltpu.make_async_copy(wo_hbm, wostage, sems.at[5])
    pre_ = scope('pre'); pre_.__enter__()

    def w0_dma(i):
        rows = pl.ds(POFF[i], PIECES[i])
        return pltpu.make_async_copy(wq_hbm.at[rows, pl.ds(0, 16), :], wstage.at[0, rows], qsem.at[i])

    def xq_dma(i):
        cols = pl.ds(POFF[i], PIECES[i])
        return pltpu.make_async_copy(x_hbm.at[pl.ds(0, PRO), cols], x_v.at[pl.ds(0, PRO), cols], xsem.at[i])
    for i in range(NQ):
        xq_dma(i).start()
        w0_dma(i).start()

    kf[0:8, :] = jnp.zeros((8, 128), f32)
    dd = d_v[...].astype(f32)
    sk = sk_v[...].astype(f32)
    for t in range(NT):
        tapbuf[t, 0:4, :] = sk[:, t * 128:(t + 1) * 128]
        tapbuf[t, 4:5, :] = dd[t:t + 1, :]
    obuf_x[pl.ds(0, FILL), :] = jnp.zeros((FILL, H * E), bf16)
    def rl_rows(slot, base, i):
        for j in range(8):
            d = i * 16 + 2 * j
            a = pltpu.bitcast(wstage[slot, d], u32)
            b = pltpu.bitcast(wstage[slot, d + 1], u32)
            ev = (a & LO) | (b << 16)
            od = (a >> 16) | (b & HI)
            r = base + i * 8 + j
            wqkv[pl.ds(r, 8, stride=WS), :] = ev
            wqkv[pl.ds(r + 8 * WS, 8, stride=WS), :] = od

    def adot(sl_):
        wv = pltpu.bitcast(wqkv[pl.ds(sl_ * WS, 512), :], bf16)
        xx = jnp.concatenate([pltpu.bitcast(xp[kk], bf16) for kk in range(8)], axis=1)
        y = jnp.dot(xx, wv, preferred_element_type=f32)
        ring[sl_, pl.ds(ROFF, PRO), :] = y.astype(bf16)

    def relayout(c, slot, after_wait=None):
        with scope('wwait'):
            wdma(c, slot, wq_hbm).wait()
        if after_wait is not None:
            after_wait()
        base = c * 16 * WS

        def rl(i, _):
            for r_ in range(RLU):
                rl_rows(slot, base, i * RLU + r_)
            return 0
        lax.fori_loop(0, D // 16 // RLU, rl, 0)

    def more_dmas():
        start_w(1, 1)
    for i in range(NQ):
        with scope('qw%d' % i):
            xq_dma(i).wait()
            w0_dma(i).wait()
        if i == MD:
            more_dmas()
        if i == MB:
            for c in in_dmas(0):
                c.start()
        RQ = PIECES[i]
        KU = max(1, min(16, KUM * 128 // RQ))
        kks = range(POFF[i] // 128, (POFF[i] + RQ) // 128)
        for kk in kks:
            xp[kk, 0:PRO // 2, :] = pltpu.bitcast(x_v[0:PRO, kk * 128:(kk + 1) * 128], u32)

        RLQ = min(RLU, RQ // 16)

        def rlq(u, _, i=i, RLQ=RLQ):
            for r_ in range(RLQ):
                rl_rows(0, 0, POFF[i] // 16 + u * RLQ + r_)
            return 0
        if RQ // 16 // RLQ == 1:
            rlq(0, 0)
        else:
            lax.fori_loop(0, RQ // 16 // RLQ, rlq, 0)

        def part(u, _, i=i, kks=kks, KU=KU, RQ=RQ):
            for r_ in range(KU):
                sl_ = u * KU + r_
                wv = pltpu.bitcast(wqkv[pl.ds(sl_ * WS + POFF[i] // 2, RQ // 2), :], bf16)
                xx = jnp.concatenate([pltpu.bitcast(xp[kk], bf16) for kk in kks], axis=1)
                y = jnp.dot(xx, wv, preferred_element_type=f32)
                if i == 0:
                    pacc[sl_] = y
                elif i < NQ - 1:
                    pacc[sl_] = pacc[sl_] + y
                else:
                    ring[sl_, pl.ds(ROFF, PRO), :] = (pacc[sl_] + y).astype(bf16)
            return 0
        with scope('qp%d' % i):
            if KU == 16:
                part(0, 0)
            else:
                lax.fori_loop(0, 16 // KU, part, 0)
    pre_.__exit__(None, None, None)
    def tile(t, _):
        sl = t % 2
        c = t + 1 - (t >= 3).astype(jnp.int32) - (t >= 6).astype(jnp.int32)

        @pl.when(t >= 2)
        def _():
            o_dma(t - 2).wait()


        @pl.when((t != 2) & (t != 5) & (t != 7))
        def _():
            def early():
                @pl.when(t == 0)
                def _():
                    start_w(2, 0)
                    for cp in in_dmas(1):
                        cp.start()
            with scope('rl'):
                relayout(c, c % 2, early)

            @pl.when(c + 2 < 6)
            def _():
                start_w(c + 2, c % 2)

        @pl.when(t == 2)
        def _():
            wod.start(priority=1)

        @pl.when(t == 5)
        def _():
            x1.start()
            m0.start()

        @pl.when(t == 7)
        def _():
            wod.wait()

            def wo_rl(i, _):
                for n in range(8):
                    wo[n, pl.ds(i * 64, 64), :] = pltpu.bitcast(wostage[pl.ds(i * 128, 128), n * 128:(n + 1) * 128], u32)
                return 0
            lax.fori_loop(0, 32, wo_rl, 0)

        with scope('binwait'):
            for cp in in_dmas(t):
                cp.wait()

        sc_ = scope('main'); sc_.__enter__()

        w = [jnp.broadcast_to(tapbuf[t, j:j + 1, :], (8, 128)) for j in range(4)]
        kf[8:, :] = kbuf[sl].astype(f32)

        zz = jnp.minimum(t, 0)

        def spec(j):
            for u in range(8):
                rows = []
                for hf in range(2):
                    r = j * 128 + u * 16 + hf * 8
                    acc = kf[pl.ds(r + 5, 8), :] * w[3]
                    acc = acc + kf[pl.ds(r + 6, 8), :] * w[2]
                    acc = acc + kf[pl.ds(r + 7, 8), :] * w[1]
                    acc = acc + kf[pl.ds(r + 8, 8), :] * w[0]
                    rows.append(acc)
                ks = jnp.concatenate(rows, axis=0)
                rr = pl.ds(pl.multiple_of(j * 128 + u * 16, 16), 16)
                kvbuf[pl.ds(pl.multiple_of(zz * 16 + j * 128 + u * 16, 16), 16), :] = (ks * vbuf[sl, rr, :].astype(f32)).astype(bf16)
            rj = pl.ds(pl.multiple_of(j * 128, 128), 128)
            xs[j] = jnp.dot(F_v[...], kvbuf[rj, :], preferred_element_type=f32)
            as_[j] = lax.dot_general(F_v[...], hbuf[sl, :, rj], (((1,), (1,)), ((), ())), preferred_element_type=f32)

        def conv_gen(b):
            re = pl.ds(pl.multiple_of(b * 8, 8), 8)
            im = pl.ds(pl.multiple_of(128 + b * 8, 8), 8)
            prev = None
            for i0 in range(0, NC, BLK):
                acc = {}
                acache = {}
                for j in range(0, i0 + BLK):
                    xr = xs[zz + j, re, :]
                    xi = xs[zz + j, im, :]
                    xsum = xr + xi
                    for i in range(max(i0, j), i0 + BLK):
                        if i - j not in acache:
                            ar = as_[zz + (i - j), re, :]
                            ai = as_[zz + (i - j), im, :]
                            acache[i - j] = (ar, ai, ar + ai)
                        ar, ai, asum = acache[i - j]
                        t_ = (ar * xr, ai * xi, asum * xsum)
                        acc[i] = t_ if i not in acc else tuple(u_ + v_ for u_, v_ in zip(acc[i], t_))
                    yield
                for i in range(i0, i0 + BLK):
                    p1, p2, p3 = acc[i]
                    yr, yi = p1 - p2, (p3 - p1) - p2
                    if prev is None:
                        ybuf[zz + i, re, :] = yr
                        ybuf[zz + i, im, :] = yi
                    else:
                        ybuf[zz + i, re, :] = yr - sgn * prev[1]
                        ybuf[zz + i, im, :] = yi + sgn * prev[0]
                    prev = (yr, yi)

        def conv(b):
            for _ in conv_gen(b):
                pass

        dv = jnp.broadcast_to(tapbuf[t, 4:5, :], (128, 128))

        def inv(i):
            y = jnp.dot(G_v[...], ybuf[i].astype(bf16), preferred_element_type=f32)
            rr = pl.ds(pl.multiple_of(i * 128, 128), 128)
            kv = kvbuf[rr, :].astype(f32)
            qq = qbuf[sl, rr, :].astype(f32)
            bobuf[sl, rr, :] = (qq * (y + kv * dv)).astype(bf16)

        P0, PZ, PE = (3, (0, 3, 6, 9, 12, 15), 1)
        assert P0 + len(PZ) + PE == 10
        nxt = iter(range(10))
        for _ in range(P0):
            adot(16 + 10 * t + next(nxt))
        for z in range(NC):
            spec(z)
        for z in range(16):
            if z in PZ:
                adot(16 + 10 * t + next(nxt))
            conv(z)
        for z in range(NC):
            inv(z)
        for _ in range(PE):
            adot(16 + 10 * t + next(nxt))
        sc_.__exit__(None, None, None)
        o_dma(t).start()

        @pl.when(t + 2 < NT)
        def _():
            for cp in in_dmas(t + 2):
                cp.start()
        return 0
    if '0' != '1':
        with scope('phase1'):
            lax.fori_loop(0, NT, tile, 0)
    else:
        x1.start(); m0.start()

    mid_ = scope('mid'); mid_.__enter__()
    x1.wait()
    m0.wait()

    def fill_cur(s):
        rpos = pl.multiple_of((SEG * s + ROFF) % RING, 32)
        for sl in range(96):
            cur[sl] = pltpu.bitcast(ring[sl, pl.ds(rpos, SEG), :], u32)
    fill_cur(0)

    mid_.__exit__(None, None, None)
    scale = E ** -0.5
    L2 = 2 * (SEG + M)
    ri = lax.broadcasted_iota(jnp.int32, (L2, L2), 0)
    ci = lax.broadcasted_iota(jnp.int32, (L2, L2), 1)

    def head_and_pos(i):
        is_mem = i >= 2 * SEG
        hd = jnp.where(is_mem, (i - 2 * SEG) // M, i // SEG)
        return is_mem, hd, i % SEG
    r_mem, r_hd, r_pos = head_and_pos(ri)
    c_mem, c_hd, c_pos = head_and_pos(ci)
    same_head = r_hd == c_hd
    visible = r_mem | c_mem | (c_pos <= r_pos)
    keep = same_head & visible
    fill = jnp.where(same_head, -1e9, -jnp.inf).astype(f32)

    def step(s, mem, tail=False, split=False):
        fresh = FILL - M * (NSEG - 1 - s)
        final = s == NSEG - 1
        xrow = pl.multiple_of(PRO + FILL * s, 8)
        xin = x_v[pl.ds(xrow, FILL), :]
        lhs = jnp.concatenate([mem.astype(bf16), xin], axis=0)
        wpos = pl.multiple_of((FILL * s) % RING, 8)
        prow = pl.multiple_of(jnp.maximum(FILL * (s - 1), 0), 8)
        lo_scr[M:, :] = obuf_x[pl.ds(prow, FILL), :]
        parts, S_, P_, O_ = {}, {}, {}, {}

        newx = {}

        early = {}
        for k_ in range(8 if split else 0):
            for n_ in range(KM):
                sl = (n_ % 3) * 32 + n_ // 3
                w = pltpu.bitcast(wqkv[pl.ds(sl * WS + 64 * k_, 64), :], bf16)
                y = jnp.dot(lhs[:, 128 * k_:128 * (k_ + 1)], w, preferred_element_type=f32)
                early[sl] = y if k_ == 0 else early[sl] + y

        def st_qkv(j):
            ps = []
            for m in range(3):
                sl = m * 32 + j
                if sl in early:
                    y = early.pop(sl)
                else:
                    w = pltpu.bitcast(wqkv[pl.ds(sl * WS, 512), :], bf16)
                    y = jnp.dot(lhs, w, preferred_element_type=f32)
                ring[sl, pl.ds(wpos, FILL), :] = y[M:].astype(bf16)
                if tail:
                    newx[sl] = y[M:]
                ps.append(y[:M])
            parts[j] = ps

        npos = pl.multiple_of((SEG * (s + 1) + ROFF) % RING, 32)

        def refill(sl):
            cur[sl] = pltpu.bitcast(ring[sl, pl.ds(npos, SEG), :], u32)

        def tokens(sl):
            c_ = pltpu.bitcast(cur[sl], bf16)
            if tail:
                o_ = c_.astype(f32)
                n_ = newx.pop(sl)
                f0, f1, f2 = n_[0:8], n_[8:16], n_[16:24]
                c_ = jnp.concatenate([
                    o_[0:8],
                    jnp.where(fresh == 24, f0, o_[8:16]),
                    jnp.where(fresh == 24, f1, jnp.where(fresh == 16, f0, o_[16:24])),
                    jnp.where(fresh == 24, f2, jnp.where(fresh == 16, f1, jnp.where(fresh == 8, f0, o_[24:32]))),
                ], axis=0).astype(bf16)
            return c_

        def pair(m, p_):
            ja, jb = 2 * p_, 2 * p_ + 1
            mm = jnp.concatenate([parts[ja][m], parts[jb][m]], axis=0).astype(bf16)
            return jnp.concatenate([tokens(m * 32 + ja), tokens(m * 32 + jb), mm], axis=0)

        def st_qk(p_):
            q, k = pair(0, p_), pair(1, p_)
            S_[p_] = lax.dot_general(q, k, (((1,), (1,)), ((), ())), preferred_element_type=f32)
            for j in (2 * p_, 2 * p_ + 1):
                refill(j)
                refill(32 + j)

        def st_sm(p_):
            sc = jnp.where(keep, S_.pop(p_) * scale, fill)
            e = jnp.exp(sc - jnp.max(sc, axis=-1, keepdims=True))
            P_[p_] = (e / jnp.sum(e, axis=-1, keepdims=True)).astype(bf16)

        def st_pv(p_):
            O_[p_] = jnp.dot(P_.pop(p_), pair(2, p_), preferred_element_type=f32)
            for j in (2 * p_, 2 * p_ + 1):
                refill(64 + j)

        def st_ost(p_):
            o = O_.pop(p_)
            for z, j in enumerate((2 * p_, 2 * p_ + 1)):
                obuf_x[pl.ds(pl.multiple_of(SEG * s, 32), SEG), j * E:(j + 1) * E] = o[z * SEG:(z + 1) * SEG].astype(bf16)
                om = o[2 * SEG + z * M:2 * SEG + (z + 1) * M].astype(bf16)
                if tail:
                    om = jnp.where(final, obuf_x[pl.ds(S - EPI - M, M), j * E:(j + 1) * E], om)
                lo_scr[0:M, j * E:(j + 1) * E] = om

        accs = {}

        def st_o(t, j0, j1):
            acc = accs.get(t)
            for j in range(j0, j1):
                hh = head_of_slot(j)
                w = pltpu.bitcast(wo[t, pl.ds(hh * 64, 64), :], bf16)
                y = jnp.dot(lo_scr[:, j * E:(j + 1) * E], w, preferred_element_type=f32)
                acc = y if acc is None else acc + y
            accs[t] = acc

        A, B_, C_, D_ = SKEW
        ou = {}
        for (j0, j1), slots in OCFG:
            assert 2 * ((j1 - 1) // 2) + 1 + D_ < min(slots)
            for t_, sl_ in enumerate(slots):
                ou.setdefault(sl_, []).append((t_, j0, j1))
        last = max(max(ou), H - 1 + D_)

        def due(t, lag):
            u = t - lag - 1
            return u // 2 if (u >= 0 and u % 2 == 0 and u // 2 < H // 2) else None
        for t in range(last + 1):
            if t < H:
                st_qkv(t)
            for u in ou.get(t, []):
                st_o(*u)
            for lag, fn in ((A, st_qk), (B_, st_sm), (C_, st_pv), (D_, st_ost)):
                p_ = due(t, lag)
                if p_ is not None:
                    fn(p_)
        y = jnp.concatenate([accs[t] for t in range(8)], axis=1)
        obuf[pl.ds(prow, FILL), :] = y[M:].astype(bf16)
        if tail:
            obuf[pl.ds(S - EPI - M, M), :] = y[:M].astype(bf16)
        return y[:M]

    NLOOP = NSEG - 4

    def main_steps(u, mem):
        for i in range(UN):
            mem = step(u * UN + i, mem, split=i > 0)
        done = (u + 1) * UN - 1

        @pl.when((done % 8 < UN) & (done >= 8))
        def _():
            a_dma(done // 8 - 1).start()
        return mem

    with scope('steps'):
        mem = lax.fori_loop(0, NLOOP // UN, main_steps, mem_v[...].astype(f32))
        lax.fori_loop(NLOOP, NSEG, lambda s_, m_: step(s_, m_, tail=True), mem)

    r0 = S - EPI
    e0 = (NT - 1) * 8 * FILL
    tail = pltpu.make_async_copy(obuf.at[pl.ds(e0, r0 - e0)], out_hbm.at[pl.ds(e0, r0 - e0), pl.ds(0, D)], osem.at[1])
    tail.start()

    def e_dma(t):
        cols = pl.ds(pl.multiple_of(t * 128, 128), 128)
        return pltpu.make_async_copy(obuf.at[pl.ds(r0, EPI), cols], out_hbm.at[pl.ds(r0, EPI), cols], osem.at[2])

    def epi(t, _):
        acc = None
        for j in range(H):
            hh = head_of_slot(j)
            w = pltpu.bitcast(wo[t, pl.ds(hh * 64, 64), :], bf16)
            y = jnp.dot(obuf_x[pl.ds(r0, EPI), j * E:(j + 1) * E], w, preferred_element_type=f32)
            acc = y if acc is None else acc + y
        obuf[pl.ds(r0, EPI), pl.ds(pl.multiple_of(t * 128, 128), 128)] = acc.astype(bf16)
        e_dma(t).start()
        return 0
    with scope('epi'):
        lax.fori_loop(0, 8, epi, 0)
    post_ = scope('post'); post_.__enter__()
    for c in range(NT - 1):
        a_dma(c).wait()
    o_dma(NT - 2).wait()
    o_dma(NT - 1).wait()
    tail.wait()
    for t in range(8):
        e_dma(t).wait()
    post_.__exit__(None, None, None)


@jax.jit
def run(A_x, A_mem0, A_Wq, A_Wk, A_Wv, A_Wo, B_q, B_k, B_v, B_shift_k, B_ssm_k, B_ssm_D):
    F, G = dft_consts()
    anyspec = pl.BlockSpec(memory_space=pl.ANY)
    vm = pl.BlockSpec(memory_space=pltpu.VMEM)
    out = pl.pallas_call(
        kernel,
        out_shape=jax.ShapeDtypeStruct((S, 2 * D), bf16),
        in_specs=[anyspec] * 10 + [vm] * 4, out_specs=anyspec,
        scratch_shapes=[
            pltpu.VMEM((S, D), bf16),
            pltpu.VMEM((8, PRO // 2, 128), u32),
            pltpu.VMEM((M, D), bf16),
            pltpu.VMEM((96 * WS, E), u32),
            pltpu.VMEM((8, 2048, 128), u32),
            pltpu.VMEM((2, D, 16, E), bf16),
            pltpu.VMEM((H * E, D), bf16),
            pltpu.VMEM((96, RING, E), bf16),
            pltpu.VMEM((S, H * E), bf16),
            pltpu.VMEM((S, D), bf16),
            pltpu.VMEM((32, H * E), bf16),
            pltpu.VMEM((96, SEG // 2, E), u32),
            pltpu.SemaphoreType.DMA((6,)),
            pltpu.SemaphoreType.DMA((3,)),
            pltpu.SemaphoreType.DMA((NQ,)),
            pltpu.SemaphoreType.DMA((NQ,)),
            pltpu.VMEM((16, PRO, E), f32),
            pltpu.VMEM((2, S, 128), bf16), pltpu.VMEM((2, S, 128), bf16), pltpu.VMEM((2, 128, S), bf16),
            pltpu.VMEM((2, S, 128), bf16), pltpu.VMEM((2, S, 128), bf16),
            pltpu.VMEM((S + 8, 128), f32), pltpu.VMEM((S, 128), bf16),
            pltpu.VMEM((NC, 256, 128), f32), pltpu.VMEM((NC, 256, 128), f32),
            pltpu.VMEM((NC, 256, 128), f32), pltpu.VMEM((NT, 8, 128), f32),
            pltpu.SemaphoreType.DMA((5, 2)),
        ],
        compiler_params=pltpu.CompilerParams(vmem_limit_bytes=120 * 1024 * 1024),
        name="fused",
    )(A_x.reshape(S, D), A_mem0.reshape(M, D), A_Wq, A_Wk, A_Wv, A_Wo.reshape(H * E, D),
      B_k.reshape(S, D), B_v.reshape(S, D), B_q.reshape(S, D), B_ssm_k, B_shift_k.T, B_ssm_D.reshape(8, 128), F, G)
    return out.reshape(1, S, 2 * D)


def pallas_concat_heads__memory_aug_recurrent_mem_tr__ssm_conv_h3__prompt_kernel(
    A_x, A_mem0, A_Wq, A_Wk, A_Wv, A_Wo, A_seg_len,
    B_q, B_k, B_v, B_shift_k, B_ssm_k, B_ssm_D,
):
    assert A_seg_len == SEG
    return run(A_x, A_mem0, A_Wq, A_Wk, A_Wv, A_Wo, B_q, B_k, B_v, B_shift_k, B_ssm_k, B_ssm_D)
```

```python
import jax
import jax.numpy as jnp
import numpy as np
import ml_dtypes
from jax import lax
from jax.experimental import pallas as pl
from jax.experimental.pallas import tpu as pltpu

S, D, H, E, M, SEG = 2048, 1024, 32, 128, 8, 32
NSEG = S // SEG
FILL = 24
PRO = S - FILL * NSEG
EPI = S - FILL * (NSEG - 1) - M
RING = 576
ROFF = 64
WS = 516
C = 128
NC = S // C
NT = D // 128
SKEW = tuple(int(c) for c in '1,1,4,4'.split(','))
OCFG = [((0, 24), [29, 30, 31, 32, 33, 34, 35, 36]), ((24, 32), [40] * 8)]
BLK = int('4')
RLU = int('16')
MD = int('1')
MB = int('3')
PIECES = (128, 128, 256, 512)
KUM = int('16')
KM = int('6')
UN = int('3')
QORD = tuple(int(c) for c in '021')
LORD = 'qo0123'
EORD = tuple(int(c) for c in '012')
REF = 'kkp'
EU = int('2')
POFF = tuple(sum(PIECES[:i]) for i in range(len(PIECES)))
import contextlib
SCOPES = '0' == '1'
scope = jax.named_scope if SCOPES else (lambda n: contextlib.nullcontext())
NQ = len(PIECES)
bf16, f32, u32 = jnp.bfloat16, jnp.float32, jnp.uint32


def head_of_slot(j):
    return (j // 16) * 16 + 2 * (j % 8) + ((j // 8) % 2)


def dft_consts():
    k = np.arange(C)[:, None].astype(np.float64)
    t = np.arange(C)[None, :].astype(np.float64)
    th = np.pi * (2 * k + 1) * t / (2 * C)
    F = np.concatenate([np.cos(th), -np.sin(th)], 0)
    G = np.concatenate([np.cos(th).T, -np.sin(th).T], 1) / C
    return F.astype(ml_dtypes.bfloat16), G.astype(ml_dtypes.bfloat16)


def kernel(x_hbm, mem0_hbm, wq_hbm, wk_hbm, wv_hbm, wo_hbm, k_hbm, v_hbm, q_hbm, h_hbm, sk_v, d_v, F_v, G_v,
           out_hbm,
           x_v, xp, mem_v, wqkv, wo, wstage, wostage, ring, obuf_x, obuf, lo_scr, cur, sems, osem, qsem, xsem, pacc,
           kbuf, vbuf, hbuf, qbuf, bobuf, kf, kvbuf, xs, as_, ybuf, tapbuf, bsem):
    LO = 0xFFFF
    HI = np.uint32(0xFFFF0000)
    sgn = (1 - 2 * (lax.broadcasted_iota(jnp.int32, (8, 128), 0) % 2)).astype(f32)

    def in_dmas(t):
        sl = t % 2
        c0 = pl.multiple_of(t * 128, 128)
        return [pltpu.make_async_copy(k_hbm.at[:, pl.ds(c0, 128)], kbuf.at[sl], bsem.at[0, sl]),
                pltpu.make_async_copy(v_hbm.at[:, pl.ds(c0, 128)], vbuf.at[sl], bsem.at[1, sl]),
                pltpu.make_async_copy(h_hbm.at[pl.ds(c0, 128), :], hbuf.at[sl], bsem.at[2, sl]),
                pltpu.make_async_copy(q_hbm.at[:, pl.ds(c0, 128)], qbuf.at[sl], bsem.at[3, sl])]

    def o_dma(t):
        sl = t % 2
        return pltpu.make_async_copy(bobuf.at[sl], out_hbm.at[:, pl.ds(pl.multiple_of(D + t * 128, 128), 128)], bsem.at[4, sl])

    def wdma(c, slot, src):
        return pltpu.make_async_copy(src.at[:, pl.ds((c % 2) * 16, 16), :], wstage.at[slot], sems.at[slot])

    def start_w(c, slot):
        for m, src in enumerate((wq_hbm, wk_hbm, wv_hbm)):
            @pl.when(c // 2 == m)
            def _():
                wdma(c, slot, src).start()

    def a_dma(c):
        rows = pl.ds(pl.multiple_of(c * 8 * FILL, 8), 8 * FILL)
        return pltpu.make_async_copy(obuf.at[rows], out_hbm.at[rows, pl.ds(0, D)], osem.at[0])

    x1 = pltpu.make_async_copy(x_hbm.at[pl.ds(PRO, S - PRO)], x_v.at[pl.ds(PRO, S - PRO)], sems.at[3])
    m0 = pltpu.make_async_copy(mem0_hbm, mem_v, sems.at[4])
    wod = pltpu.make_async_copy(wo_hbm, wostage, sems.at[5])
    pre_ = scope('pre'); pre_.__enter__()

    def w0_dma(i):
        rows = pl.ds(POFF[i], PIECES[i])
        return pltpu.make_async_copy(wq_hbm.at[rows, pl.ds(0, 16), :], wstage.at[0, rows], qsem.at[i])

    def xq_dma(i):
        cols = pl.ds(POFF[i], PIECES[i])
        return pltpu.make_async_copy(x_hbm.at[pl.ds(0, PRO), cols], x_v.at[pl.ds(0, PRO), cols], xsem.at[i])
    for i in range(NQ):
        xq_dma(i).start()
        w0_dma(i).start()

    kf[0:8, :] = jnp.zeros((8, 128), f32)
    dd = d_v[...].astype(f32)
    sk = sk_v[...].astype(f32)
    for t in range(NT):
        tapbuf[t, 0:4, :] = sk[:, t * 128:(t + 1) * 128]
        tapbuf[t, 4:5, :] = dd[t:t + 1, :]
    obuf_x[pl.ds(0, FILL), :] = jnp.zeros((FILL, H * E), bf16)
    def rl_rows(slot, base, i):
        for j in range(8):
            d = i * 16 + 2 * j
            a = pltpu.bitcast(wstage[slot, d], u32)
            b = pltpu.bitcast(wstage[slot, d + 1], u32)
            ev = (a & LO) | (b << 16)
            od = (a >> 16) | (b & HI)
            r = base + i * 8 + j
            wqkv[pl.ds(r, 8, stride=WS), :] = ev
            wqkv[pl.ds(r + 8 * WS, 8, stride=WS), :] = od

    def adot(sl_):
        wv = pltpu.bitcast(wqkv[pl.ds(sl_ * WS, 512), :], bf16)
        xx = jnp.concatenate([pltpu.bitcast(xp[kk], bf16) for kk in range(8)], axis=1)
        y = jnp.dot(xx, wv, preferred_element_type=f32)
        ring[sl_, pl.ds(ROFF, PRO), :] = y.astype(bf16)

    def relayout(c, slot, after_wait=None):
        with scope('wwait'):
            wdma(c, slot, wq_hbm).wait()
        if after_wait is not None:
            after_wait()
        base = c * 16 * WS

        def rl(i, _):
            for r_ in range(RLU):
                rl_rows(slot, base, i * RLU + r_)
            return 0
        lax.fori_loop(0, D // 16 // RLU, rl, 0)

    def more_dmas():
        start_w(1, 1)
    for i in range(NQ):
        with scope('qw%d' % i):
            xq_dma(i).wait()
            w0_dma(i).wait()
        if i == MD:
            more_dmas()
        if i == MB:
            for c in in_dmas(0):
                c.start()
        RQ = PIECES[i]
        KU = max(1, min(16, KUM * 128 // RQ))
        kks = range(POFF[i] // 128, (POFF[i] + RQ) // 128)
        for kk in kks:
            xp[kk, 0:PRO // 2, :] = pltpu.bitcast(x_v[0:PRO, kk * 128:(kk + 1) * 128], u32)

        RLQ = min(RLU, RQ // 16)

        def rlq(u, _, i=i, RLQ=RLQ):
            for r_ in range(RLQ):
                rl_rows(0, 0, POFF[i] // 16 + u * RLQ + r_)
            return 0
        if RQ // 16 // RLQ == 1:
            rlq(0, 0)
        else:
            lax.fori_loop(0, RQ // 16 // RLQ, rlq, 0)

        def part(u, _, i=i, kks=kks, KU=KU, RQ=RQ):
            for r_ in range(KU):
                sl_ = u * KU + r_
                wv = pltpu.bitcast(wqkv[pl.ds(sl_ * WS + POFF[i] // 2, RQ // 2), :], bf16)
                xx = jnp.concatenate([pltpu.bitcast(xp[kk], bf16) for kk in kks], axis=1)
                y = jnp.dot(xx, wv, preferred_element_type=f32)
                if i == 0:
                    pacc[sl_] = y
                elif i < NQ - 1:
                    pacc[sl_] = pacc[sl_] + y
                else:
                    ring[sl_, pl.ds(ROFF, PRO), :] = (pacc[sl_] + y).astype(bf16)
            return 0
        with scope('qp%d' % i):
            if KU == 16:
                part(0, 0)
            else:
                lax.fori_loop(0, 16 // KU, part, 0)
    pre_.__exit__(None, None, None)
    def tile(t, _):
        sl = t % 2
        c = t + 1 - (t >= 3).astype(jnp.int32) - (t >= 6).astype(jnp.int32)

        @pl.when(t >= 2)
        def _():
            o_dma(t - 2).wait()


        @pl.when((t != 2) & (t != 5) & (t != 7))
        def _():
            def early():
                @pl.when(t == 0)
                def _():
                    start_w(2, 0)
                    for cp in in_dmas(1):
                        cp.start()
            with scope('rl'):
                relayout(c, c % 2, early)

            @pl.when(c + 2 < 6)
            def _():
                start_w(c + 2, c % 2)

        @pl.when(t == 2)
        def _():
            wod.start(priority=1)

        @pl.when(t == 5)
        def _():
            x1.start()
            m0.start()

        @pl.when(t == 7)
        def _():
            wod.wait()

            def wo_rl(i, _):
                for n in range(8):
                    wo[n, pl.ds(i * 64, 64), :] = pltpu.bitcast(wostage[pl.ds(i * 128, 128), n * 128:(n + 1) * 128], u32)
                return 0
            lax.fori_loop(0, 32, wo_rl, 0)

        with scope('binwait'):
            for cp in in_dmas(t):
                cp.wait()

        sc_ = scope('main'); sc_.__enter__()

        w = [jnp.broadcast_to(tapbuf[t, j:j + 1, :], (8, 128)) for j in range(4)]
        kf[8:, :] = kbuf[sl].astype(f32)

        zz = jnp.minimum(t, 0)

        def spec(j):
            for u in range(8):
                rows = []
                for hf in range(2):
                    r = j * 128 + u * 16 + hf * 8
                    acc = kf[pl.ds(r + 5, 8), :] * w[3]
                    acc = acc + kf[pl.ds(r + 6, 8), :] * w[2]
                    acc = acc + kf[pl.ds(r + 7, 8), :] * w[1]
                    acc = acc + kf[pl.ds(r + 8, 8), :] * w[0]
                    rows.append(acc)
                ks = jnp.concatenate(rows, axis=0)
                rr = pl.ds(pl.multiple_of(j * 128 + u * 16, 16), 16)
                kvbuf[pl.ds(pl.multiple_of(zz * 16 + j * 128 + u * 16, 16), 16), :] = (ks * vbuf[sl, rr, :].astype(f32)).astype(bf16)
            rj = pl.ds(pl.multiple_of(j * 128, 128), 128)
            xs[j] = jnp.dot(F_v[...], kvbuf[rj, :], preferred_element_type=f32)
            as_[j] = lax.dot_general(F_v[...], hbuf[sl, :, rj], (((1,), (1,)), ((), ())), preferred_element_type=f32)

        def conv_gen(b):
            re = pl.ds(pl.multiple_of(b * 8, 8), 8)
            im = pl.ds(pl.multiple_of(128 + b * 8, 8), 8)
            prev = None
            for i0 in range(0, NC, BLK):
                acc = {}
                acache = {}
                for j in range(0, i0 + BLK):
                    xr = xs[zz + j, re, :]
                    xi = xs[zz + j, im, :]
                    xsum = xr + xi
                    for i in range(max(i0, j), i0 + BLK):
                        if i - j not in acache:
                            ar = as_[zz + (i - j), re, :]
                            ai = as_[zz + (i - j), im, :]
                            acache[i - j] = (ar, ai, ar + ai)
                        ar, ai, asum = acache[i - j]
                        t_ = (ar * xr, ai * xi, asum * xsum)
                        acc[i] = t_ if i not in acc else tuple(u_ + v_ for u_, v_ in zip(acc[i], t_))
                    yield
                for i in range(i0, i0 + BLK):
                    p1, p2, p3 = acc[i]
                    yr, yi = p1 - p2, (p3 - p1) - p2
                    if prev is None:
                        ybuf[zz + i, re, :] = yr
                        ybuf[zz + i, im, :] = yi
                    else:
                        ybuf[zz + i, re, :] = yr - sgn * prev[1]
                        ybuf[zz + i, im, :] = yi + sgn * prev[0]
                    prev = (yr, yi)

        def conv(b):
            for _ in conv_gen(b):
                pass

        dv = jnp.broadcast_to(tapbuf[t, 4:5, :], (128, 128))

        def inv(i):
            y = jnp.dot(G_v[...], ybuf[i].astype(bf16), preferred_element_type=f32)
            rr = pl.ds(pl.multiple_of(i * 128, 128), 128)
            kv = kvbuf[rr, :].astype(f32)
            qq = qbuf[sl, rr, :].astype(f32)
            bobuf[sl, rr, :] = (qq * (y + kv * dv)).astype(bf16)

        P0, PZ, PE = (3, (0, 3, 6, 9, 12, 15), 1)
        assert P0 + len(PZ) + PE == 10
        nxt = iter(range(10))
        for _ in range(P0):
            adot(16 + 10 * t + next(nxt))
        for z in range(NC):
            spec(z)
        for z in range(16):
            if z in PZ:
                adot(16 + 10 * t + next(nxt))
            conv(z)
        for z in range(NC):
            inv(z)
        for _ in range(PE):
            adot(16 + 10 * t + next(nxt))
        sc_.__exit__(None, None, None)
        o_dma(t).start()

        @pl.when(t + 2 < NT)
        def _():
            for cp in in_dmas(t + 2):
                cp.start()
        return 0
    if '0' != '1':
        with scope('phase1'):
            lax.fori_loop(0, NT, tile, 0)
    else:
        x1.start(); m0.start()

    mid_ = scope('mid'); mid_.__enter__()
    x1.wait()
    m0.wait()

    def fill_cur(s):
        rpos = pl.multiple_of((SEG * s + ROFF) % RING, 32)
        for sl in range(96):
            cur[sl] = pltpu.bitcast(ring[sl, pl.ds(rpos, SEG), :], u32)
    fill_cur(0)

    mid_.__exit__(None, None, None)
    scale = E ** -0.5
    L2 = 2 * (SEG + M)
    ri = lax.broadcasted_iota(jnp.int32, (L2, L2), 0)
    ci = lax.broadcasted_iota(jnp.int32, (L2, L2), 1)

    def head_and_pos(i):
        is_mem = i >= 2 * SEG
        hd = jnp.where(is_mem, (i - 2 * SEG) // M, i // SEG)
        return is_mem, hd, i % SEG
    r_mem, r_hd, r_pos = head_and_pos(ri)
    c_mem, c_hd, c_pos = head_and_pos(ci)
    same_head = r_hd == c_hd
    visible = r_mem | c_mem | (c_pos <= r_pos)
    keep = same_head & visible
    fill = jnp.where(same_head, -1e9, -jnp.inf).astype(f32)

    def step(s, mem, tail=False, split=False):
        fresh = FILL - M * (NSEG - 1 - s)
        final = s == NSEG - 1
        xrow = pl.multiple_of(PRO + FILL * s, 8)
        xin = x_v[pl.ds(xrow, FILL), :]
        lhs = jnp.concatenate([mem.astype(bf16), xin], axis=0)
        wpos = pl.multiple_of((FILL * s) % RING, 8)
        prow = pl.multiple_of(jnp.maximum(FILL * (s - 1), 0), 8)
        lo_scr[M:, :] = obuf_x[pl.ds(prow, FILL), :]
        parts, S_, P_, O_ = {}, {}, {}, {}

        newx = {}

        early = {}
        for k_ in range(8 if split else 0):
            for n_ in range(KM):
                sl = EORD[n_ % 3] * 32 + n_ // 3
                w = pltpu.bitcast(wqkv[pl.ds(sl * WS + 64 * k_, 64), :], bf16)
                y = jnp.dot(lhs[:, 128 * k_:128 * (k_ + 1)], w, preferred_element_type=f32)
                early[sl] = y if k_ == 0 else early[sl] + y

        def st_qkv(j):
            ps = {}
            for m in QORD:
                sl = m * 32 + j
                if sl in early:
                    y = early.pop(sl)
                else:
                    w = pltpu.bitcast(wqkv[pl.ds(sl * WS, 512), :], bf16)
                    y = jnp.dot(lhs, w, preferred_element_type=f32)
                ring[sl, pl.ds(wpos, FILL), :] = y[M:].astype(bf16)
                if tail:
                    newx[sl] = y[M:]
                ps[m] = y[:M]
            parts[j] = ps

        npos = pl.multiple_of((SEG * (s + 1) + ROFF) % RING, 32)

        def refill(sl):
            cur[sl] = pltpu.bitcast(ring[sl, pl.ds(npos, SEG), :], u32)

        def refills(p_, where):
            for j in (2 * p_, 2 * p_ + 1):
                for m in range(3):
                    if REF[m] == where:
                        refill(m * 32 + j)

        def tokens(sl):
            c_ = pltpu.bitcast(cur[sl], bf16)
            if tail:
                o_ = c_.astype(f32)
                n_ = newx.pop(sl)
                f0, f1, f2 = n_[0:8], n_[8:16], n_[16:24]
                c_ = jnp.concatenate([
                    o_[0:8],
                    jnp.where(fresh == 24, f0, o_[8:16]),
                    jnp.where(fresh == 24, f1, jnp.where(fresh == 16, f0, o_[16:24])),
                    jnp.where(fresh == 24, f2, jnp.where(fresh == 16, f1, jnp.where(fresh == 8, f0, o_[24:32]))),
                ], axis=0).astype(bf16)
            return c_

        def pair(m, p_):
            ja, jb = 2 * p_, 2 * p_ + 1
            mm = jnp.concatenate([parts[ja][m], parts[jb][m]], axis=0).astype(bf16)
            return jnp.concatenate([tokens(m * 32 + ja), tokens(m * 32 + jb), mm], axis=0)

        def st_qk(p_):
            q, k = pair(0, p_), pair(1, p_)
            S_[p_] = lax.dot_general(q, k, (((1,), (1,)), ((), ())), preferred_element_type=f32)
            refills(p_, 'k')

        def st_sm(p_):
            sc = jnp.where(keep, S_.pop(p_) * scale, fill)
            e = jnp.exp(sc - jnp.max(sc, axis=-1, keepdims=True))
            P_[p_] = (e / jnp.sum(e, axis=-1, keepdims=True)).astype(bf16)
            refills(p_, 's')

        def st_pv(p_):
            O_[p_] = jnp.dot(P_.pop(p_), pair(2, p_), preferred_element_type=f32)
            refills(p_, 'p')

        def st_ost(p_):
            o = O_.pop(p_)
            refills(p_, 'o')
            for z, j in enumerate((2 * p_, 2 * p_ + 1)):
                obuf_x[pl.ds(pl.multiple_of(SEG * s, 32), SEG), j * E:(j + 1) * E] = o[z * SEG:(z + 1) * SEG].astype(bf16)
                om = o[2 * SEG + z * M:2 * SEG + (z + 1) * M].astype(bf16)
                if tail:
                    om = jnp.where(final, obuf_x[pl.ds(S - EPI - M, M), j * E:(j + 1) * E], om)
                lo_scr[0:M, j * E:(j + 1) * E] = om

        accs = {}

        def st_o(t, j0, j1):
            acc = accs.get(t)
            for j in range(j0, j1):
                hh = head_of_slot(j)
                w = pltpu.bitcast(wo[t, pl.ds(hh * 64, 64), :], bf16)
                y = jnp.dot(lo_scr[:, j * E:(j + 1) * E], w, preferred_element_type=f32)
                acc = y if acc is None else acc + y
            accs[t] = acc

        A, B_, C_, D_ = SKEW
        ou = {}
        for (j0, j1), slots in OCFG:
            assert 2 * ((j1 - 1) // 2) + 1 + D_ < min(slots)
            for t_, sl_ in enumerate(slots):
                ou.setdefault(sl_, []).append((t_, j0, j1))
        last = max(max(ou), H - 1 + D_)

        def due(t, lag):
            u = t - lag - 1
            return u // 2 if (u >= 0 and u % 2 == 0 and u // 2 < H // 2) else None
        for t in range(last + 1):
            for what in LORD:
                if what == 'q':
                    if t < H:
                        st_qkv(t)
                elif what == 'o':
                    for u in ou.get(t, []):
                        st_o(*u)
                else:
                    lag, fn = ((A, st_qk), (B_, st_sm), (C_, st_pv), (D_, st_ost))[int(what)]
                    p_ = due(t, lag)
                    if p_ is not None:
                        fn(p_)
        y = jnp.concatenate([accs[t] for t in range(8)], axis=1)
        obuf[pl.ds(prow, FILL), :] = y[M:].astype(bf16)
        if tail:
            obuf[pl.ds(S - EPI - M, M), :] = y[:M].astype(bf16)
        return y[:M]

    NLOOP = NSEG - 4

    def main_steps(u, mem):
        for i in range(UN):
            mem = step(u * UN + i, mem, split=i > 0)
        done = (u + 1) * UN - 1

        @pl.when((done % 8 < UN) & (done >= 8))
        def _():
            a_dma(done // 8 - 1).start()
        return mem

    with scope('steps'):
        mem = lax.fori_loop(0, NLOOP // UN, main_steps, mem_v[...].astype(f32))
        lax.fori_loop(NLOOP, NSEG, lambda s_, m_: step(s_, m_, tail=True), mem)

    r0 = S - EPI
    e0 = (NT - 1) * 8 * FILL
    tail = pltpu.make_async_copy(obuf.at[pl.ds(e0, r0 - e0)], out_hbm.at[pl.ds(e0, r0 - e0), pl.ds(0, D)], osem.at[1])
    tail.start()

    def e_dma(t):
        cols = pl.ds(pl.multiple_of(t * 128, 128), 128)
        return pltpu.make_async_copy(obuf.at[pl.ds(r0, EPI), cols], out_hbm.at[pl.ds(r0, EPI), cols], osem.at[2])

    def epi(t):
        acc = None
        for j in range(H):
            hh = head_of_slot(j)
            w = pltpu.bitcast(wo[t, pl.ds(hh * 64, 64), :], bf16)
            y = jnp.dot(obuf_x[pl.ds(r0, EPI), j * E:(j + 1) * E], w, preferred_element_type=f32)
            acc = y if acc is None else acc + y
        obuf[pl.ds(r0, EPI), pl.ds(pl.multiple_of(t * 128, 128), 128)] = acc.astype(bf16)

    def epis(u, _):
        for i in range(EU):
            epi(u * EU + i)
        for i in range(EU):
            e_dma(u * EU + i).start()
        return 0
    with scope('epi'):
        lax.fori_loop(0, 8 // EU, epis, 0)
    post_ = scope('post'); post_.__enter__()
    for c in range(NT - 1):
        a_dma(c).wait()
    o_dma(NT - 2).wait()
    o_dma(NT - 1).wait()
    tail.wait()
    for t in range(8):
        e_dma(t).wait()
    post_.__exit__(None, None, None)


@jax.jit
def run(A_x, A_mem0, A_Wq, A_Wk, A_Wv, A_Wo, B_q, B_k, B_v, B_shift_k, B_ssm_k, B_ssm_D):
    F, G = dft_consts()
    anyspec = pl.BlockSpec(memory_space=pl.ANY)
    vm = pl.BlockSpec(memory_space=pltpu.VMEM)
    out = pl.pallas_call(
        kernel,
        out_shape=jax.ShapeDtypeStruct((S, 2 * D), bf16),
        in_specs=[anyspec] * 10 + [vm] * 4, out_specs=anyspec,
        scratch_shapes=[
            pltpu.VMEM((S, D), bf16),
            pltpu.VMEM((8, PRO // 2, 128), u32),
            pltpu.VMEM((M, D), bf16),
            pltpu.VMEM((96 * WS, E), u32),
            pltpu.VMEM((8, 2048, 128), u32),
            pltpu.VMEM((2, D, 16, E), bf16),
            pltpu.VMEM((H * E, D), bf16),
            pltpu.VMEM((96, RING, E), bf16),
            pltpu.VMEM((S, H * E), bf16),
            pltpu.VMEM((S, D), bf16),
            pltpu.VMEM((32, H * E), bf16),
            pltpu.VMEM((96, SEG // 2, E), u32),
            pltpu.SemaphoreType.DMA((6,)),
            pltpu.SemaphoreType.DMA((3,)),
            pltpu.SemaphoreType.DMA((NQ,)),
            pltpu.SemaphoreType.DMA((NQ,)),
            pltpu.VMEM((16, PRO, E), f32),
            pltpu.VMEM((2, S, 128), bf16), pltpu.VMEM((2, S, 128), bf16), pltpu.VMEM((2, 128, S), bf16),
            pltpu.VMEM((2, S, 128), bf16), pltpu.VMEM((2, S, 128), bf16),
            pltpu.VMEM((S + 8, 128), f32), pltpu.VMEM((S, 128), bf16),
            pltpu.VMEM((NC, 256, 128), f32), pltpu.VMEM((NC, 256, 128), f32),
            pltpu.VMEM((NC, 256, 128), f32), pltpu.VMEM((NT, 8, 128), f32),
            pltpu.SemaphoreType.DMA((5, 2)),
        ],
        compiler_params=pltpu.CompilerParams(vmem_limit_bytes=120 * 1024 * 1024),
        name="fused",
    )(A_x.reshape(S, D), A_mem0.reshape(M, D), A_Wq, A_Wk, A_Wv, A_Wo.reshape(H * E, D),
      B_k.reshape(S, D), B_v.reshape(S, D), B_q.reshape(S, D), B_ssm_k, B_shift_k.T, B_ssm_D.reshape(8, 128), F, G)
    return out.reshape(1, S, 2 * D)


def pallas_concat_heads__memory_aug_recurrent_mem_tr__ssm_conv_h3__prompt_kernel(
    A_x, A_mem0, A_Wq, A_Wk, A_Wv, A_Wo, A_seg_len,
    B_q, B_k, B_v, B_shift_k, B_ssm_k, B_ssm_D,
):
    assert A_seg_len == SEG
    return run(A_x, A_mem0, A_Wq, A_Wk, A_Wv, A_Wo, B_q, B_k, B_v, B_shift_k, B_ssm_k, B_ssm_D)
```

```python
import jax
import jax.numpy as jnp
import numpy as np
import ml_dtypes
from jax import lax
from jax.experimental import pallas as pl
from jax.experimental.pallas import tpu as pltpu

S, D, H, E, M, SEG = 2048, 1024, 32, 128, 8, 32
NSEG = S // SEG
FILL = 24
PRO = S - FILL * NSEG
EPI = S - FILL * (NSEG - 1) - M
RING = 576
ROFF = 64
WS = 516
C = 128
NC = S // C
NT = D // 128
SKEW = tuple(int(c) for c in '1,1,4,4'.split(','))
OCFG = [((0, 24), [29, 30, 31, 32, 33, 34, 35, 36]), ((24, 32), [40] * 8)]
BLK = int('4')
RLU = int('16')
MD = int('1')
KUX = int('8')
NA = int('4')
PIECES = (128, 128, 256, 512)
KUM = int('16')
KM = int('6')
UN = int('3')
QORD = tuple(int(c) for c in '021')
LORD = 'qo0123'
EORD = tuple(int(c) for c in '012')
REF = 'kkp'
EU = int('2')
POFF = tuple(sum(PIECES[:i]) for i in range(len(PIECES)))
import contextlib
SCOPES = '0' == '1'
scope = jax.named_scope if SCOPES else (lambda n: contextlib.nullcontext())
NQ = len(PIECES)
bf16, f32, u32 = jnp.bfloat16, jnp.float32, jnp.uint32


def head_of_slot(j):
    return (j // 16) * 16 + 2 * (j % 8) + ((j // 8) % 2)


def dft_consts():
    k = np.arange(C)[:, None].astype(np.float64)
    t = np.arange(C)[None, :].astype(np.float64)
    th = np.pi * (2 * k + 1) * t / (2 * C)
    F = np.concatenate([np.cos(th), -np.sin(th)], 0)
    G = np.concatenate([np.cos(th).T, -np.sin(th).T], 1) / C
    return F.astype(ml_dtypes.bfloat16), G.astype(ml_dtypes.bfloat16)


def kernel(x_hbm, mem0_hbm, wq_hbm, wk_hbm, wv_hbm, wo_hbm, k_hbm, v_hbm, q_hbm, h_hbm, sk_v, d_v, F_v, G_v,
           out_hbm,
           x_v, xp, mem_v, wqkv, wo, wstage, wostage, ring, obuf_x, obuf, lo_scr, cur, sems, osem, qsem, xsem, pacc,
           kbuf, vbuf, hbuf, qbuf, bobuf, kf, kvbuf, xs, as_, ybuf, tapbuf, bsem):
    LO = 0xFFFF
    HI = np.uint32(0xFFFF0000)
    sgn = (1 - 2 * (lax.broadcasted_iota(jnp.int32, (8, 128), 0) % 2)).astype(f32)

    def in_dmas(t):
        sl = t % 2
        c0 = pl.multiple_of(t * 128, 128)
        return [pltpu.make_async_copy(k_hbm.at[:, pl.ds(c0, 128)], kbuf.at[sl], bsem.at[0, sl]),
                pltpu.make_async_copy(v_hbm.at[:, pl.ds(c0, 128)], vbuf.at[sl], bsem.at[1, sl]),
                pltpu.make_async_copy(h_hbm.at[pl.ds(c0, 128), :], hbuf.at[sl], bsem.at[2, sl]),
                pltpu.make_async_copy(q_hbm.at[:, pl.ds(c0, 128)], qbuf.at[sl], bsem.at[3, sl])]

    def o_dma(t):
        sl = t % 2
        return pltpu.make_async_copy(bobuf.at[sl], out_hbm.at[:, pl.ds(pl.multiple_of(D + t * 128, 128), 128)], bsem.at[4, sl])

    def wdma(c, slot, src):
        return pltpu.make_async_copy(src.at[:, pl.ds((c % 2) * 16, 16), :], wstage.at[slot], sems.at[slot])

    def start_w(c, slot):
        for m, src in enumerate((wq_hbm, wk_hbm, wv_hbm)):
            @pl.when(c // 2 == m)
            def _():
                wdma(c, slot, src).start()

    def a_dma(c):
        rows = pl.ds(pl.multiple_of(c * 8 * FILL, 8), 8 * FILL)
        return pltpu.make_async_copy(obuf.at[rows], out_hbm.at[rows, pl.ds(0, D)], osem.at[0])

    x1 = pltpu.make_async_copy(x_hbm.at[pl.ds(PRO, S - PRO)], x_v.at[pl.ds(PRO, S - PRO)], sems.at[3])
    m0 = pltpu.make_async_copy(mem0_hbm, mem_v, sems.at[4])
    wod = pltpu.make_async_copy(wo_hbm, wostage, sems.at[5])
    pre_ = scope('pre'); pre_.__enter__()

    def w0_dma(i):
        rows = pl.ds(POFF[i], PIECES[i])
        return pltpu.make_async_copy(wq_hbm.at[rows, pl.ds(0, 16), :], wstage.at[0, rows], qsem.at[i])

    def xq_dma(i):
        cols = pl.ds(POFF[i], PIECES[i])
        return pltpu.make_async_copy(x_hbm.at[pl.ds(0, PRO), cols], x_v.at[pl.ds(0, PRO), cols], xsem.at[i])
    for i in range(NQ):
        xq_dma(i).start()
        w0_dma(i).start()

    kf[0:8, :] = jnp.zeros((8, 128), f32)
    dd = d_v[...].astype(f32)
    sk = sk_v[...].astype(f32)
    for t in range(NT):
        tapbuf[t, 0:4, :] = sk[:, t * 128:(t + 1) * 128]
        tapbuf[t, 4:5, :] = dd[t:t + 1, :]
    obuf_x[pl.ds(0, FILL), :] = jnp.zeros((FILL, H * E), bf16)
    def rl_rows(slot, base, i):
        for j in range(8):
            d = i * 16 + 2 * j
            a = pltpu.bitcast(wstage[slot, d], u32)
            b = pltpu.bitcast(wstage[slot, d + 1], u32)
            ev = (a & LO) | (b << 16)
            od = (a >> 16) | (b & HI)
            r = base + i * 8 + j
            wqkv[pl.ds(r, 8, stride=WS), :] = ev
            wqkv[pl.ds(r + 8 * WS, 8, stride=WS), :] = od

    def adot(sl_):
        wv = pltpu.bitcast(wqkv[pl.ds(sl_ * WS, 512), :], bf16)
        xx = jnp.concatenate([pltpu.bitcast(xp[kk], bf16) for kk in range(8)], axis=1)
        y = jnp.dot(xx, wv, preferred_element_type=f32)
        ring[sl_, pl.ds(ROFF, PRO), :] = y.astype(bf16)

    def relayout(c, slot, after_wait=None):
        with scope('wwait'):
            wdma(c, slot, wq_hbm).wait()
        if after_wait is not None:
            after_wait()
        base = c * 16 * WS

        def rl(i, _):
            for r_ in range(RLU):
                rl_rows(slot, base, i * RLU + r_)
            return 0
        lax.fori_loop(0, D // 16 // RLU, rl, 0)

    def more_dmas():
        start_w(1, 1)
    for i in range(NQ):
        with scope('qw%d' % i):
            xq_dma(i).wait()
            w0_dma(i).wait()
        if i == MD:
            more_dmas()
        RQ = PIECES[i]
        KU = max(1, min(KUX, KUM * 128 // RQ))
        kks = range(POFF[i] // 128, (POFF[i] + RQ) // 128)
        for kk in kks:
            xp[kk, 0:PRO // 2, :] = pltpu.bitcast(x_v[0:PRO, kk * 128:(kk + 1) * 128], u32)

        RLQ = min(RLU, RQ // 16)

        def rlq(u, _, i=i, RLQ=RLQ):
            for r_ in range(RLQ):
                rl_rows(0, 0, POFF[i] // 16 + u * RLQ + r_)
            return 0
        if RQ // 16 // RLQ == 1:
            rlq(0, 0)
        else:
            lax.fori_loop(0, RQ // 16 // RLQ, rlq, 0)

        if i == NQ - 1:
            start_w(2, 0)

        def part(u, _, i=i, kks=kks, KU=KU, RQ=RQ):
            for r_ in range(KU):
                sl_ = u * KU + r_
                wv = pltpu.bitcast(wqkv[pl.ds(sl_ * WS + POFF[i] // 2, RQ // 2), :], bf16)
                xx = jnp.concatenate([pltpu.bitcast(xp[kk], bf16) for kk in kks], axis=1)
                y = jnp.dot(xx, wv, preferred_element_type=f32)
                if i == 0:
                    pacc[sl_] = y
                elif i < NQ - 1:
                    pacc[sl_] = pacc[sl_] + y
                else:
                    ring[sl_, pl.ds(ROFF, PRO), :] = (pacc[sl_] + y).astype(bf16)
            return 0
        with scope('qp%d' % i):
            if KU == 16:
                part(0, 0)
            else:
                lax.fori_loop(0, 16 // KU, part, 0)

    def first_inputs():
        for t_ in range(2):
            for cp in in_dmas(t_):
                cp.start()
    relayout(1, 1, first_inputs)

    NG = 16 // NA
    NR = (D // 16) // (NG // 2)

    def slots16(g, _):
        late = g >= NG // 2

        @pl.when(g == NG // 2)
        def _():
            wdma(2, 0, wq_hbm).wait()
            start_w(3, 1)
        slot = jnp.where(late, 0, 1)
        base = jnp.where(late, 2, 1) * (16 * WS)
        for a_ in range(NA):
            adot(16 + g * NA + a_)
            for r_ in range(NR // NA):
                rl_rows(slot, base, (g % (NG // 2)) * NR + a_ * (NR // NA) + r_)
        return 0
    with scope('g16'):
        lax.fori_loop(0, NG, slots16, 0)
    pre_.__exit__(None, None, None)
    def tile(t, _):
        sl = t % 2
        c = t + 1 - (t >= 3).astype(jnp.int32) - (t >= 5).astype(jnp.int32)

        @pl.when(t >= 2)
        def _():
            o_dma(t - 2).wait()


        @pl.when(t == 0)
        def _():
            start_w(4, 0)

        @pl.when((t >= 2) & (t % 2 == 0))
        def _():
            with scope('rl'):
                relayout(c, c % 2)

            @pl.when(t == 2)
            def _():
                start_w(5, 1)

        @pl.when(t == 2)
        def _():
            wod.start(priority=1)

        @pl.when(t == 5)
        def _():
            x1.start()
            m0.start()

        @pl.when(t == 7)
        def _():
            wod.wait()

            def wo_rl(i, _):
                for n in range(8):
                    wo[n, pl.ds(i * 64, 64), :] = pltpu.bitcast(wostage[pl.ds(i * 128, 128), n * 128:(n + 1) * 128], u32)
                return 0
            lax.fori_loop(0, 32, wo_rl, 0)

        with scope('binwait'):
            for cp in in_dmas(t):
                cp.wait()

        sc_ = scope('main'); sc_.__enter__()

        w = [jnp.broadcast_to(tapbuf[t, j:j + 1, :], (8, 128)) for j in range(4)]
        kf[8:, :] = kbuf[sl].astype(f32)

        zz = jnp.minimum(t, 0)

        def spec(j):
            for u in range(8):
                rows = []
                for hf in range(2):
                    r = j * 128 + u * 16 + hf * 8
                    acc = kf[pl.ds(r + 5, 8), :] * w[3]
                    acc = acc + kf[pl.ds(r + 6, 8), :] * w[2]
                    acc = acc + kf[pl.ds(r + 7, 8), :] * w[1]
                    acc = acc + kf[pl.ds(r + 8, 8), :] * w[0]
                    rows.append(acc)
                ks = jnp.concatenate(rows, axis=0)
                rr = pl.ds(pl.multiple_of(j * 128 + u * 16, 16), 16)
                kvbuf[pl.ds(pl.multiple_of(zz * 16 + j * 128 + u * 16, 16), 16), :] = (ks * vbuf[sl, rr, :].astype(f32)).astype(bf16)
            rj = pl.ds(pl.multiple_of(j * 128, 128), 128)
            xs[j] = jnp.dot(F_v[...], kvbuf[rj, :], preferred_element_type=f32)
            as_[j] = lax.dot_general(F_v[...], hbuf[sl, :, rj], (((1,), (1,)), ((), ())), preferred_element_type=f32)

        def conv_gen(b):
            re = pl.ds(pl.multiple_of(b * 8, 8), 8)
            im = pl.ds(pl.multiple_of(128 + b * 8, 8), 8)
            prev = None
            for i0 in range(0, NC, BLK):
                acc = {}
                acache = {}
                for j in range(0, i0 + BLK):
                    xr = xs[zz + j, re, :]
                    xi = xs[zz + j, im, :]
                    xsum = xr + xi
                    for i in range(max(i0, j), i0 + BLK):
                        if i - j not in acache:
                            ar = as_[zz + (i - j), re, :]
                            ai = as_[zz + (i - j), im, :]
                            acache[i - j] = (ar, ai, ar + ai)
                        ar, ai, asum = acache[i - j]
                        t_ = (ar * xr, ai * xi, asum * xsum)
                        acc[i] = t_ if i not in acc else tuple(u_ + v_ for u_, v_ in zip(acc[i], t_))
                    yield
                for i in range(i0, i0 + BLK):
                    p1, p2, p3 = acc[i]
                    yr, yi = p1 - p2, (p3 - p1) - p2
                    if prev is None:
                        ybuf[zz + i, re, :] = yr
                        ybuf[zz + i, im, :] = yi
                    else:
                        ybuf[zz + i, re, :] = yr - sgn * prev[1]
                        ybuf[zz + i, im, :] = yi + sgn * prev[0]
                    prev = (yr, yi)

        def conv(b):
            for _ in conv_gen(b):
                pass

        dv = jnp.broadcast_to(tapbuf[t, 4:5, :], (128, 128))

        def inv(i):
            y = jnp.dot(G_v[...], ybuf[i].astype(bf16), preferred_element_type=f32)
            rr = pl.ds(pl.multiple_of(i * 128, 128), 128)
            kv = kvbuf[rr, :].astype(f32)
            qq = qbuf[sl, rr, :].astype(f32)
            bobuf[sl, rr, :] = (qq * (y + kv * dv)).astype(bf16)

        P0, PZ, PE = (1, (0, 3, 6, 9, 12, 15), 1)
        assert P0 + len(PZ) + PE == 8
        nxt = iter(range(8))
        for _ in range(P0):
            adot(32 + 8 * t + next(nxt))
        for z in range(NC):
            spec(z)
        for z in range(16):
            if z in PZ:
                adot(32 + 8 * t + next(nxt))
            conv(z)
        for z in range(NC):
            inv(z)
        for _ in range(PE):
            adot(32 + 8 * t + next(nxt))
        sc_.__exit__(None, None, None)
        o_dma(t).start()

        @pl.when(t + 2 < NT)
        def _():
            for cp in in_dmas(t + 2):
                cp.start()
        return 0
    if '0' != '1':
        with scope('phase1'):
            lax.fori_loop(0, NT, tile, 0)
    else:
        x1.start(); m0.start()

    mid_ = scope('mid'); mid_.__enter__()
    x1.wait()
    m0.wait()

    def fill_cur(s):
        rpos = pl.multiple_of((SEG * s + ROFF) % RING, 32)
        for sl in range(96):
            cur[sl] = pltpu.bitcast(ring[sl, pl.ds(rpos, SEG), :], u32)
    fill_cur(0)

    mid_.__exit__(None, None, None)
    scale = E ** -0.5
    L2 = 2 * (SEG + M)
    ri = lax.broadcasted_iota(jnp.int32, (L2, L2), 0)
    ci = lax.broadcasted_iota(jnp.int32, (L2, L2), 1)

    def head_and_pos(i):
        is_mem = i >= 2 * SEG
        hd = jnp.where(is_mem, (i - 2 * SEG) // M, i // SEG)
        return is_mem, hd, i % SEG
    r_mem, r_hd, r_pos = head_and_pos(ri)
    c_mem, c_hd, c_pos = head_and_pos(ci)
    same_head = r_hd == c_hd
    visible = r_mem | c_mem | (c_pos <= r_pos)
    keep = same_head & visible
    fill = jnp.where(same_head, -1e9, -jnp.inf).astype(f32)

    def step(s, mem, tail=False, split=False):
        fresh = FILL - M * (NSEG - 1 - s)
        final = s == NSEG - 1
        xrow = pl.multiple_of(PRO + FILL * s, 8)
        xin = x_v[pl.ds(xrow, FILL), :]
        lhs = jnp.concatenate([mem.astype(bf16), xin], axis=0)
        wpos = pl.multiple_of((FILL * s) % RING, 8)
        prow = pl.multiple_of(jnp.maximum(FILL * (s - 1), 0), 8)
        lo_scr[M:, :] = obuf_x[pl.ds(prow, FILL), :]
        parts, S_, P_, O_ = {}, {}, {}, {}

        newx = {}

        early = {}
        for k_ in range(8 if split else 0):
            for n_ in range(KM):
                sl = EORD[n_ % 3] * 32 + n_ // 3
                w = pltpu.bitcast(wqkv[pl.ds(sl * WS + 64 * k_, 64), :], bf16)
                y = jnp.dot(lhs[:, 128 * k_:128 * (k_ + 1)], w, preferred_element_type=f32)
                early[sl] = y if k_ == 0 else early[sl] + y

        def st_qkv(j):
            ps = {}
            for m in QORD:
                sl = m * 32 + j
                if sl in early:
                    y = early.pop(sl)
                else:
                    w = pltpu.bitcast(wqkv[pl.ds(sl * WS, 512), :], bf16)
                    y = jnp.dot(lhs, w, preferred_element_type=f32)
                ring[sl, pl.ds(wpos, FILL), :] = y[M:].astype(bf16)
                if tail:
                    newx[sl] = y[M:]
                ps[m] = y[:M]
            parts[j] = ps

        npos = pl.multiple_of((SEG * (s + 1) + ROFF) % RING, 32)

        def refill(sl):
            cur[sl] = pltpu.bitcast(ring[sl, pl.ds(npos, SEG), :], u32)

        def refills(p_, where):
            for j in (2 * p_, 2 * p_ + 1):
                for m in range(3):
                    if REF[m] == where:
                        refill(m * 32 + j)

        def tokens(sl):
            c_ = pltpu.bitcast(cur[sl], bf16)
            if tail:
                o_ = c_.astype(f32)
                n_ = newx.pop(sl)
                f0, f1, f2 = n_[0:8], n_[8:16], n_[16:24]
                c_ = jnp.concatenate([
                    o_[0:8],
                    jnp.where(fresh == 24, f0, o_[8:16]),
                    jnp.where(fresh == 24, f1, jnp.where(fresh == 16, f0, o_[16:24])),
                    jnp.where(fresh == 24, f2, jnp.where(fresh == 16, f1, jnp.where(fresh == 8, f0, o_[24:32]))),
                ], axis=0).astype(bf16)
            return c_

        def pair(m, p_):
            ja, jb = 2 * p_, 2 * p_ + 1
            mm = jnp.concatenate([parts[ja][m], parts[jb][m]], axis=0).astype(bf16)
            return jnp.concatenate([tokens(m * 32 + ja), tokens(m * 32 + jb), mm], axis=0)

        def st_qk(p_):
            q, k = pair(0, p_), pair(1, p_)
            S_[p_] = lax.dot_general(q, k, (((1,), (1,)), ((), ())), preferred_element_type=f32)
            refills(p_, 'k')

        def st_sm(p_):
            sc = jnp.where(keep, S_.pop(p_) * scale, fill)
            e = jnp.exp(sc - jnp.max(sc, axis=-1, keepdims=True))
            P_[p_] = (e / jnp.sum(e, axis=-1, keepdims=True)).astype(bf16)
            refills(p_, 's')

        def st_pv(p_):
            O_[p_] = jnp.dot(P_.pop(p_), pair(2, p_), preferred_element_type=f32)
            refills(p_, 'p')

        def st_ost(p_):
            o = O_.pop(p_)
            refills(p_, 'o')
            for z, j in enumerate((2 * p_, 2 * p_ + 1)):
                obuf_x[pl.ds(pl.multiple_of(SEG * s, 32), SEG), j * E:(j + 1) * E] = o[z * SEG:(z + 1) * SEG].astype(bf16)
                om = o[2 * SEG + z * M:2 * SEG + (z + 1) * M].astype(bf16)
                if tail:
                    om = jnp.where(final, obuf_x[pl.ds(S - EPI - M, M), j * E:(j + 1) * E], om)
                lo_scr[0:M, j * E:(j + 1) * E] = om

        accs = {}

        def st_o(t, j0, j1):
            acc = accs.get(t)
            for j in range(j0, j1):
                hh = head_of_slot(j)
                w = pltpu.bitcast(wo[t, pl.ds(hh * 64, 64), :], bf16)
                y = jnp.dot(lo_scr[:, j * E:(j + 1) * E], w, preferred_element_type=f32)
                acc = y if acc is None else acc + y
            accs[t] = acc

        A, B_, C_, D_ = SKEW
        ou = {}
        for (j0, j1), slots in OCFG:
            assert 2 * ((j1 - 1) // 2) + 1 + D_ < min(slots)
            for t_, sl_ in enumerate(slots):
                ou.setdefault(sl_, []).append((t_, j0, j1))
        last = max(max(ou), H - 1 + D_)

        def due(t, lag):
            u = t - lag - 1
            return u // 2 if (u >= 0 and u % 2 == 0 and u // 2 < H // 2) else None
        for t in range(last + 1):
            for what in LORD:
                if what == 'q':
                    if t < H:
                        st_qkv(t)
                elif what == 'o':
                    for u in ou.get(t, []):
                        st_o(*u)
                else:
                    lag, fn = ((A, st_qk), (B_, st_sm), (C_, st_pv), (D_, st_ost))[int(what)]
                    p_ = due(t, lag)
                    if p_ is not None:
                        fn(p_)
        y = jnp.concatenate([accs[t] for t in range(8)], axis=1)
        obuf[pl.ds(prow, FILL), :] = y[M:].astype(bf16)
        if tail:
            obuf[pl.ds(S - EPI - M, M), :] = y[:M].astype(bf16)
        return y[:M]

    NLOOP = NSEG - 4

    def main_steps(u, mem):
        for i in range(UN):
            mem = step(u * UN + i, mem, split=i > 0)
        done = (u + 1) * UN - 1

        @pl.when((done % 8 < UN) & (done >= 8))
        def _():
            a_dma(done // 8 - 1).start()
        return mem

    with scope('steps'):
        mem = lax.fori_loop(0, NLOOP // UN, main_steps, mem_v[...].astype(f32))
        lax.fori_loop(NLOOP, NSEG, lambda s_, m_: step(s_, m_, tail=True), mem)

    r0 = S - EPI
    e0 = (NT - 1) * 8 * FILL
    tail = pltpu.make_async_copy(obuf.at[pl.ds(e0, r0 - e0)], out_hbm.at[pl.ds(e0, r0 - e0), pl.ds(0, D)], osem.at[1])
    tail.start()

    def e_dma(t):
        cols = pl.ds(pl.multiple_of(t * 128, 128), 128)
        return pltpu.make_async_copy(obuf.at[pl.ds(r0, EPI), cols], out_hbm.at[pl.ds(r0, EPI), cols], osem.at[2])

    def epi(t):
        acc = None
        for j in range(H):
            hh = head_of_slot(j)
            w = pltpu.bitcast(wo[t, pl.ds(hh * 64, 64), :], bf16)
            y = jnp.dot(obuf_x[pl.ds(r0, EPI), j * E:(j + 1) * E], w, preferred_element_type=f32)
            acc = y if acc is None else acc + y
        obuf[pl.ds(r0, EPI), pl.ds(pl.multiple_of(t * 128, 128), 128)] = acc.astype(bf16)

    def epis(u, _):
        for i in range(EU):
            epi(u * EU + i)
            e_dma(u * EU + i).start()
        return 0
    with scope('epi'):
        lax.fori_loop(0, 8 // EU, epis, 0)
    post_ = scope('post'); post_.__enter__()
    for c in range(NT - 1):
        a_dma(c).wait()
    o_dma(NT - 2).wait()
    o_dma(NT - 1).wait()
    tail.wait()
    for t in range(8):
        e_dma(t).wait()
    post_.__exit__(None, None, None)


@jax.jit
def run(A_x, A_mem0, A_Wq, A_Wk, A_Wv, A_Wo, B_q, B_k, B_v, B_shift_k, B_ssm_k, B_ssm_D):
    F, G = dft_consts()
    anyspec = pl.BlockSpec(memory_space=pl.ANY)
    vm = pl.BlockSpec(memory_space=pltpu.VMEM)
    out = pl.pallas_call(
        kernel,
        out_shape=jax.ShapeDtypeStruct((S, 2 * D), bf16),
        in_specs=[anyspec] * 10 + [vm] * 4, out_specs=anyspec,
        scratch_shapes=[
            pltpu.VMEM((S, D), bf16),
            pltpu.VMEM((8, PRO // 2, 128), u32),
            pltpu.VMEM((M, D), bf16),
            pltpu.VMEM((96 * WS, E), u32),
            pltpu.VMEM((8, 2048, 128), u32),
            pltpu.VMEM((2, D, 16, E), bf16),
            pltpu.VMEM((H * E, D), bf16),
            pltpu.VMEM((96, RING, E), bf16),
            pltpu.VMEM((S, H * E), bf16),
            pltpu.VMEM((S, D), bf16),
            pltpu.VMEM((32, H * E), bf16),
            pltpu.VMEM((96, SEG // 2, E), u32),
            pltpu.SemaphoreType.DMA((6,)),
            pltpu.SemaphoreType.DMA((3,)),
            pltpu.SemaphoreType.DMA((NQ,)),
            pltpu.SemaphoreType.DMA((NQ,)),
            pltpu.VMEM((16, PRO, E), f32),
            pltpu.VMEM((2, S, 128), bf16), pltpu.VMEM((2, S, 128), bf16), pltpu.VMEM((2, 128, S), bf16),
            pltpu.VMEM((2, S, 128), bf16), pltpu.VMEM((2, S, 128), bf16),
            pltpu.VMEM((S + 8, 128), f32), pltpu.VMEM((S, 128), bf16),
            pltpu.VMEM((NC, 256, 128), f32), pltpu.VMEM((NC, 256, 128), f32),
            pltpu.VMEM((NC, 256, 128), f32), pltpu.VMEM((NT, 8, 128), f32),
            pltpu.SemaphoreType.DMA((5, 2)),
        ],
        compiler_params=pltpu.CompilerParams(vmem_limit_bytes=120 * 1024 * 1024),
        name="fused",
    )(A_x.reshape(S, D), A_mem0.reshape(M, D), A_Wq, A_Wk, A_Wv, A_Wo.reshape(H * E, D),
      B_k.reshape(S, D), B_v.reshape(S, D), B_q.reshape(S, D), B_ssm_k, B_shift_k.T, B_ssm_D.reshape(8, 128), F, G)
    return out.reshape(1, S, 2 * D)


def pallas_concat_heads__memory_aug_recurrent_mem_tr__ssm_conv_h3__prompt_kernel(
    A_x, A_mem0, A_Wq, A_Wk, A_Wv, A_Wo, A_seg_len,
    B_q, B_k, B_v, B_shift_k, B_ssm_k, B_ssm_D,
):
    assert A_seg_len == SEG
    return run(A_x, A_mem0, A_Wq, A_Wk, A_Wv, A_Wo, B_q, B_k, B_v, B_shift_k, B_ssm_k, B_ssm_D)
```

```python
import jax
import jax.numpy as jnp
import numpy as np
import ml_dtypes
from jax import lax
from jax.experimental import pallas as pl
from jax.experimental.pallas import tpu as pltpu

S, D, H, E, M, SEG = 2048, 1024, 32, 128, 8, 32
NSEG = S // SEG
FILL = 24
PRO = S - FILL * NSEG
EPI = S - FILL * (NSEG - 1) - M
RING = 576
ROFF = 64
WS = 516
C = 128
NC = S // C
NT = D // 128
SKEW = tuple(int(c) for c in '1,1,4,4'.split(','))
OCFG = [((0, 24), [29, 30, 31, 32, 33, 34, 35, 36]), ((24, 32), [40] * 8)]
BLK = int('4')
RLU = int('16')
MD = int('1')
KUX = int('8')
NA = int('4')
PIECES = (128, 128, 256, 512)
KUM = int('16')
KM = int('6')
UN = int('3')
QORD = tuple(int(c) for c in '021')
LORD = 'qo0123'
EORD = tuple(int(c) for c in '012')
REF = 'kkp'
EU = int('2')
POFF = tuple(sum(PIECES[:i]) for i in range(len(PIECES)))
import contextlib
SCOPES = '0' == '1'
SL = ''.split(',')
scope = lambda n: jax.named_scope(n) if n in SL else contextlib.nullcontext()
NQ = len(PIECES)
bf16, f32, u32 = jnp.bfloat16, jnp.float32, jnp.uint32


def head_of_slot(j):
    return (j // 16) * 16 + 2 * (j % 8) + ((j // 8) % 2)


def dft_consts():
    k = np.arange(C)[:, None].astype(np.float64)
    t = np.arange(C)[None, :].astype(np.float64)
    th = np.pi * (2 * k + 1) * t / (2 * C)
    F = np.concatenate([np.cos(th), -np.sin(th)], 0)
    G = np.concatenate([np.cos(th).T, -np.sin(th).T], 1) / C
    return F.astype(ml_dtypes.bfloat16), G.astype(ml_dtypes.bfloat16)


def kernel(x_hbm, mem0_hbm, wq_hbm, wk_hbm, wv_hbm, wo_hbm, k_hbm, v_hbm, q_hbm, h_hbm, sk_v, d_v, F_v, G_v,
           out_hbm,
           x_v, xp, mem_v, wqkv, wo, wstage, wostage, ring, obuf_x, obuf, lo_scr, cur, sems, osem, qsem, xsem, pacc,
           kbuf, vbuf, hbuf, qbuf, bobuf, kf, kvbuf, xs, as_, ybuf, tapbuf, bsem):
    LO = 0xFFFF
    HI = np.uint32(0xFFFF0000)
    sgn = (1 - 2 * (lax.broadcasted_iota(jnp.int32, (8, 128), 0) % 2)).astype(f32)

    def in_dmas(t):
        sl = t % 2
        c0 = pl.multiple_of(t * 128, 128)
        return [pltpu.make_async_copy(k_hbm.at[:, pl.ds(c0, 128)], kbuf.at[sl], bsem.at[0, sl]),
                pltpu.make_async_copy(v_hbm.at[:, pl.ds(c0, 128)], vbuf.at[sl], bsem.at[1, sl]),
                pltpu.make_async_copy(h_hbm.at[pl.ds(c0, 128), :], hbuf.at[sl], bsem.at[2, sl]),
                pltpu.make_async_copy(q_hbm.at[:, pl.ds(c0, 128)], qbuf.at[sl], bsem.at[3, sl]),
                pltpu.make_async_copy(wo_hbm.at[pl.ds(pl.multiple_of(t * 512, 512), 512)], wostage.at[sl], bsem.at[5, sl])]

    def o_dma(t):
        sl = t % 2
        return pltpu.make_async_copy(bobuf.at[sl], out_hbm.at[:, pl.ds(pl.multiple_of(D + t * 128, 128), 128)], bsem.at[4, sl])

    def wdma(c, slot, src):
        return pltpu.make_async_copy(src.at[:, pl.ds((c % 2) * 16, 16), :], wstage.at[slot], sems.at[slot])

    def start_w(c, slot):
        for m, src in enumerate((wq_hbm, wk_hbm, wv_hbm)):
            @pl.when(c // 2 == m)
            def _():
                wdma(c, slot, src).start()

    def a_dma(c):
        rows = pl.ds(pl.multiple_of(c * 8 * FILL, 8), 8 * FILL)
        return pltpu.make_async_copy(obuf.at[rows], out_hbm.at[rows, pl.ds(0, D)], osem.at[0])

    x1 = pltpu.make_async_copy(x_hbm.at[pl.ds(PRO, S - PRO)], x_v.at[pl.ds(PRO, S - PRO)], sems.at[3])
    m0 = pltpu.make_async_copy(mem0_hbm, mem_v, sems.at[4])
    pre_ = scope('pre'); pre_.__enter__()

    def w0_dma(i):
        rows = pl.ds(POFF[i], PIECES[i])
        return pltpu.make_async_copy(wq_hbm.at[rows, pl.ds(0, 16), :], wstage.at[0, rows], qsem.at[i])

    def xq_dma(i):
        cols = pl.ds(POFF[i], PIECES[i])
        return pltpu.make_async_copy(x_hbm.at[pl.ds(0, PRO), cols], x_v.at[pl.ds(0, PRO), cols], xsem.at[i])
    for i in range(NQ):
        xq_dma(i).start()
        w0_dma(i).start()

    kf[0:8, :] = jnp.zeros((8, 128), f32)
    dd = d_v[...].astype(f32)
    sk = sk_v[...].astype(f32)
    for t in range(NT):
        tapbuf[t, 0:4, :] = sk[:, t * 128:(t + 1) * 128]
        tapbuf[t, 4:5, :] = dd[t:t + 1, :]
    obuf_x[pl.ds(0, FILL), :] = jnp.zeros((FILL, H * E), bf16)
    def rl_rows(slot, base, i):
        for j in range(8):
            d = i * 16 + 2 * j
            a = pltpu.bitcast(wstage[slot, d], u32)
            b = pltpu.bitcast(wstage[slot, d + 1], u32)
            ev = (a & LO) | (b << 16)
            od = (a >> 16) | (b & HI)
            r = base + i * 8 + j
            wqkv[pl.ds(r, 8, stride=WS), :] = ev
            wqkv[pl.ds(r + 8 * WS, 8, stride=WS), :] = od

    def adot(sl_):
        wv = pltpu.bitcast(wqkv[pl.ds(sl_ * WS, 512), :], bf16)
        xx = jnp.concatenate([pltpu.bitcast(xp[kk], bf16) for kk in range(8)], axis=1)
        y = jnp.dot(xx, wv, preferred_element_type=f32)
        ring[sl_, pl.ds(ROFF, PRO), :] = y.astype(bf16)

    def relayout(c, slot, after_wait=None):
        with scope('wwait'):
            wdma(c, slot, wq_hbm).wait()
        if after_wait is not None:
            after_wait()
        base = c * 16 * WS

        def rl(i, _):
            for r_ in range(RLU):
                rl_rows(slot, base, i * RLU + r_)
            return 0
        lax.fori_loop(0, D // 16 // RLU, rl, 0)

    def more_dmas():
        start_w(1, 1)
    for i in range(NQ):
        with scope('qw%d' % i):
            xq_dma(i).wait()
            w0_dma(i).wait()
        if i == MD:
            more_dmas()
        RQ = PIECES[i]
        KU = max(1, min(KUX, KUM * 128 // RQ))
        kks = range(POFF[i] // 128, (POFF[i] + RQ) // 128)
        for kk in kks:
            xp[kk, 0:PRO // 2, :] = pltpu.bitcast(x_v[0:PRO, kk * 128:(kk + 1) * 128], u32)

        RLQ = min(RLU, RQ // 16)

        def rlq(u, _, i=i, RLQ=RLQ):
            for r_ in range(RLQ):
                rl_rows(0, 0, POFF[i] // 16 + u * RLQ + r_)
            return 0
        if RQ // 16 // RLQ == 1:
            rlq(0, 0)
        else:
            lax.fori_loop(0, RQ // 16 // RLQ, rlq, 0)

        if i == NQ - 1:
            start_w(2, 0)

        def part(u, _, i=i, kks=kks, KU=KU, RQ=RQ):
            for r_ in range(KU):
                sl_ = u * KU + r_
                wv = pltpu.bitcast(wqkv[pl.ds(sl_ * WS + POFF[i] // 2, RQ // 2), :], bf16)
                xx = jnp.concatenate([pltpu.bitcast(xp[kk], bf16) for kk in kks], axis=1)
                y = jnp.dot(xx, wv, preferred_element_type=f32)
                if i == 0:
                    pacc[sl_] = y
                elif i < NQ - 1:
                    pacc[sl_] = pacc[sl_] + y
                else:
                    ring[sl_, pl.ds(ROFF, PRO), :] = (pacc[sl_] + y).astype(bf16)
            return 0
        with scope('qp%d' % i):
            if KU == 16:
                part(0, 0)
            else:
                lax.fori_loop(0, 16 // KU, part, 0)

    def first_inputs():
        for t_ in range(2):
            for cp in in_dmas(t_):
                cp.start()
    relayout(1, 1, first_inputs)

    NG = 16 // NA
    NR = (D // 16) // (NG // 2)

    def slots16(g, _):
        late = g >= NG // 2

        @pl.when(g == NG // 2)
        def _():
            wdma(2, 0, wq_hbm).wait()
            start_w(3, 1)
        slot = jnp.where(late, 0, 1)
        base = jnp.where(late, 2, 1) * (16 * WS)
        for a_ in range(NA):
            adot(16 + g * NA + a_)
            for r_ in range(NR // NA):
                rl_rows(slot, base, (g % (NG // 2)) * NR + a_ * (NR // NA) + r_)
        return 0
    with scope('g16'):
        lax.fori_loop(0, NG, slots16, 0)
    pre_.__exit__(None, None, None)
    def tile(t, _):
        sl = t % 2
        c = t + 1 - (t >= 3).astype(jnp.int32) - (t >= 5).astype(jnp.int32)

        @pl.when(t >= 1)
        def _():
            o_dma(t - 1).start()

        @pl.when((t >= 1) & (t + 1 < NT))
        def _():
            for cp in in_dmas(t + 1):
                cp.start()

        @pl.when(t >= 2)
        def _():
            o_dma(t - 2).wait()


        @pl.when(t == 0)
        def _():
            start_w(4, 0)

        @pl.when((t >= 2) & (t % 2 == 0))
        def _():
            with scope('rl'):
                relayout(c, c % 2)

            @pl.when(t == 2)
            def _():
                start_w(5, 1)

        @pl.when(t == 5)
        def _():
            x1.start()
            m0.start()

        with scope('binwait'):
            for cp in in_dmas(t):
                cp.wait()

        sc_ = scope('main'); sc_.__enter__()

        w = [jnp.broadcast_to(tapbuf[t, j:j + 1, :], (8, 128)) for j in range(4)]
        kf[8:, :] = kbuf[sl].astype(f32)

        zz = jnp.minimum(t, 0)

        def spec(j):
            for u in range(8):
                rows = []
                for hf in range(2):
                    r = j * 128 + u * 16 + hf * 8
                    acc = kf[pl.ds(r + 5, 8), :] * w[3]
                    acc = acc + kf[pl.ds(r + 6, 8), :] * w[2]
                    acc = acc + kf[pl.ds(r + 7, 8), :] * w[1]
                    acc = acc + kf[pl.ds(r + 8, 8), :] * w[0]
                    rows.append(acc)
                ks = jnp.concatenate(rows, axis=0)
                rr = pl.ds(pl.multiple_of(j * 128 + u * 16, 16), 16)
                kvbuf[pl.ds(pl.multiple_of(zz * 16 + j * 128 + u * 16, 16), 16), :] = (ks * vbuf[sl, rr, :].astype(f32)).astype(bf16)
            rj = pl.ds(pl.multiple_of(j * 128, 128), 128)
            xs[j] = jnp.dot(F_v[...], kvbuf[rj, :], preferred_element_type=f32)
            as_[j] = lax.dot_general(F_v[...], hbuf[sl, :, rj], (((1,), (1,)), ((), ())), preferred_element_type=f32)

        def conv_gen(b):
            re = pl.ds(pl.multiple_of(b * 8, 8), 8)
            im = pl.ds(pl.multiple_of(128 + b * 8, 8), 8)
            prev = None
            for i0 in range(0, NC, BLK):
                acc = {}
                acache = {}
                for j in range(0, i0 + BLK):
                    xr = xs[zz + j, re, :]
                    xi = xs[zz + j, im, :]
                    xsum = xr + xi
                    for i in range(max(i0, j), i0 + BLK):
                        if i - j not in acache:
                            ar = as_[zz + (i - j), re, :]
                            ai = as_[zz + (i - j), im, :]
                            acache[i - j] = (ar, ai, ar + ai)
                        ar, ai, asum = acache[i - j]
                        t_ = (ar * xr, ai * xi, asum * xsum)
                        acc[i] = t_ if i not in acc else tuple(u_ + v_ for u_, v_ in zip(acc[i], t_))
                    yield
                for i in range(i0, i0 + BLK):
                    p1, p2, p3 = acc[i]
                    yr, yi = p1 - p2, (p3 - p1) - p2
                    if prev is None:
                        ybuf[zz + i, re, :] = yr
                        ybuf[zz + i, im, :] = yi
                    else:
                        ybuf[zz + i, re, :] = yr - sgn * prev[1]
                        ybuf[zz + i, im, :] = yi + sgn * prev[0]
                    prev = (yr, yi)

        def conv(b):
            for _ in conv_gen(b):
                pass

        dv = jnp.broadcast_to(tapbuf[t, 4:5, :], (128, 128))

        def inv(i):
            y = jnp.dot(G_v[...], ybuf[i].astype(bf16), preferred_element_type=f32)
            rr = pl.ds(pl.multiple_of(i * 128, 128), 128)
            kv = kvbuf[rr, :].astype(f32)
            qq = qbuf[sl, rr, :].astype(f32)
            bobuf[sl, rr, :] = (qq * (y + kv * dv)).astype(bf16)

        P0, PZ, PE = (1, (0, 3, 6, 9, 12, 15), 1)
        assert P0 + len(PZ) + PE == 8
        nxt = iter(range(8))
        WP = 'b'

        def wcopy(r0, r1):
            for r_ in range(r0, r1):
                for n in range(8):
                    wo[n, pl.ds(pl.multiple_of(t * 256 + r_ * 8, 8), 8), :] = pltpu.bitcast(wostage[sl, r_ * 16:(r_ + 1) * 16, n * 128:(n + 1) * 128], u32)
        if WP == 'b':
            wcopy(0, 32)
        for _ in range(P0):
            adot(32 + 8 * t + next(nxt))
        for z in range(NC):
            spec(z)
            if WP == 's':
                wcopy(2 * z, 2 * z + 2)
        for z in range(16):
            if z in PZ:
                adot(32 + 8 * t + next(nxt))
            conv(z)
            if WP == 'c':
                wcopy(2 * z, 2 * z + 2)
        for z in range(NC):
            inv(z)
            if WP == 'i':
                wcopy(2 * z, 2 * z + 2)
        for _ in range(PE):
            adot(32 + 8 * t + next(nxt))
        if WP == 'e':
            wcopy(0, 32)
        sc_.__exit__(None, None, None)
        return 0
    if '0' != '1':
        with scope('phase1'):
            lax.fori_loop(0, NT, tile, 0)
        o_dma(NT - 1).start()
    else:
        x1.start(); m0.start()

    mid_ = scope('mid'); mid_.__enter__()
    x1.wait()
    m0.wait()

    def fill_cur(s):
        rpos = pl.multiple_of((SEG * s + ROFF) % RING, 32)
        for sl in range(96):
            cur[sl] = pltpu.bitcast(ring[sl, pl.ds(rpos, SEG), :], u32)
    fill_cur(0)

    mid_.__exit__(None, None, None)
    scale = E ** -0.5
    L2 = 2 * (SEG + M)
    ri = lax.broadcasted_iota(jnp.int32, (L2, L2), 0)
    ci = lax.broadcasted_iota(jnp.int32, (L2, L2), 1)

    def head_and_pos(i):
        is_mem = i >= 2 * SEG
        hd = jnp.where(is_mem, (i - 2 * SEG) // M, i // SEG)
        return is_mem, hd, i % SEG
    r_mem, r_hd, r_pos = head_and_pos(ri)
    c_mem, c_hd, c_pos = head_and_pos(ci)
    same_head = r_hd == c_hd
    visible = r_mem | c_mem | (c_pos <= r_pos)
    keep = same_head & visible
    fill = jnp.where(same_head, -1e9, -jnp.inf).astype(f32)

    def step(s, mem, tail=False, split=False):
        fresh = FILL - M * (NSEG - 1 - s)
        final = s == NSEG - 1
        xrow = pl.multiple_of(PRO + FILL * s, 8)
        xin = x_v[pl.ds(xrow, FILL), :]
        lhs = jnp.concatenate([mem.astype(bf16), xin], axis=0)
        wpos = pl.multiple_of((FILL * s) % RING, 8)
        prow = pl.multiple_of(jnp.maximum(FILL * (s - 1), 0), 8)
        lo_scr[M:, :] = obuf_x[pl.ds(prow, FILL), :]
        parts, S_, P_, O_ = {}, {}, {}, {}

        newx = {}

        early = {}
        for k_ in range(8 if split else 0):
            for n_ in range(KM):
                sl = EORD[n_ % 3] * 32 + n_ // 3
                w = pltpu.bitcast(wqkv[pl.ds(sl * WS + 64 * k_, 64), :], bf16)
                y = jnp.dot(lhs[:, 128 * k_:128 * (k_ + 1)], w, preferred_element_type=f32)
                early[sl] = y if k_ == 0 else early[sl] + y

        def st_qkv(j):
            ps = {}
            for m in QORD:
                sl = m * 32 + j
                if sl in early:
                    y = early.pop(sl)
                else:
                    w = pltpu.bitcast(wqkv[pl.ds(sl * WS, 512), :], bf16)
                    y = jnp.dot(lhs, w, preferred_element_type=f32)
                ring[sl, pl.ds(wpos, FILL), :] = y[M:].astype(bf16)
                if tail:
                    newx[sl] = y[M:]
                ps[m] = y[:M]
            parts[j] = ps

        npos = pl.multiple_of((SEG * (s + 1) + ROFF) % RING, 32)

        def refill(sl):
            cur[sl] = pltpu.bitcast(ring[sl, pl.ds(npos, SEG), :], u32)

        def refills(p_, where):
            for j in (2 * p_, 2 * p_ + 1):
                for m in range(3):
                    if REF[m] == where:
                        refill(m * 32 + j)

        def tokens(sl):
            c_ = pltpu.bitcast(cur[sl], bf16)
            if tail:
                o_ = c_.astype(f32)
                n_ = newx.pop(sl)
                f0, f1, f2 = n_[0:8], n_[8:16], n_[16:24]
                c_ = jnp.concatenate([
                    o_[0:8],
                    jnp.where(fresh == 24, f0, o_[8:16]),
                    jnp.where(fresh == 24, f1, jnp.where(fresh == 16, f0, o_[16:24])),
                    jnp.where(fresh == 24, f2, jnp.where(fresh == 16, f1, jnp.where(fresh == 8, f0, o_[24:32]))),
                ], axis=0).astype(bf16)
            return c_

        def pair(m, p_):
            ja, jb = 2 * p_, 2 * p_ + 1
            mm = jnp.concatenate([parts[ja][m], parts[jb][m]], axis=0).astype(bf16)
            return jnp.concatenate([tokens(m * 32 + ja), tokens(m * 32 + jb), mm], axis=0)

        def st_qk(p_):
            q, k = pair(0, p_), pair(1, p_)
            S_[p_] = lax.dot_general(q, k, (((1,), (1,)), ((), ())), preferred_element_type=f32)
            refills(p_, 'k')

        def st_sm(p_):
            sc = jnp.where(keep, S_.pop(p_) * scale, fill)
            e = jnp.exp(sc - jnp.max(sc, axis=-1, keepdims=True))
            P_[p_] = (e / jnp.sum(e, axis=-1, keepdims=True)).astype(bf16)
            refills(p_, 's')

        def st_pv(p_):
            O_[p_] = jnp.dot(P_.pop(p_), pair(2, p_), preferred_element_type=f32)
            refills(p_, 'p')

        def st_ost(p_):
            o = O_.pop(p_)
            refills(p_, 'o')
            for z, j in enumerate((2 * p_, 2 * p_ + 1)):
                obuf_x[pl.ds(pl.multiple_of(SEG * s, 32), SEG), j * E:(j + 1) * E] = o[z * SEG:(z + 1) * SEG].astype(bf16)
                om = o[2 * SEG + z * M:2 * SEG + (z + 1) * M].astype(bf16)
                if tail:
                    om = jnp.where(final, obuf_x[pl.ds(S - EPI - M, M), j * E:(j + 1) * E], om)
                lo_scr[0:M, j * E:(j + 1) * E] = om

        accs = {}

        def st_o(t, j0, j1):
            acc = accs.get(t)
            for j in range(j0, j1):
                hh = head_of_slot(j)
                w = pltpu.bitcast(wo[t, pl.ds(hh * 64, 64), :], bf16)
                y = jnp.dot(lo_scr[:, j * E:(j + 1) * E], w, preferred_element_type=f32)
                acc = y if acc is None else acc + y
            accs[t] = acc

        A, B_, C_, D_ = SKEW
        ou = {}
        for (j0, j1), slots in OCFG:
            assert 2 * ((j1 - 1) // 2) + 1 + D_ < min(slots)
            for t_, sl_ in enumerate(slots):
                ou.setdefault(sl_, []).append((t_, j0, j1))
        last = max(max(ou), H - 1 + D_)

        def due(t, lag):
            u = t - lag - 1
            return u // 2 if (u >= 0 and u % 2 == 0 and u // 2 < H // 2) else None
        for t in range(last + 1):
            for what in LORD:
                if what == 'q':
                    if t < H:
                        st_qkv(t)
                elif what == 'o':
                    for u in ou.get(t, []):
                        st_o(*u)
                else:
                    lag, fn = ((A, st_qk), (B_, st_sm), (C_, st_pv), (D_, st_ost))[int(what)]
                    p_ = due(t, lag)
                    if p_ is not None:
                        fn(p_)
        y = jnp.concatenate([accs[t] for t in range(8)], axis=1)
        obuf[pl.ds(prow, FILL), :] = y[M:].astype(bf16)
        if tail:
            obuf[pl.ds(S - EPI - M, M), :] = y[:M].astype(bf16)
        return y[:M]

    NLOOP = NSEG - 4

    def main_steps(u, mem):
        for i in range(UN):
            mem = step(u * UN + i, mem, split=i > 0)
        done = (u + 1) * UN - 1

        @pl.when((done % 8 < UN) & (done >= 8))
        def _():
            a_dma(done // 8 - 1).start()
        return mem

    with scope('steps'):
        mem = lax.fori_loop(0, NLOOP // UN, main_steps, mem_v[...].astype(f32))
        lax.fori_loop(NLOOP, NSEG, lambda s_, m_: step(s_, m_, tail=True), mem)

    r0 = S - EPI
    e0 = (NT - 1) * 8 * FILL
    tail = pltpu.make_async_copy(obuf.at[pl.ds(e0, r0 - e0)], out_hbm.at[pl.ds(e0, r0 - e0), pl.ds(0, D)], osem.at[1])
    tail.start()

    def e_dma(t):
        cols = pl.ds(pl.multiple_of(t * 128, 128), 128)
        return pltpu.make_async_copy(obuf.at[pl.ds(r0, EPI), cols], out_hbm.at[pl.ds(r0, EPI), cols], osem.at[2])

    def epi(t):
        acc = None
        for j in range(H):
            hh = head_of_slot(j)
            w = pltpu.bitcast(wo[t, pl.ds(hh * 64, 64), :], bf16)
            y = jnp.dot(obuf_x[pl.ds(r0, EPI), j * E:(j + 1) * E], w, preferred_element_type=f32)
            acc = y if acc is None else acc + y
        obuf[pl.ds(r0, EPI), pl.ds(pl.multiple_of(t * 128, 128), 128)] = acc.astype(bf16)

    def epis(u, _):
        for i in range(EU):
            epi(u * EU + i)
            e_dma(u * EU + i).start()
        return 0
    with scope('epi'):
        lax.fori_loop(0, 8 // EU, epis, 0)
    post_ = scope('post'); post_.__enter__()
    for c in range(NT - 1):
        a_dma(c).wait()
    o_dma(NT - 2).wait()
    o_dma(NT - 1).wait()
    tail.wait()
    for t in range(8):
        e_dma(t).wait()
    post_.__exit__(None, None, None)


@jax.jit
def run(A_x, A_mem0, A_Wq, A_Wk, A_Wv, A_Wo, B_q, B_k, B_v, B_shift_k, B_ssm_k, B_ssm_D):
    F, G = dft_consts()
    anyspec = pl.BlockSpec(memory_space=pl.ANY)
    vm = pl.BlockSpec(memory_space=pltpu.VMEM)
    out = pl.pallas_call(
        kernel,
        out_shape=jax.ShapeDtypeStruct((S, 2 * D), bf16),
        in_specs=[anyspec] * 10 + [vm] * 4, out_specs=anyspec,
        scratch_shapes=[
            pltpu.VMEM((S, D), bf16),
            pltpu.VMEM((8, PRO // 2, 128), u32),
            pltpu.VMEM((M, D), bf16),
            pltpu.VMEM((96 * WS, E), u32),
            pltpu.VMEM((8, 2048, 128), u32),
            pltpu.VMEM((2, D, 16, E), bf16),
            pltpu.VMEM((2, 512, D), bf16),
            pltpu.VMEM((96, RING, E), bf16),
            pltpu.VMEM((S, H * E), bf16),
            pltpu.VMEM((S, D), bf16),
            pltpu.VMEM((32, H * E), bf16),
            pltpu.VMEM((96, SEG // 2, E), u32),
            pltpu.SemaphoreType.DMA((5,)),
            pltpu.SemaphoreType.DMA((3,)),
            pltpu.SemaphoreType.DMA((NQ,)),
            pltpu.SemaphoreType.DMA((NQ,)),
            pltpu.VMEM((16, PRO, E), f32),
            pltpu.VMEM((2, S, 128), bf16), pltpu.VMEM((2, S, 128), bf16), pltpu.VMEM((2, 128, S), bf16),
            pltpu.VMEM((2, S, 128), bf16), pltpu.VMEM((2, S, 128), bf16),
            pltpu.VMEM((S + 8, 128), f32), pltpu.VMEM((S, 128), bf16),
            pltpu.VMEM((NC, 256, 128), f32), pltpu.VMEM((NC, 256, 128), f32),
            pltpu.VMEM((NC, 256, 128), f32), pltpu.VMEM((NT, 8, 128), f32),
            pltpu.SemaphoreType.DMA((6, 2)),
        ],
        compiler_params=pltpu.CompilerParams(vmem_limit_bytes=120 * 1024 * 1024),
        name="fused",
    )(A_x.reshape(S, D), A_mem0.reshape(M, D), A_Wq, A_Wk, A_Wv, A_Wo.reshape(H * E, D),
      B_k.reshape(S, D), B_v.reshape(S, D), B_q.reshape(S, D), B_ssm_k, B_shift_k.T, B_ssm_D.reshape(8, 128), F, G)
    return out.reshape(1, S, 2 * D)


def pallas_concat_heads__memory_aug_recurrent_mem_tr__ssm_conv_h3__prompt_kernel(
    A_x, A_mem0, A_Wq, A_Wk, A_Wv, A_Wo, A_seg_len,
    B_q, B_k, B_v, B_shift_k, B_ssm_k, B_ssm_D,
):
    assert A_seg_len == SEG
    return run(A_x, A_mem0, A_Wq, A_Wk, A_Wv, A_Wo, B_q, B_k, B_v, B_shift_k, B_ssm_k, B_ssm_D)
```

```python
import jax
import jax.numpy as jnp
import numpy as np
import ml_dtypes
from jax import lax
from jax.experimental import pallas as pl
from jax.experimental.pallas import tpu as pltpu

S, D, H, E, M, SEG = 2048, 1024, 32, 128, 8, 32
NSEG = S // SEG
FILL = 24
PRO = S - FILL * NSEG
EPI = S - FILL * (NSEG - 1) - M
RING = 576
ROFF = 64
WS = 516
C = 128
NC = S // C
NT = D // 128
SKEW = (1, 1, 4, 4)
OCFG = [((0, 24), [29, 30, 31, 32, 33, 34, 35, 36]), ((24, 32), [40] * 8)]
BLK = 4
RLU = 16
NA = 4
PIECES = (128, 128, 256, 512)
KM = 6
UN = 3
QORD = (0, 2, 1)
LORD = 'qo0123'
EU = 2
POFF = tuple(sum(PIECES[:i]) for i in range(len(PIECES)))
NQ = len(PIECES)
bf16, f32, u32 = jnp.bfloat16, jnp.float32, jnp.uint32


def head_of_slot(j):
    return (j // 16) * 16 + 2 * (j % 8) + ((j // 8) % 2)


def dft_consts():
    k = np.arange(C)[:, None].astype(np.float64)
    t = np.arange(C)[None, :].astype(np.float64)
    th = np.pi * (2 * k + 1) * t / (2 * C)
    F = np.concatenate([np.cos(th), -np.sin(th)], 0)
    G = np.concatenate([np.cos(th).T, -np.sin(th).T], 1) / C
    return F.astype(ml_dtypes.bfloat16), G.astype(ml_dtypes.bfloat16)


def kernel(x_hbm, mem0_hbm, wq_hbm, wk_hbm, wv_hbm, wo_hbm, k_hbm, v_hbm, q_hbm, h_hbm, sk_v, d_v, F_v, G_v,
           out_hbm,
           x_v, xp, mem_v, wqkv, wo, wstage, wostage, ring, obuf_x, obuf, lo_scr, cur, sems, osem, qsem, xsem, pacc,
           kbuf, vbuf, hbuf, qbuf, bobuf, kf, kvbuf, xs, as_, ybuf, tapbuf, bsem):
    LO = 0xFFFF
    HI = np.uint32(0xFFFF0000)
    sgn = (1 - 2 * (lax.broadcasted_iota(jnp.int32, (8, 128), 0) % 2)).astype(f32)

    def in_dmas(t):
        sl = t % 2
        c0 = pl.multiple_of(t * 128, 128)
        return [pltpu.make_async_copy(k_hbm.at[:, pl.ds(c0, 128)], kbuf.at[sl], bsem.at[0, sl]),
                pltpu.make_async_copy(v_hbm.at[:, pl.ds(c0, 128)], vbuf.at[sl], bsem.at[1, sl]),
                pltpu.make_async_copy(h_hbm.at[pl.ds(c0, 128), :], hbuf.at[sl], bsem.at[2, sl]),
                pltpu.make_async_copy(q_hbm.at[:, pl.ds(c0, 128)], qbuf.at[sl], bsem.at[3, sl]),
                pltpu.make_async_copy(wo_hbm.at[pl.ds(pl.multiple_of(t * 512, 512), 512)], wostage.at[sl], bsem.at[5, sl])]

    def o_dma(t):
        sl = t % 2
        return pltpu.make_async_copy(bobuf.at[sl], out_hbm.at[:, pl.ds(pl.multiple_of(D + t * 128, 128), 128)], bsem.at[4, sl])

    def wdma(c, slot, src):
        return pltpu.make_async_copy(src.at[:, pl.ds((c % 2) * 16, 16), :], wstage.at[slot], sems.at[slot])

    def start_w(c, slot):
        for m, src in enumerate((wq_hbm, wk_hbm, wv_hbm)):
            @pl.when(c // 2 == m)
            def _():
                wdma(c, slot, src).start()

    def a_dma(c):
        rows = pl.ds(pl.multiple_of(c * 8 * FILL, 8), 8 * FILL)
        return pltpu.make_async_copy(obuf.at[rows], out_hbm.at[rows, pl.ds(0, D)], osem.at[0])

    x1 = pltpu.make_async_copy(x_hbm.at[pl.ds(PRO, S - PRO)], x_v.at[pl.ds(PRO, S - PRO)], sems.at[3])
    m0 = pltpu.make_async_copy(mem0_hbm, mem_v, sems.at[4])

    def w0_dma(i):
        rows = pl.ds(POFF[i], PIECES[i])
        return pltpu.make_async_copy(wq_hbm.at[rows, pl.ds(0, 16), :], wstage.at[0, rows], qsem.at[i])

    def xq_dma(i):
        cols = pl.ds(POFF[i], PIECES[i])
        return pltpu.make_async_copy(x_hbm.at[pl.ds(0, PRO), cols], x_v.at[pl.ds(0, PRO), cols], xsem.at[i])
    for i in range(NQ):
        xq_dma(i).start()
        w0_dma(i).start()

    kf[0:8, :] = jnp.zeros((8, 128), f32)
    dd = d_v[...].astype(f32)
    sk = sk_v[...].astype(f32)
    for t in range(NT):
        tapbuf[t, 0:4, :] = sk[:, t * 128:(t + 1) * 128]
        tapbuf[t, 4:5, :] = dd[t:t + 1, :]
    obuf_x[pl.ds(0, FILL), :] = jnp.zeros((FILL, H * E), bf16)
    def rl_rows(slot, base, i):
        for j in range(8):
            d = i * 16 + 2 * j
            a = pltpu.bitcast(wstage[slot, d], u32)
            b = pltpu.bitcast(wstage[slot, d + 1], u32)
            ev = (a & LO) | (b << 16)
            od = (a >> 16) | (b & HI)
            r = base + i * 8 + j
            wqkv[pl.ds(r, 8, stride=WS), :] = ev
            wqkv[pl.ds(r + 8 * WS, 8, stride=WS), :] = od

    def adot(sl_):
        wv = pltpu.bitcast(wqkv[pl.ds(sl_ * WS, 512), :], bf16)
        xx = jnp.concatenate([pltpu.bitcast(xp[kk], bf16) for kk in range(8)], axis=1)
        y = jnp.dot(xx, wv, preferred_element_type=f32)
        ring[sl_, pl.ds(ROFF, PRO), :] = y.astype(bf16)

    def relayout(c, slot, after_wait=None):
        wdma(c, slot, wq_hbm).wait()
        if after_wait is not None:
            after_wait()
        base = c * 16 * WS

        def rl(i, _):
            for r_ in range(RLU):
                rl_rows(slot, base, i * RLU + r_)
            return 0
        lax.fori_loop(0, D // 16 // RLU, rl, 0)

    def more_dmas():
        start_w(1, 1)
    for i in range(NQ):
        xq_dma(i).wait()
        w0_dma(i).wait()
        if i == 1:
            more_dmas()
        RQ = PIECES[i]
        KU = min(8, 16 * 128 // RQ)
        kks = range(POFF[i] // 128, (POFF[i] + RQ) // 128)
        for kk in kks:
            xp[kk, 0:PRO // 2, :] = pltpu.bitcast(x_v[0:PRO, kk * 128:(kk + 1) * 128], u32)

        RLQ = min(RLU, RQ // 16)

        def rlq(u, _, i=i, RLQ=RLQ):
            for r_ in range(RLQ):
                rl_rows(0, 0, POFF[i] // 16 + u * RLQ + r_)
            return 0
        if RQ // 16 // RLQ == 1:
            rlq(0, 0)
        else:
            lax.fori_loop(0, RQ // 16 // RLQ, rlq, 0)

        if i == NQ - 1:
            start_w(2, 0)

        def part(u, _, i=i, kks=kks, KU=KU, RQ=RQ):
            for r_ in range(KU):
                sl_ = u * KU + r_
                wv = pltpu.bitcast(wqkv[pl.ds(sl_ * WS + POFF[i] // 2, RQ // 2), :], bf16)
                xx = jnp.concatenate([pltpu.bitcast(xp[kk], bf16) for kk in kks], axis=1)
                y = jnp.dot(xx, wv, preferred_element_type=f32)
                if i == 0:
                    pacc[sl_] = y
                elif i < NQ - 1:
                    pacc[sl_] = pacc[sl_] + y
                else:
                    ring[sl_, pl.ds(ROFF, PRO), :] = (pacc[sl_] + y).astype(bf16)
            return 0
        if KU == 16:
            part(0, 0)
        else:
            lax.fori_loop(0, 16 // KU, part, 0)

    def first_inputs():
        for t_ in range(2):
            for cp in in_dmas(t_):
                cp.start()
    relayout(1, 1, first_inputs)

    NG = 16 // NA
    NR = (D // 16) // (NG // 2)

    def slots16(g, _):
        late = g >= NG // 2

        @pl.when(g == NG // 2)
        def _():
            wdma(2, 0, wq_hbm).wait()
            start_w(3, 1)
        slot = jnp.where(late, 0, 1)
        base = jnp.where(late, 2, 1) * (16 * WS)
        for a_ in range(NA):
            adot(16 + g * NA + a_)
            for r_ in range(NR // NA):
                rl_rows(slot, base, (g % (NG // 2)) * NR + a_ * (NR // NA) + r_)
        return 0
    lax.fori_loop(0, NG, slots16, 0)
    def tile(t, _):
        sl = t % 2
        c = t + 1 - (t >= 3).astype(jnp.int32) - (t >= 5).astype(jnp.int32)

        @pl.when(t >= 1)
        def _():
            o_dma(t - 1).start()

        @pl.when((t >= 1) & (t + 1 < NT))
        def _():
            for cp in in_dmas(t + 1):
                cp.start()

        @pl.when(t >= 2)
        def _():
            o_dma(t - 2).wait()

        @pl.when(t == 0)
        def _():
            start_w(4, 0)

        @pl.when((t >= 2) & (t % 2 == 0))
        def _():
            relayout(c, c % 2)

            @pl.when(t == 2)
            def _():
                start_w(5, 1)

        @pl.when(t == 5)
        def _():
            x1.start()
            m0.start()

        for cp in in_dmas(t):
            cp.wait()

        w = [jnp.broadcast_to(tapbuf[t, j:j + 1, :], (8, 128)) for j in range(4)]
        kf[8:, :] = kbuf[sl].astype(f32)

        zz = jnp.minimum(t, 0)

        def spec(j):
            for u in range(8):
                rows = []
                for hf in range(2):
                    r = j * 128 + u * 16 + hf * 8
                    acc = kf[pl.ds(r + 5, 8), :] * w[3]
                    acc = acc + kf[pl.ds(r + 6, 8), :] * w[2]
                    acc = acc + kf[pl.ds(r + 7, 8), :] * w[1]
                    acc = acc + kf[pl.ds(r + 8, 8), :] * w[0]
                    rows.append(acc)
                ks = jnp.concatenate(rows, axis=0)
                rr = pl.ds(pl.multiple_of(j * 128 + u * 16, 16), 16)
                kvbuf[pl.ds(pl.multiple_of(zz * 16 + j * 128 + u * 16, 16), 16), :] = (ks * vbuf[sl, rr, :].astype(f32)).astype(bf16)
            rj = pl.ds(pl.multiple_of(j * 128, 128), 128)
            xs[j] = jnp.dot(F_v[...], kvbuf[rj, :], preferred_element_type=f32)
            as_[j] = lax.dot_general(F_v[...], hbuf[sl, :, rj], (((1,), (1,)), ((), ())), preferred_element_type=f32)

        def conv_gen(b):
            re = pl.ds(pl.multiple_of(b * 8, 8), 8)
            im = pl.ds(pl.multiple_of(128 + b * 8, 8), 8)
            prev = None
            for i0 in range(0, NC, BLK):
                acc = {}
                acache = {}
                for j in range(0, i0 + BLK):
                    xr = xs[zz + j, re, :]
                    xi = xs[zz + j, im, :]
                    xsum = xr + xi
                    for i in range(max(i0, j), i0 + BLK):
                        if i - j not in acache:
                            ar = as_[zz + (i - j), re, :]
                            ai = as_[zz + (i - j), im, :]
                            acache[i - j] = (ar, ai, ar + ai)
                        ar, ai, asum = acache[i - j]
                        t_ = (ar * xr, ai * xi, asum * xsum)
                        acc[i] = t_ if i not in acc else tuple(u_ + v_ for u_, v_ in zip(acc[i], t_))
                    yield
                for i in range(i0, i0 + BLK):
                    p1, p2, p3 = acc[i]
                    yr, yi = p1 - p2, (p3 - p1) - p2
                    if prev is None:
                        ybuf[zz + i, re, :] = yr
                        ybuf[zz + i, im, :] = yi
                    else:
                        ybuf[zz + i, re, :] = yr - sgn * prev[1]
                        ybuf[zz + i, im, :] = yi + sgn * prev[0]
                    prev = (yr, yi)

        def conv(b):
            for _ in conv_gen(b):
                pass

        dv = jnp.broadcast_to(tapbuf[t, 4:5, :], (128, 128))

        def inv(i):
            y = jnp.dot(G_v[...], ybuf[i].astype(bf16), preferred_element_type=f32)
            rr = pl.ds(pl.multiple_of(i * 128, 128), 128)
            kv = kvbuf[rr, :].astype(f32)
            qq = qbuf[sl, rr, :].astype(f32)
            bobuf[sl, rr, :] = (qq * (y + kv * dv)).astype(bf16)

        P0, PZ, PE = (1, (0, 3, 6, 9, 12, 15), 1)
        assert P0 + len(PZ) + PE == 8
        nxt = iter(range(8))

        def wcopy(r0, r1):
            for r_ in range(r0, r1):
                for n in range(8):
                    wo[n, pl.ds(pl.multiple_of(t * 256 + r_ * 8, 8), 8), :] = pltpu.bitcast(wostage[sl, r_ * 16:(r_ + 1) * 16, n * 128:(n + 1) * 128], u32)
        wcopy(0, 32)
        for _ in range(P0):
            adot(32 + 8 * t + next(nxt))
        for z in range(NC):
            spec(z)
        for z in range(16):
            if z in PZ:
                adot(32 + 8 * t + next(nxt))
            conv(z)
        for z in range(NC):
            inv(z)
        for _ in range(PE):
            adot(32 + 8 * t + next(nxt))
        return 0
    lax.fori_loop(0, NT, tile, 0)
    o_dma(NT - 1).start()
    x1.wait()
    m0.wait()

    def fill_cur(s):
        rpos = pl.multiple_of((SEG * s + ROFF) % RING, 32)
        for sl in range(96):
            cur[sl] = pltpu.bitcast(ring[sl, pl.ds(rpos, SEG), :], u32)
    fill_cur(0)

    scale = E ** -0.5
    L2 = 2 * (SEG + M)
    ri = lax.broadcasted_iota(jnp.int32, (L2, L2), 0)
    ci = lax.broadcasted_iota(jnp.int32, (L2, L2), 1)

    def head_and_pos(i):
        is_mem = i >= 2 * SEG
        hd = jnp.where(is_mem, (i - 2 * SEG) // M, i // SEG)
        return is_mem, hd, i % SEG
    r_mem, r_hd, r_pos = head_and_pos(ri)
    c_mem, c_hd, c_pos = head_and_pos(ci)
    same_head = r_hd == c_hd
    visible = r_mem | c_mem | (c_pos <= r_pos)
    keep = same_head & visible
    fill = jnp.where(same_head, -1e9, -jnp.inf).astype(f32)

    def step(s, mem, tail=False, split=False):
        fresh = FILL - M * (NSEG - 1 - s)
        final = s == NSEG - 1
        xrow = pl.multiple_of(PRO + FILL * s, 8)
        xin = x_v[pl.ds(xrow, FILL), :]
        lhs = jnp.concatenate([mem.astype(bf16), xin], axis=0)
        wpos = pl.multiple_of((FILL * s) % RING, 8)
        prow = pl.multiple_of(jnp.maximum(FILL * (s - 1), 0), 8)
        lo_scr[M:, :] = obuf_x[pl.ds(prow, FILL), :]
        parts, S_, P_, O_ = {}, {}, {}, {}

        newx = {}

        early = {}
        for k_ in range(8 if split else 0):
            for n_ in range(KM):
                sl = (n_ % 3) * 32 + n_ // 3
                w = pltpu.bitcast(wqkv[pl.ds(sl * WS + 64 * k_, 64), :], bf16)
                y = jnp.dot(lhs[:, 128 * k_:128 * (k_ + 1)], w, preferred_element_type=f32)
                early[sl] = y if k_ == 0 else early[sl] + y

        def st_qkv(j):
            ps = {}
            for m in QORD:
                sl = m * 32 + j
                if sl in early:
                    y = early.pop(sl)
                else:
                    w = pltpu.bitcast(wqkv[pl.ds(sl * WS, 512), :], bf16)
                    y = jnp.dot(lhs, w, preferred_element_type=f32)
                ring[sl, pl.ds(wpos, FILL), :] = y[M:].astype(bf16)
                if tail:
                    newx[sl] = y[M:]
                ps[m] = y[:M]
            parts[j] = ps

        npos = pl.multiple_of((SEG * (s + 1) + ROFF) % RING, 32)

        def refill(sl):
            cur[sl] = pltpu.bitcast(ring[sl, pl.ds(npos, SEG), :], u32)

        def refills(p_, ms):
            for j in (2 * p_, 2 * p_ + 1):
                for m in ms:
                    refill(m * 32 + j)

        def tokens(sl):
            c_ = pltpu.bitcast(cur[sl], bf16)
            if tail:
                o_ = c_.astype(f32)
                n_ = newx.pop(sl)
                f0, f1, f2 = n_[0:8], n_[8:16], n_[16:24]
                c_ = jnp.concatenate([
                    o_[0:8],
                    jnp.where(fresh == 24, f0, o_[8:16]),
                    jnp.where(fresh == 24, f1, jnp.where(fresh == 16, f0, o_[16:24])),
                    jnp.where(fresh == 24, f2, jnp.where(fresh == 16, f1, jnp.where(fresh == 8, f0, o_[24:32]))),
                ], axis=0).astype(bf16)
            return c_

        def pair(m, p_):
            ja, jb = 2 * p_, 2 * p_ + 1
            mm = jnp.concatenate([parts[ja][m], parts[jb][m]], axis=0).astype(bf16)
            return jnp.concatenate([tokens(m * 32 + ja), tokens(m * 32 + jb), mm], axis=0)

        def st_qk(p_):
            q, k = pair(0, p_), pair(1, p_)
            S_[p_] = lax.dot_general(q, k, (((1,), (1,)), ((), ())), preferred_element_type=f32)
            refills(p_, (0, 1))

        def st_sm(p_):
            sc = jnp.where(keep, S_.pop(p_) * scale, fill)
            e = jnp.exp(sc - jnp.max(sc, axis=-1, keepdims=True))
            P_[p_] = (e / jnp.sum(e, axis=-1, keepdims=True)).astype(bf16)

        def st_pv(p_):
            O_[p_] = jnp.dot(P_.pop(p_), pair(2, p_), preferred_element_type=f32)
            refills(p_, (2,))

        def st_ost(p_):
            o = O_.pop(p_)
            for z, j in enumerate((2 * p_, 2 * p_ + 1)):
                obuf_x[pl.ds(pl.multiple_of(SEG * s, 32), SEG), j * E:(j + 1) * E] = o[z * SEG:(z + 1) * SEG].astype(bf16)
                om = o[2 * SEG + z * M:2 * SEG + (z + 1) * M].astype(bf16)
                if tail:
                    om = jnp.where(final, obuf_x[pl.ds(S - EPI - M, M), j * E:(j + 1) * E], om)
                lo_scr[0:M, j * E:(j + 1) * E] = om

        accs = {}

        def st_o(t, j0, j1):
            acc = accs.get(t)
            for j in range(j0, j1):
                hh = head_of_slot(j)
                w = pltpu.bitcast(wo[t, pl.ds(hh * 64, 64), :], bf16)
                y = jnp.dot(lo_scr[:, j * E:(j + 1) * E], w, preferred_element_type=f32)
                acc = y if acc is None else acc + y
            accs[t] = acc

        A, B_, C_, D_ = SKEW
        ou = {}
        for (j0, j1), slots in OCFG:
            assert 2 * ((j1 - 1) // 2) + 1 + D_ < min(slots)
            for t_, sl_ in enumerate(slots):
                ou.setdefault(sl_, []).append((t_, j0, j1))
        last = max(max(ou), H - 1 + D_)

        def due(t, lag):
            u = t - lag - 1
            return u // 2 if (u >= 0 and u % 2 == 0 and u // 2 < H // 2) else None
        for t in range(last + 1):
            for what in LORD:
                if what == 'q':
                    if t < H:
                        st_qkv(t)
                elif what == 'o':
                    for u in ou.get(t, []):
                        st_o(*u)
                else:
                    lag, fn = ((A, st_qk), (B_, st_sm), (C_, st_pv), (D_, st_ost))[int(what)]
                    p_ = due(t, lag)
                    if p_ is not None:
                        fn(p_)
        y = jnp.concatenate([accs[t] for t in range(8)], axis=1)
        obuf[pl.ds(prow, FILL), :] = y[M:].astype(bf16)
        if tail:
            obuf[pl.ds(S - EPI - M, M), :] = y[:M].astype(bf16)
        return y[:M]

    NLOOP = NSEG - 4

    def main_steps(u, mem):
        for i in range(UN):
            mem = step(u * UN + i, mem, split=i > 0)
        done = (u + 1) * UN - 1

        @pl.when((done % 8 < UN) & (done >= 8))
        def _():
            a_dma(done // 8 - 1).start()
        return mem

    mem = lax.fori_loop(0, NLOOP // UN, main_steps, mem_v[...].astype(f32))
    lax.fori_loop(NLOOP, NSEG, lambda s_, m_: step(s_, m_, tail=True), mem)

    r0 = S - EPI
    e0 = (NT - 1) * 8 * FILL
    tail = pltpu.make_async_copy(obuf.at[pl.ds(e0, r0 - e0)], out_hbm.at[pl.ds(e0, r0 - e0), pl.ds(0, D)], osem.at[1])
    tail.start()

    def e_dma(t):
        cols = pl.ds(pl.multiple_of(t * 128, 128), 128)
        return pltpu.make_async_copy(obuf.at[pl.ds(r0, EPI), cols], out_hbm.at[pl.ds(r0, EPI), cols], osem.at[2])

    def epi(t):
        acc = None
        for j in range(H):
            hh = head_of_slot(j)
            w = pltpu.bitcast(wo[t, pl.ds(hh * 64, 64), :], bf16)
            y = jnp.dot(obuf_x[pl.ds(r0, EPI), j * E:(j + 1) * E], w, preferred_element_type=f32)
            acc = y if acc is None else acc + y
        obuf[pl.ds(r0, EPI), pl.ds(pl.multiple_of(t * 128, 128), 128)] = acc.astype(bf16)

    def epis(u, _):
        for i in range(EU):
            epi(u * EU + i)
            e_dma(u * EU + i).start()
        return 0
    lax.fori_loop(0, 8 // EU, epis, 0)
    for c in range(NT - 1):
        a_dma(c).wait()
    o_dma(NT - 2).wait()
    o_dma(NT - 1).wait()
    tail.wait()
    for t in range(8):
        e_dma(t).wait()


@jax.jit
def run(A_x, A_mem0, A_Wq, A_Wk, A_Wv, A_Wo, B_q, B_k, B_v, B_shift_k, B_ssm_k, B_ssm_D):
    F, G = dft_consts()
    anyspec = pl.BlockSpec(memory_space=pl.ANY)
    vm = pl.BlockSpec(memory_space=pltpu.VMEM)
    out = pl.pallas_call(
        kernel,
        out_shape=jax.ShapeDtypeStruct((S, 2 * D), bf16),
        in_specs=[anyspec] * 10 + [vm] * 4, out_specs=anyspec,
        scratch_shapes=[
            pltpu.VMEM((S, D), bf16),
            pltpu.VMEM((8, PRO // 2, 128), u32),
            pltpu.VMEM((M, D), bf16),
            pltpu.VMEM((96 * WS, E), u32),
            pltpu.VMEM((8, 2048, 128), u32),
            pltpu.VMEM((2, D, 16, E), bf16),
            pltpu.VMEM((2, 512, D), bf16),
            pltpu.VMEM((96, RING, E), bf16),
            pltpu.VMEM((S, H * E), bf16),
            pltpu.VMEM((S, D), bf16),
            pltpu.VMEM((32, H * E), bf16),
            pltpu.VMEM((96, SEG // 2, E), u32),
            pltpu.SemaphoreType.DMA((5,)),
            pltpu.SemaphoreType.DMA((3,)),
            pltpu.SemaphoreType.DMA((NQ,)),
            pltpu.SemaphoreType.DMA((NQ,)),
            pltpu.VMEM((16, PRO, E), f32),
            pltpu.VMEM((2, S, 128), bf16), pltpu.VMEM((2, S, 128), bf16), pltpu.VMEM((2, 128, S), bf16),
            pltpu.VMEM((2, S, 128), bf16), pltpu.VMEM((2, S, 128), bf16),
            pltpu.VMEM((S + 8, 128), f32), pltpu.VMEM((S, 128), bf16),
            pltpu.VMEM((NC, 256, 128), f32), pltpu.VMEM((NC, 256, 128), f32),
            pltpu.VMEM((NC, 256, 128), f32), pltpu.VMEM((NT, 8, 128), f32),
            pltpu.SemaphoreType.DMA((6, 2)),
        ],
        compiler_params=pltpu.CompilerParams(vmem_limit_bytes=120 * 1024 * 1024),
        name="fused",
    )(A_x.reshape(S, D), A_mem0.reshape(M, D), A_Wq, A_Wk, A_Wv, A_Wo.reshape(H * E, D),
      B_k.reshape(S, D), B_v.reshape(S, D), B_q.reshape(S, D), B_ssm_k, B_shift_k.T, B_ssm_D.reshape(8, 128), F, G)
    return out.reshape(1, S, 2 * D)


def pallas_concat_heads__memory_aug_recurrent_mem_tr__ssm_conv_h3__prompt_kernel(
    A_x, A_mem0, A_Wq, A_Wk, A_Wv, A_Wo, A_seg_len,
    B_q, B_k, B_v, B_shift_k, B_ssm_k, B_ssm_D,
):
    assert A_seg_len == SEG
    return run(A_x, A_mem0, A_Wq, A_Wk, A_Wv, A_Wo, B_q, B_k, B_v, B_shift_k, B_ssm_k, B_ssm_D)
```
